```python
import jax
import jax.numpy as jnp

def _softmax(x, axis=-1):
    return jax.nn.softmax(x, axis=axis)
def _gelu(x):
    return jax.nn.gelu(x, approximate=True)
def _silu(x):
    return jax.nn.silu(x)
def _sigmoid(x):
    return jax.nn.sigmoid(x)
def _layernorm(x, axis=-1, eps=1e-5):
    m = jnp.mean(x, axis=axis, keepdims=True)
    v = jnp.var(x, axis=axis, keepdims=True)
    return (x - m) / jnp.sqrt(v + eps)
def _scatter_add(tgt, idx, src, axis=0):
    return tgt.at[idx].add(src)
def _segment_sum(src, seg, n):
    return jax.ops.segment_sum(src, seg, n)
class _Rng:
    def __init__(self, key):
        self._k = key
    def _next(self):
        self._k, sub = jax.random.split(self._k)
        return sub
    def normal(self, shape):
        return jax.random.normal(self._next(), shape, dtype=jnp.bfloat16)
    def randint(self, lo, hi, shape):
        return jax.random.randint(self._next(), shape, lo, hi, dtype=jnp.int32)
    def uniform(self, shape, lo=0.0, hi=1.0):
        return jax.random.uniform(self._next(), shape, jnp.bfloat16, lo, hi)
    def permutation(self, n):
        return jax.random.permutation(self._next(), n)


kernel_name = 'sequential_preLN__sliding_local_dilated__glu_gated_geglu__prompt'

def setup_inputs():
    _rng = _Rng(jax.random.key(int.from_bytes(__import__("os").urandom(4), "little")))
    _w = (lambda a: (lambda t: t.astype(jnp.bfloat16) if jnp.issubdtype(t.dtype, jnp.floating) else t)(jnp.asarray(a)))
    def _A_setup():
        B, S, D = 1, 2048, 1024
        return {
            "x": _w((lambda *s: _rng.normal(s) * 0.05)(B, S, D)),
            "wqkv": _w((lambda *s: _rng.normal(s) * 0.05)(D, 3 * D)),
            "wo": _w((lambda *s: _rng.normal(s) * 0.05)(D, D)),
        }
    _A_in = _A_setup()

    def _B_setup():
        B, S, Dm, Df = 1, 2048, 1024, 3584
        return {
            "x": _w((lambda *s: _rng.normal(s) * 0.05)(B, S, Dm)),
            "w_gate": _w((lambda *s: _rng.normal(s) * 0.05)(Dm, Df) * (Dm ** -0.5)),
            "w_up": _w((lambda *s: _rng.normal(s) * 0.05)(Dm, Df) * (Dm ** -0.5)),
            "w_down": _w((lambda *s: _rng.normal(s) * 0.05)(Df, Dm) * (Df ** -0.5)),
        }
    _B_in = _B_setup()

    return {
        "A_x": _A_in["x"],
        "A_wqkv": _A_in["wqkv"],
        "A_wo": _A_in["wo"],
        "B_x": _B_in["x"],
        "B_w_gate": _B_in["w_gate"],
        "B_w_up": _B_in["w_up"],
        "B_w_down": _B_in["w_down"],
    }

def reference(A_x, A_wqkv, A_wo, B_x, B_w_gate, B_w_up, B_w_down):
    def _A_ref(x, wqkv, wo):
        B, S, D = x.shape
        H = 32; Dh = D // H
        W, dil = 8, 2
        qkv = (lambda x, *d: x.transpose(*d))((x @ wqkv).reshape(B, S, 3, H, Dh), 2, 0, 3, 1, 4)
        q, k, v = qkv[0], qkv[1], qkv[2]
        scale = Dh ** -0.5
        pos = jnp.arange(S)
        off = jnp.arange(W) * dil
        idx = pos[:, None] - off[None, :]
        mask = idx >= 0
        idx_c = jnp.where(mask, idx, 0).reshape(-1)
        kg = k[:, :, idx_c, :].reshape(B, H, S, W, Dh)
        vg = v[:, :, idx_c, :].reshape(B, H, S, W, Dh)
        logits = jnp.einsum("bhsd,bhswd->bhsw", q, kg) * scale
        logits = jnp.where(mask[None, None, :, :], logits, -1e9)
        attn = _softmax(logits, axis=-1)
        o = jnp.einsum("bhsw,bhswd->bhsd", attn, vg)
        return (lambda x, *d: x.transpose(*d))(o, 0, 2, 1, 3).reshape(B, S, D) @ wo

    def _B_ref(x, w_gate, w_up, w_down):
        g = jnp.einsum("bsd,df->bsf", x, w_gate)
        u = jnp.einsum("bsd,df->bsf", x, w_up)
        h = _gelu(g) * u
        return jnp.einsum("bsf,fd->bsd", h, w_down)

    x = A_x
    h = x + _A_ref(_layernorm(x, axis=-1), A_wqkv, A_wo)
    h2 = h + _B_ref(_layernorm(h, axis=-1), B_w_gate, B_w_up, B_w_down)
    return h2
```

```python
import functools
import math
import jax
import jax.numpy as jnp
from jax import lax
import jax.experimental.pallas as pl
import jax.experimental.pallas.tpu as pltpu

H = 32
W = 8
DIL = 2
HALO = 16
EPS = 1e-5
LANES = 128


def _swap_digits(tiles):
    tiles = list(tiles)
    lane = lax.broadcasted_iota(jnp.int32, tiles[0].shape, 1)
    for tb, lb in ((1, 4), (2, 8), (4, 16)):
        m = (lane & lb) != 0
        for a in range(8):
            if a & tb:
                continue
            A, B = tiles[a], tiles[a | tb]
            tiles[a] = jnp.where(m, pltpu.roll(B, lb, 1), A)
            tiles[a | tb] = jnp.where(m, B, pltpu.roll(A, LANES - lb, 1))
    return tiles


def _ln(x):
    m = jnp.mean(x, axis=-1, keepdims=True)
    c = x - m
    v = jnp.mean(c * c, axis=-1, keepdims=True)
    return c * lax.rsqrt(v + EPS)


def _gelu(x):
    c = math.sqrt(2.0 / math.pi)
    inner = x * (c + (c * 0.044715) * (x * x))
    hx = 0.5 * x
    return hx + hx * jnp.tanh(inner)


def _kernel(x_ref, wqkv_h, wo_h, wg_h, wu_h, wd_h, o_ref,
            wqkv, wo, wg, wu, wd, q_s, k_s, v_s, ao_s, h_s, hn_s, a_s, sems, *, TM, TF, RA):
    i = pl.program_id(0)
    D = wo.shape[0]
    F = wg.shape[1]
    NT = D // LANES
    cps = [pltpu.make_async_copy(s, d, sems.at[n]) for n, (s, d) in enumerate(
        ((wqkv_h, wqkv), (wo_h, wo), (wg_h, wg), (wu_h, wu), (wd_h, wd)))]

    @pl.when(i == 0)
    def _():
        for c in cps:
            c.start()
        cps[0].wait()

        def body(r, _):
            rows = pl.ds(pl.multiple_of(r * 64, 64), 64)
            for p in range(3):
                ts = [pltpu.bitcast(wqkv[rows, pl.ds(p * D + t * LANES, LANES)], jnp.uint32) for t in range(NT)]
                ts = _swap_digits(ts)
                for t in range(NT):
                    wqkv[rows, pl.ds(p * D + t * LANES, LANES)] = pltpu.bitcast(ts[t], jnp.bfloat16)
        lax.fori_loop(0, D // 64, body, None)

    @pl.when(i > 0)
    def _():
        for t in range(NT):
            k_s[t, 0:HALO, :] = k_s[t, TM:TM + HALO, :]
            v_s[t, 0:HALO, :] = v_s[t, TM:TM + HALO, :]

    x = x_ref[...].astype(jnp.float32)
    xn = _ln(x).astype(jnp.bfloat16)
    for p, (dst, off) in enumerate(((q_s, 0), (k_s, HALO), (v_s, HALO))):
        r = jnp.dot(xn, wqkv[:, p * D:(p + 1) * D], preferred_element_type=jnp.float32)
        for t in range(NT):
            dst[t, off:off + TM, :] = r[:, t * LANES:(t + 1) * LANES]

    @pl.when(i == 0)
    def _():
        for t in range(NT):
            k_s[t, 0:HALO, :] = jnp.broadcast_to(k_s[t, HALO:HALO + 1, :], (HALO, LANES))
            v_s[t, 0:HALO, :] = jnp.broadcast_to(v_s[t, HALO:HALO + 1, :], (HALO, LANES))
        cps[1].wait()

    scale = (D // H) ** -0.5
    lane = lax.broadcasted_iota(jnp.int32, (RA, LANES), 1)
    m1 = (lane & 1) != 0
    m2 = (lane & 2) != 0
    for r0 in range(0, TM, RA):
        q = [q_s[t, r0:r0 + RA, :] for t in range(NT)]
        ls = []
        for w in range(W):
            s0 = HALO + r0 - DIL * w
            a = q[0] * k_s[0, s0:s0 + RA, :]
            for t in range(1, NT):
                a = a + q[t] * k_s[t, s0:s0 + RA, :]
            a = a + jnp.where(m1, pltpu.roll(a, 1, 1), pltpu.roll(a, LANES - 1, 1))
            a = a + jnp.where(m2, pltpu.roll(a, 2, 1), pltpu.roll(a, LANES - 2, 1))
            if r0 < DIL * w:
                pos = i * TM + r0 + lax.broadcasted_iota(jnp.int32, (RA, LANES), 0)
                a = jnp.where(pos >= DIL * w, a, -1e9 / scale)
            ls.append(a)
        m = functools.reduce(jnp.maximum, ls)
        ps = [jnp.exp2((a - m) * (scale * math.log2(math.e))) for a in ls]
        inv = 1.0 / functools.reduce(lambda a, b: a + b, ps)
        ps = [p * inv for p in ps]
        os_ = []
        for t in range(NT):
            o = None
            for w in range(W):
                s0 = HALO + r0 - DIL * w
                c = ps[w] * v_s[t, s0:s0 + RA, :]
                o = c if o is None else o + c
            os_.append(pltpu.bitcast(o.astype(jnp.bfloat16), jnp.uint32))
        os_ = _swap_digits(os_)
        for t in range(NT):
            ao_s[r0:r0 + RA, t * LANES:(t + 1) * LANES] = pltpu.bitcast(os_[t], jnp.bfloat16)

    h = x_ref[...].astype(jnp.float32) + jnp.dot(ao_s[...], wo[...], preferred_element_type=jnp.float32)
    h_s[...] = h
    hn_s[...] = _ln(h).astype(jnp.bfloat16)

    @pl.when(i == 0)
    def _():
        cps[2].wait()
        cps[3].wait()
        cps[4].wait()

    for j in range(F // TF):
        cols = slice(j * TF, (j + 1) * TF)
        hn = hn_s[...]
        g = jnp.dot(hn, wg[:, cols], preferred_element_type=jnp.float32)
        u = jnp.dot(hn, wu[:, cols], preferred_element_type=jnp.float32)
        a_s[:, cols] = (_gelu(g) * u).astype(jnp.bfloat16)
    o_ref[...] = (h_s[...] + jnp.dot(a_s[...], wd[...], preferred_element_type=jnp.float32)).astype(o_ref.dtype)


def make(TM=512, TF=512, RA=16, flags=None):
    @jax.jit
    def fn(A_x, A_wqkv, A_wo, B_x, B_w_gate, B_w_up, B_w_down):
        B, S, D = A_x.shape
        F = B_w_gate.shape[1]
        NT = D // LANES
        bf = jnp.bfloat16
        f32 = jnp.float32
        anyspec = pl.BlockSpec(memory_space=pl.ANY)
        out = pl.pallas_call(
            functools.partial(_kernel, TM=TM, TF=TF, RA=RA),
            grid=(S // TM,),
            in_specs=[pl.BlockSpec((TM, D), lambda i: (i, 0))] + [anyspec] * 5,
            out_specs=pl.BlockSpec((TM, D), lambda i: (i, 0)),
            out_shape=jax.ShapeDtypeStruct((S, D), A_x.dtype),
            scratch_shapes=[
                pltpu.VMEM((D, 3 * D), bf), pltpu.VMEM((D, D), bf),
                pltpu.VMEM((D, F), bf), pltpu.VMEM((D, F), bf), pltpu.VMEM((F, D), bf),
                pltpu.VMEM((NT, TM, LANES), f32),
                pltpu.VMEM((NT, TM + HALO, LANES), f32),
                pltpu.VMEM((NT, TM + HALO, LANES), f32),
                pltpu.VMEM((TM, D), bf), pltpu.VMEM((TM, D), f32), pltpu.VMEM((TM, D), bf),
                pltpu.VMEM((TM, F), bf),
                pltpu.SemaphoreType.DMA((5,)),
            ],
            compiler_params=pltpu.CompilerParams(
                dimension_semantics=("arbitrary",), vmem_limit_bytes=120 * 1024 * 1024, flags=flags),
        )(A_x.reshape(S, D), A_wqkv, A_wo, B_w_gate, B_w_up, B_w_down)
        return out.reshape(B, S, D)
    return fn


pallas_sequential_preLN__sliding_local_dilated__glu_gated_geglu__prompt_kernel = make(TM=256)
```

```python
import functools
import math
import jax
import jax.numpy as jnp
from jax import lax
import jax.experimental.pallas as pl
import jax.experimental.pallas.tpu as pltpu

H = 32
W = 8
DIL = 2
HALO = 16
EPS = 1e-5
LANES = 128
BF = jnp.bfloat16
F32 = jnp.float32


def _swap_digits(tiles):
    lane = lax.broadcasted_iota(jnp.int32, tiles[0].shape, 1)
    t = [x if a == 0 else pltpu.roll(x, 4 * a, 1) for a, x in enumerate(tiles)]
    t = [t[(-c) % 8] for c in range(8)]
    for b in (1, 2, 4):
        m = (lane & (4 * b)) != 0
        t = [jnp.where(m, t[(c - b) % 8], t[c]) for c in range(8)]
    return [x if c == 0 else pltpu.roll(x, LANES - 4 * c, 1) for c, x in enumerate(t)]


def _ln(x):
    m = jnp.mean(x, axis=-1, keepdims=True)
    c = x - m
    v = jnp.mean(c * c, axis=-1, keepdims=True)
    return c * lax.rsqrt(v + EPS)


def _gelu(x):
    c = math.sqrt(2.0 / math.pi)
    inner = x * (c + (c * 0.044715) * (x * x))
    hx = 0.5 * x
    return hx + hx * jnp.tanh(inner)


def _lhs7(a11, a12, a21, a22):
    return (a11 + a22, a21 + a22, a11, a22, a11 + a12, a21 - a11, a12 - a22)


def _rhs5(b11, b12, b21, b22):
    return (b11 + b22, b12 - b22, b21 - b11, b11 + b12, b21 + b22)


def _dot(a, b):
    return jnp.dot(a, b, preferred_element_type=F32)


def _strassen(lhs, rhs, init=None, fill=None):
    def m(p):
        r = _dot(lhs(p), rhs(p))
        if fill is not None:
            fill(r)
        return r
    m1 = m(0)
    m4 = m(3)
    c11 = m1 + m4
    m2 = m(1)
    c21 = m2 + m4
    c22 = m1 - m2
    c11 = c11 + m(6)
    m5 = m(4)
    c11 = c11 - m5
    m3 = m(2)
    c12 = m3 + m5
    c22 = c22 + m3
    c22 = c22 + m(5)
    return c11, c12, c21, c22


def _filler(tasks, slots, after=None, lag=1):
    state = [0, 0]
    pend = {}

    def fill(dep=None, flush=False):
        state[0] += 1
        if state[0] in pend:
            after(pend.pop(state[0]))
        target = len(tasks) if flush else min(len(tasks), -(-state[0] * len(tasks) // slots))
        while state[1] < target:
            v = tasks[state[1]](dep)
            dep = None
            if after is not None:
                pend[state[0] + lag] = v
            state[1] += 1
    return fill


def _kernel(x_h, wqkv_h, wo_h, wg_h, wu_h, wd_h, o_h,
            x_s, wa, sg, su, sd, qkv_s, ao_s, xc, oc, h_s, ac, o_s, sems, osem,
            *, TM, TF, RA, TN, TD, AS, RP, PA, PL, PP, EU, PQ, PS, LA, LL, RS):
    S, D = x_h.shape
    F = wg_h.shape[1]
    NT = D // LANES
    NB = S // TM
    HM, HD, HF = TM // 2, D // 2, TF // 2
    NJ = F // TF
    mo = pl.multiple_of

    def quad_cp(n, src, r, c, hr, hc, dst):
        return [pltpu.make_async_copy(src.at[pl.ds(r + a * hr, hr), pl.ds(c + b * hc, hc)],
                                      dst(1 + 2 * a + b), sems.at[n]) for a in range(2) for b in range(2)]
    x0_cp = pltpu.make_async_copy(x_h.at[pl.ds(0, TM)], x_s.at[pl.ds(0, TM)], sems.at[0])
    x1_cp = pltpu.make_async_copy(x_h.at[pl.ds(TM, S - TM)], x_s.at[pl.ds(TM, S - TM)], sems.at[1])
    w_cp = [quad_cp(2 + p, wqkv_h, 0, p * D, HD, HD, lambda n, p=p: wa.at[p, n, pl.ds(0, HD)]) for p in range(3)]
    w_cp.append(quad_cp(5, wo_h, 0, 0, HD, HD, lambda n: wa.at[3, n, pl.ds(0, HD)]))

    def ffn_cp(j):
        c = mo(j * TF, TF)
        cd = pl.ds(mo(j * HF, HF), HF)
        return (quad_cp(6 + j, wg_h, 0, c, HD, HF, lambda n: sg.at[n, pl.ds(0, HD), cd])
                + quad_cp(6 + j, wu_h, 0, c, HD, HF, lambda n: su.at[n, pl.ds(0, HD), cd])
                + quad_cp(6 + j, wd_h, c, 0, HF, HD, lambda n: sd.at[n, cd, :]))

    def start(cs):
        for c in cs:
            c.start()

    def wait(cs):
        for c in cs:
            c.wait()

    zero = [None]

    def pin(ref, lead, row, val):
        ref[(*lead, pl.ds(mo(row + zero[0], 16), 16), slice(0, LANES))] = val[-16:, -LANES:].astype(ref.dtype)

    def ln_task(src, base, r):
        def run(dep):
            if dep is not None and PL & 1:
                pin(src, (), S, dep)
            a = _ln(src[pl.ds(mo(base + r, RA), RA), :].astype(F32))
            b = _ln(src[pl.ds(mo(base + HM + r, RA), RA), :].astype(F32))
            for p, v in enumerate(_lhs7(a[:, :HD], a[:, HD:], b[:, :HD], b[:, HD:])):
                xc[p, pl.ds(r, RA), :] = v.astype(BF)
            return v
        return run

    def combine(get, put):
        vs = [get(n).astype(F32) for n in (1, 2, 3, 4)]
        for n, v in zip((0, 2, 3, 5, 6), _rhs5(*vs)):
            put(n, v.astype(BF))

    def prep_att(p, r, dep=None):
        rows = pl.ds(r, RP)
        hv = {}
        for n in (1, 3):
            t0 = [pltpu.bitcast(wa[p, n + t // 4, rows, (t % 4) * LANES:(t % 4 + 1) * LANES], jnp.uint32)
                  for t in range(NT)]
            ts = [pltpu.bitcast(jnp.where(p < 3, a, b), BF) for a, b in zip(_swap_digits(t0), t0)]
            hv[n] = jnp.concatenate(ts[:NT // 2], axis=1)
            hv[n + 1] = jnp.concatenate(ts[NT // 2:], axis=1)

        def put(n, v):
            wa[p, n, rows, :] = v
        put(1, hv[1])
        put(4, hv[4])
        combine(hv.__getitem__, put)

    def prep(ref, rows, cols, dep):
        if dep is not None and PQ:
            for rf in (sg, su, sd):
                pin(rf, (0,), rf.shape[1] - 16, dep)

        def put(n, v):
            ref[n, rows, cols] = v
        combine(lambda n: ref[n, rows, cols], put)

    def prep_ffn_tasks(j):
        ts = []
        cd = pl.ds(mo(j * HF, HF), HF)
        for r in range(0, HF, PP):
            for ref in (sg, su):
                ts.append(functools.partial(prep, ref, pl.ds(r * HD // HF, PP * HD // HF), cd))
            ts.append(functools.partial(prep, sd, pl.ds(mo(j * HF + r, PP), PP), slice(0, HD)))
        return ts

    def qkv(p, base, fill):
        for c0 in range(0, HD, TN):
            cs = _strassen(lambda n: xc[n], lambda n: wa[p, n, :HD, c0:c0 + TN], fill=fill)
            for n, c in enumerate(cs):
                rows = pl.ds(mo(base + (n // 2) * HM, 8), HM)
                for t in range(TN // LANES):
                    qkv_s[p * NT + ((n % 2) * HD + c0) // LANES + t, rows, :] = (
                        c[:, t * LANES:(t + 1) * LANES])

    scale = (D // H) ** -0.5

    def attn_rows(base, r0, first, dep=None):
        lane = lax.broadcasted_iota(jnp.int32, (RS, LANES), 1)
        m1 = (lane & 1) != 0
        m2 = (lane & 2) != 0
        outs = []
        for rr in range(0, RA, RS):
            ld = lambda t, w: qkv_s[t, pl.ds(base + (HALO + r0 + rr - DIL * w), RS), :]
            q = [ld(t, 0) for t in range(NT)]
            if dep is not None:
                never = lane < zero[0]
                q = [jnp.where(never, dep[-RS:, -LANES:], a) for a in q]
            ls = []
            for w in range(W):
                a = q[0] * ld(NT, w)
                for t in range(1, NT):
                    a = a + q[t] * ld(NT + t, w)
                ls.append(a + jnp.where(m1, pltpu.roll(a, 1, 1), pltpu.roll(a, LANES - 1, 1)))
            if PA == 1 and dep is not None:
                dep = a
            ls = [a + jnp.where(m2, pltpu.roll(a, 2, 1), pltpu.roll(a, LANES - 2, 1)) for a in ls]
            if first:
                pos = base + (r0 + rr) + lax.broadcasted_iota(jnp.int32, (RS, LANES), 0)
                ls = [jnp.where(pos >= DIL * w, a, -1e9 / scale) if w else a for w, a in enumerate(ls)]
            m = functools.reduce(jnp.maximum, ls)
            if PA == 2 and dep is not None:
                dep = m
            ps = [jnp.exp2((a - m) * (scale * math.log2(math.e))) for a in ls]
            inv = 1.0 / functools.reduce(lambda a, b: a + b, ps)
            ps = [p * inv for p in ps]
            os_ = []
            for t in range(NT):
                o = ps[0] * ld(2 * NT + t, 0)
                for w in range(1, W):
                    o = o + ps[w] * ld(2 * NT + t, w)
                os_.append(o)
            outs.append(os_)
        os_ = [pltpu.bitcast(jnp.concatenate(o, axis=0).astype(BF), jnp.uint32) for o in zip(*outs)]
        return jnp.concatenate([pltpu.bitcast(t, BF) for t in _swap_digits(os_)], axis=1)

    def put_oc(r, a, b):
        a, b = a.astype(F32), b.astype(F32)
        for p, v in enumerate(_lhs7(a[:, :HD], a[:, HD:], b[:, :HD], b[:, HD:])):
            oc[p, pl.ds(r, RA), :] = v.astype(BF)

    def attn(base, r0, dep):
        o = attn_rows(base, r0, r0 < HALO, dep if PS else None)
        if r0 < HM:
            ao_s[r0:r0 + RA, :] = o
        else:
            put_oc(r0 - HM, ao_s[r0 - HM:r0 - HM + RA, :], o)
        return o

    def wo_mm(i, fill):
        for c0 in range(0, HD, TN):
            cs = _strassen(lambda n: oc[n], lambda n: wa[3, n, :HD, c0:c0 + TN], fill=fill)
            for n, c in enumerate(cs):
                rows = pl.ds(mo(i * TM + (n // 2) * HM, HM), HM)
                cols = slice((n % 2) * HD + c0, (n % 2) * HD + c0 + TN)
                h_s[rows, cols] = x_s[rows, cols].astype(F32) + c

    def ln_loop(src, base):
        lax.fori_loop(0, HM // RA, lambda r, _: (ln_task(src, base, mo(r * RA, RA))(None), None)[1], None, unroll=4)

    NP = 7 * HD // TN
    x0_cp.start()
    start(w_cp[0])
    x0_cp.wait()
    start(w_cp[1])
    ln_loop(x_s, 0)
    wait(w_cp[0])
    start(w_cp[2])
    lax.fori_loop(0, HD // RP, lambda r, _: prep_att(0, mo(r * RP, RP)), None)

    def p0(p, _):
        for n in range(3):
            @pl.when(p == n)
            def _():
                wait(w_cp[n + 1])
                if n == 0:
                    start(w_cp[3])
                elif n == 1:
                    x1_cp.start()
                else:
                    start(ffn_cp(0))
        qkv(p, HALO, _filler([functools.partial(prep_att, p + 1, r) for r in range(0, HD, RP)], NP))
    lax.fori_loop(0, 3, p0, None)
    for t in range(NT, 3 * NT):
        qkv_s[t, 0:HALO, :] = jnp.broadcast_to(qkv_s[t, HALO:HALO + 1, :], (HALO, LANES))
    x1_cp.wait()
    ln_loop(x_s, TM)

    pin_wa = lambda v: pin(wa, (0, 0), HD, v)
    assert NJ == NB - 1

    def p1(i, _):
        slot = i % 2
        zero[0] = jnp.minimum(i, 0)

        @pl.when(i + 1 < NJ)
        def _():
            start(ffn_cp(i + 1))
        wait(ffn_cp(i))
        base = i * TM
        fa = _filler([functools.partial(attn, base, r0) for r0 in range(0, TM, RA)], int(AS * NP),
                     pin_wa if LA else None, LA)
        fa()
        fp = _filler(prep_ffn_tasks(i), 4 * NP)
        for p in range(3):
            qkv(p, base + (TM + HALO), lambda r: (fa(r), fp(r)))
        fa(flush=True)
        nxt = jnp.minimum(i + 2, NB - 1) * TM
        fl = _filler([ln_task(x_s, nxt, r) for r in range(0, HM, RA)], NP - 3, pin_wa if PL & 2 else None, LL)
        wo_mm(i, lambda r: (fl(r), fp(r)))
        fp(flush=True)
    lax.fori_loop(0, NB - 1, p1, None)

    def last_attn(r, _):
        zero[0] = jnp.minimum(r, 0)
        r = mo(r * RA, RA)
        put_oc(r, *[attn_rows(r, S - TM + d, False) for d in (0, HM)])
    lax.fori_loop(0, HM // RA, last_attn, None, unroll=EU)
    zero[0] = 0
    wo_mm(NB - 1, _filler([ln_task(h_s, 0, r) for r in range(0, HM, RA)], NP - 2))

    def out_cp(i, slot):
        return pltpu.make_async_copy(o_s.at[slot], o_h.at[pl.ds(mo(i * TM, TM), TM)], osem.at[slot])

    def p2(i, _):
        slot = i % 2
        zero[0] = jnp.minimum(i, 0)

        @pl.when(i >= 2)
        def _():
            out_cp(i - 2, slot).wait()
        for j in range(NJ):
            cd = slice(j * HF, (j + 1) * HF)
            g = _strassen(lambda n: xc[n], lambda n: sg[n, :HD, cd])
            g = [_gelu(v) for v in g]
            u = _strassen(lambda n: xc[n], lambda n: su[n, :HD, cd])
            for p, v in enumerate(_lhs7(*[a * b for a, b in zip(g, u)])):
                ac[p, :, cd] = v.astype(BF)
        nxt = jnp.minimum(i + 1, NB - 1) * TM
        fl = _filler([ln_task(h_s, nxt, r) for r in range(0, HM, RA)], 7 * HD // TD - 3,
                     (lambda v: pin(sd, (0,), F // 2, v)) if PL & 2 else None, 1)
        for c0 in range(0, HD, TD):
            cs = _strassen(lambda n: ac[n], lambda n: sd[n, :F // 2, c0:c0 + TD], fill=fl)
            for n, c in enumerate(cs):
                r0 = (n // 2) * HM
                cols = slice((n % 2) * HD + c0, (n % 2) * HD + c0 + TD)
                o_s[slot, r0:r0 + HM, cols] = (h_s[pl.ds(mo(i * TM + r0, HM), HM), cols] + c).astype(BF)
        out_cp(i, slot).start()
    lax.fori_loop(0, NB, p2, None)
    out_cp(NB - 2, 0).wait()
    out_cp(NB - 1, 1).wait()


def make(TM=256, TF=512, RA=16, TN=512, TD=512, AS=2.5, RP=64, PA=0, PL=2, PP=16, EU=2, PQ=1, PS=1, LA=0, LL=2, RS=8, flags=None):
    @jax.jit
    def fn(A_x, A_wqkv, A_wo, B_x, B_w_gate, B_w_up, B_w_down):
        B, S, D = A_x.shape
        F = B_w_gate.shape[1]
        NT = D // LANES
        HM, HD = TM // 2, D // 2
        anyspec = pl.BlockSpec(memory_space=pl.ANY)
        V = pltpu.VMEM
        out = pl.pallas_call(
            functools.partial(_kernel, TM=TM, TF=TF, RA=RA, TN=TN, TD=TD, AS=AS, RP=RP, PA=PA, PL=PL, PP=PP, EU=EU, PQ=PQ, PS=PS, LA=LA, LL=LL, RS=RS),
            in_specs=[anyspec] * 6,
            out_specs=anyspec,
            out_shape=jax.ShapeDtypeStruct((S, D), A_x.dtype),
            scratch_shapes=[
                V((S + 16, D), BF), V((4, 7, HD + 16, HD), BF), V((7, HD + 16, F // 2), BF), V((7, HD + 16, F // 2), BF),
                V((7, F // 2 + 16, HD), BF), V((3 * NT, S + HALO, LANES), F32),
                V((HM, D), BF), V((7, HM, HD), BF), V((7, HM, HD), BF), V((S + 16, D), F32), V((7, HM, F // 2), BF),
                V((2, TM, D), BF),
                pltpu.SemaphoreType.DMA((6 + F // TF,)), pltpu.SemaphoreType.DMA((2,)),
            ],
            compiler_params=pltpu.CompilerParams(vmem_limit_bytes=124 * 1024 * 1024, flags=flags),
        )(A_x.reshape(S, D), A_wqkv, A_wo, B_w_gate, B_w_up, B_w_down)
        return out.reshape(B, S, D)
    return fn


pallas_sequential_preLN__sliding_local_dilated__glu_gated_geglu__prompt_kernel = make()
```

```python
import functools
import math
import jax
import jax.numpy as jnp
from jax import lax
import jax.experimental.pallas as pl
import jax.experimental.pallas.tpu as pltpu

H = 32
W = 8
DIL = 2
HALO = 16
EPS = 1e-5
LANES = 128
RA = 16
RS = 8
BF = jnp.bfloat16
F32 = jnp.float32
U32 = jnp.uint32
SWAPPED = (0, 1, 4)


def _pack(v):
    return pltpu.bitcast(v.astype(BF), U32)


def _mm(a, b):
    return jnp.dot(pltpu.bitcast(a, BF), pltpu.bitcast(b, BF), preferred_element_type=F32)


def _skew(tiles):
    return [x if a == 0 else pltpu.roll(x, 4 * a, 1) for a, x in enumerate(tiles)]


def _unskew(t):
    lane = lax.broadcasted_iota(jnp.int32, t[0].shape, 1)
    t = [t[(-c) % 8] for c in range(8)]
    for b in (1, 2, 4):
        m = (lane & (4 * b)) != 0
        t = [jnp.where(m, t[(c - b) % 8], t[c]) for c in range(8)]
    return [x if c == 0 else pltpu.roll(x, LANES - 4 * c, 1) for c, x in enumerate(t)]


def _ln(x):
    m = jnp.mean(x, axis=-1, keepdims=True)
    c = x - m
    v = jnp.mean(c * c, axis=-1, keepdims=True)
    return c * lax.rsqrt(v + EPS)


def _gelu(x):
    c = math.sqrt(2.0 / math.pi)
    inner = x * (c + (c * 0.044715) * (x * x))
    hx = 0.5 * x
    return hx + hx * jnp.tanh(inner)


def _lhs7(a11, a12, a21, a22):
    return (a11 + a22, a21 + a22, a11, a22, a11 + a12, a21 - a11, a12 - a22)


def _rhs7(b11, b12, b21, b22):
    return (b11 + b22, b11, b12 - b22, b21 - b11, b22, b11 + b12, b21 + b22)


def _two_level(f, blk, swapped=()):
    o = {(r, c): f(blk[r][c], blk[r][2 + c], blk[2 + r][c], blk[2 + r][2 + c]) for r in range(2) for c in range(2)}
    out = []
    for p in range(7):
        s = int(p in swapped)
        out += f(o[0, s][p], o[0, 1 - s][p], o[1, s][p], o[1, 1 - s][p])
    return out


def _combine(m):
    add = lambda a, b: [x + y for x, y in zip(a, b)]
    sub = lambda a, b: [x - y for x, y in zip(a, b)]
    m1 = m(0)
    m4 = m(3)
    c11 = add(m1, m4)
    m2 = m(1)
    c21 = add(m2, m4)
    c22 = sub(m1, m2)
    c11 = add(c11, m(6))
    m5 = m(4)
    c11 = sub(c11, m5)
    m3 = m(2)
    c12 = add(m3, m5)
    c22 = add(c22, m3)
    c22 = add(c22, m(5))
    return c11, c12, c21, c22


def _strassen1(prod, fill):
    def m(p):
        r = prod(p)
        fill(r)
        return [r]
    c = _combine(m)
    return [c[0] + c[1], c[2] + c[3]]


def _strassen2(prod, fill):
    def m(p):
        (a, b), (c, d) = _strassen1(lambda q: prod(7 * p + q), fill)
        return [b, a, d, c] if p in SWAPPED else [a, b, c, d]
    c = _combine(m)
    return [[c[2 * (r // 2) + k // 2][2 * (r % 2) + k % 2] for k in range(4)] for r in range(4)]


def _paced(work, steps, first, last):
    calls = [0]

    def fill(r):
        calls[0] += 1
        if calls[0] == first:
            next(work, None)
        if first <= calls[0] <= last:
            k, n = calls[0] - first, last - first + 1
            rows, tiles = r.shape[0] // RS, r.shape[1] // LANES
            for g in range(-(-k * steps // n), -(-(k + 1) * steps // n)):
                t, a = divmod((g * n - k * steps) * rows * tiles // steps, rows)
                try:
                    work.send(r[a * RS:(a + 1) * RS, t * LANES:(t + 1) * LANES])
                    assert g + 1 < steps
                except StopIteration:
                    assert g + 1 == steps, (g, steps)
    return fill


def _run(work):
    for _ in work:
        pass


def _kernel(x_h, wqkv_h, wo_h, wg_h, wu_h, wd_h, o_h, x_s, wo, sgu, sd, qkv_s, **cfg):
    S, D = x_h.shape
    QF = wd_h.shape[1]
    TM, TN, TD, G, NS = cfg["TM"], cfg["TN"], cfg["TD"], cfg["G"], cfg["NS"]
    NT, NB, NJ = D // LANES, S // TM, QF // LANES
    HM, HD, QM, QD = TM // 2, D // 2, TM // 4, D // 4
    NP = 7 * HD // TN
    mo = pl.multiple_of
    zero = [None]

    def pin(ref, lead, val):
        rows = pl.ds(mo(ref.shape[-2] - RS + zero[0], RS), RS)
        ref[(*lead, rows, slice(0, LANES))] = pltpu.bitcast(val[-RS:, -LANES:], ref.dtype)

    def behind(dep, v):
        lane = lax.broadcasted_iota(jnp.int32, v.shape, 1)
        return jnp.where(lane < zero[0], pltpu.bitcast(dep[-RS:, -LANES:], v.dtype), v)

    def rows2(r, n=RA):
        return pl.ds(r // 2 if isinstance(r, int) else mo(r // 2, RS), n // 2)

    def ld16(dep, v):
        if dep is None:
            return v.astype(F32)
        if v.dtype == BF:
            return pltpu.bitcast(behind(dep, pltpu.bitcast(v, U32)), BF).astype(F32)
        return jnp.concatenate([behind(dep, v[:RS]), behind(dep, v[RS:])], axis=0)

    def ln_stats(src, rows):
        ld = lambda k, t, d: ld16(d, src[pl.ds(mo(rows[k], RA), RA), t * LANES:(t + 1) * LANES])
        add = lambda a, b: a + b
        ms, rs = [], []
        for k in range(len(rows)):
            d = yield
            m = jnp.sum(functools.reduce(add, [ld(k, t, d) for t in range(NT)]), axis=-1, keepdims=True)
            ms.append(jnp.broadcast_to(m * (1.0 / D), (RA, LANES)))
        for k, m in enumerate(ms):
            v = []
            for t in range(NT):
                if t % (NT // 2) == 0:
                    d = yield
                v.append(jnp.square(ld(k, t, d) - m))
            v = jnp.sum(functools.reduce(add, v), axis=-1, keepdims=True)
            rs.append(jnp.broadcast_to(lax.rsqrt(v * (1.0 / D) + EPS), (RA, LANES)))
        yield
        return lambda k, t, d: (ld(k, t, d) - ms[k]) * rs[k]

    def two_level(f, load, put, swapped=()):
        quad = lambda a, b, d: [load(2 * a + r, 2 * b + c, d) for r in range(2) for c in range(2)]

        def inner(p, q):
            for n, v in enumerate(f(q[1], q[0], q[3], q[2]) if p in swapped else f(*q)):
                put(7 * p + n, v)
            return v

        def later(q):
            if cfg["FINE"]:
                d = yield
                return [ld16(d, v) for v in q]
            return q
        q11 = quad(0, 0, (yield))
        inner(2 if f is _lhs7 else 1, q11)
        q22 = quad(1, 1, (yield))
        inner(3 if f is _lhs7 else 4, q22)
        q22 = yield from later(q22)
        inner(0, [a + b for a, b in zip(q11, q22)])
        q12 = quad(0, 1, (yield))
        inner(4 if f is _lhs7 else 5, [a + b for a, b in zip(q11, q12)])
        q12 = yield from later(q12)
        inner(6 if f is _lhs7 else 2, [a - b for a, b in zip(q12, q22)])
        q21 = quad(1, 0, (yield))
        inner(5 if f is _lhs7 else 3, [a - b for a, b in zip(q21, q11)])
        q21 = yield from later(q21)
        return inner(1 if f is _lhs7 else 6, [a + b for a, b in zip(q21, q22)])
    N2 = 7 if cfg["FINE"] else 4

    def phase_a(xc, wa, stg, tmp, fg, fu, fd, xsem, wsem, fsem):
        CH = HD // 4
        CU, CD, CO = QD // NB, QF // NB, HD // NB

        def x_cp(i):
            rows = pl.ds(mo(i * TM, TM), TM)
            return pltpu.make_async_copy(x_h.at[rows], x_s.at[rows], xsem.at[i])

        def w_cp(c):
            return pltpu.make_async_copy(wqkv_h.at[:, pl.ds(mo(c % 4 * CH, CH), CH), pl.ds(mo(c // 4 * D, D), D)],
                                         stg.at[:, pl.ds(mo(c % 4 * CH, CH), CH)], wsem.at[c % 4])
        wo_cp = pltpu.make_async_copy(wo_h, stg, wsem.at[0])

        def f_cp(i):
            s = i % NS
            return [pltpu.make_async_copy(src.at[:, pl.ds(mo(i * n, RA), n)], dst.at[s], fsem.at[s])
                    for src, dst, n in ((wg_h, fg, CU), (wu_h, fu, CU), (wd_h, fd, CD))]

        def ln_work(i, slot, rs, mark=None):
            v = None
            for r in rs:
                tile = yield from ln_stats(x_s, [i * TM + r, i * TM + HM + r])
                if mark is not None and v is not None:
                    mark(v)
                for t in range(NT // 2):
                    d = yield
                    for p, v in enumerate(_lhs7(*[tile(k, n * NT // 2 + t, d) for k in range(2) for n in range(2)])):
                        xc[slot, p, rows2(r), t * LANES:(t + 1) * LANES] = _pack(v)

        def att_work(c):
            for r in range(0, CH, RA):
                for k in range(2):
                    ts = [pltpu.bitcast(stg[k, pl.ds(mo(c % 4 * CH + r, RA), RA), t * LANES:(t + 1) * LANES], U32)
                          for t in range(NT)]
                    tmp[k, rows2(r), :] = jnp.concatenate(_skew(ts), axis=1)
            for r in range(0, CH, RA):
                hv = []
                for k in range(2):
                    d = yield
                    ts = [tmp[k, rows2(r), t * LANES:(t + 1) * LANES] for t in range(NT)]
                    hv.append(_unskew(ts if d is None else [behind(d, v) for v in ts]))
                for t in range(NT // 2):
                    d = yield
                    q = [ld16(d, pltpu.bitcast(hv[k][n * NT // 2 + t], BF)) for k in range(2) for n in range(2)]
                    for n, v in enumerate(_rhs7(*q)):
                        wa[c // 4, n, rows2(c % 4 * CH + r), t * LANES:(t + 1) * LANES] = _pack(v)

        def ffn_work(i):
            s = i % NS
            for e, src in enumerate((fg, fu)):
                for r in range(0, CU, RA):
                    for j in range(NJ):
                        def put(n, v):
                            sgu[j, n, rows2(i * CU + r), e * LANES:(e + 1) * LANES] = _pack(v)
                        yield from two_level(
                            _rhs7, lambda k, n, d: ld16(d, src[s, k, r:r + RA, pl.ds(n * QF + j * LANES, LANES)]),
                            put, SWAPPED)
            for r in range(0, CD, RA):
                for c in range(0, QD, LANES):
                    def put(n, v):
                        sd[n, rows2(i * CD + r), c:c + LANES] = _pack(v)
                    yield from two_level(
                        _rhs7, lambda k, n, d: ld16(d, fd[s, k, r:r + RA, pl.ds(n * QD + c, LANES)]), put, SWAPPED)
            for r in range(0, CO, RA):
                for c in range(0, HD, LANES):
                    d = yield
                    q = [ld16(d, stg[k, pl.ds(mo(i * CO + r, RA), RA), pl.ds(n * HD + c, LANES)])
                         for k in range(2) for n in range(2)]
                    for n, v in enumerate(_rhs7(*q)):
                        wo[n, rows2(i * CO + r), c:c + LANES] = _pack(v)
        ffn_steps = N2 * (2 * CU * NJ + CD * QD // LANES) // RA + CO * HD // (RA * LANES)

        def project(p, i, fill):
            for c0 in range(0, HD, TN):
                cs = _strassen1(lambda n: _mm(xc[i, n], wa[p, n, :HD // 2, c0:c0 + TN]), fill)
                for a in range(2):
                    for b in range(2):
                        for t in range(TN // LANES):
                            qkv_s[p * NT + (b * HD + c0) // LANES + t, pl.ds(mo(i * TM + (HALO + a * HM), RS), HM)] = (
                                cs[a][b][:, t * LANES:(t + 1) * LANES])

        x_cp(0).start()
        w_cp(0).start()
        w_cp(1).start()
        x_cp(0).wait()
        w_cp(2).start()
        lax.fori_loop(0, HM // RA, lambda r, _: _run(ln_work(0, 0, [mo(r * RA, RA)])), None, unroll=4)

        def first_weights(c, _):
            w_cp(c).wait()

            @pl.when(c < 3)
            def _():
                w_cp(c + 3).start()

            @pl.when(c >= 2)
            def _():
                x_cp(c - 1).start()
            _run(att_work(c))
        lax.fori_loop(0, 4, first_weights, None)

        def q_step(i, _):
            zero[0] = jnp.minimum(i, 0)

            @pl.when(i + 6 < 12)
            def _():
                w_cp(i + 6).start()

            @pl.when(i + 3 < NB)
            def _():
                x_cp(i + 3).start()

            @pl.when(i >= NB - NS + 1)
            def _():
                for c in f_cp(i - (NB - NS + 1)):
                    c.start()

            @pl.when(i + 1 < NB)
            def _():
                x_cp(i + 1).wait()
            w_cp(i + 4).wait()
            nxt = jnp.minimum(i + 1, NB - 1)
            fl = _paced(ln_work(nxt, i + 1, range(0, HM, RA), (lambda v: pin(xc, (0, 7), v)) if cfg["PQ"] else None),
                        11 * HM // RA, 1, NP - cfg["LQ"])
            fw = _paced(att_work(i + 4), 6 * CH // RA, 1, NP - cfg["LQ"])
            project(0, i, lambda r: (fl(r), fw(r)))
        lax.fori_loop(0, NB, q_step, None)
        wo_cp.start()

        def kv_step(i, _):
            zero[0] = jnp.minimum(i, 0)

            @pl.when(i + NS - 1 < NB)
            def _():
                for c in f_cp(i + NS - 1):
                    c.start()

            @pl.when(i == 0)
            def _():
                wo_cp.wait()
            for c in f_cp(i):
                c.wait()
            fw = _paced(ffn_work(i), ffn_steps, 1, 2 * NP - cfg['KE'])
            project(1, i, fw)
            project(2, i, fw)
        lax.fori_loop(0, NB, kv_step, None)

    def phase_b(h_s, hc, ac, oc, o_s, osem):
        scale = (D // H) ** -0.5

        def attn_work(base, rs, masked, mark=None):
            lane = lax.broadcasted_iota(jnp.int32, (RS, LANES), 1)

            def ld(r0, t, w):
                return qkv_s[t, pl.ds(base + (HALO + r0 - DIL * w), RS), :]

            def scores(r0):
                ls = [None] * W
                for t in range(NT):
                    d = yield
                    q = ld(r0, t, 0) if d is None else behind(d, ld(r0, t, 0))
                    for w in range(W):
                        c = q * ld(r0, NT + t, w)
                        ls[w] = c if t == 0 else ls[w] + c
                for b in (1, 2):
                    m = (lane & b) != 0
                    ls = [a + jnp.where(m, pltpu.roll(a, b, 1), pltpu.roll(a, LANES - b, 1)) for a in ls]
                if masked and r0 < HALO:
                    pos = base + r0 + lax.broadcasted_iota(jnp.int32, (RS, LANES), 0)
                    ls = [jnp.where(pos >= DIL * w, a, -1e9 / scale) if w else a for w, a in enumerate(ls)]
                m = functools.reduce(jnp.maximum, ls)
                ps = [jnp.exp2((a - m) * (scale * math.log2(math.e))) for a in ls]
                inv = 1.0 / functools.reduce(lambda a, b: a + b, ps)
                return [p * inv for p in ps]

            def values(r0, ps):
                os_ = [None] * NT
                for w, p in enumerate(ps):
                    d = yield
                    p = p if d is None else behind(d, p)
                    for t in range(NT):
                        c = p * ld(r0, 2 * NT + t, w)
                        os_[t] = c if w == 0 else os_[t] + c
                return os_

            starts = [r + k * HM + e for r in rs for k in range(2) for e in range(0, RA, RS)]
            ahead = cfg["AH"] if mark is not None else 1
            ps, outs, halves, v = [], [], [], None
            for n in range(len(starts) + ahead):
                if n < len(starts):
                    ps.append((yield from scores(starts[n])))
                if n >= ahead:
                    outs.append((yield from values(starts[n - ahead], ps.pop(0))))
                if len(outs) == 2:
                    if mark is not None and v is not None:
                        mark(v)
                    halves.append(_unskew(_skew([_pack(jnp.concatenate(o, axis=0)) for o in zip(*outs)])))
                    outs, v = [], halves[-1][-1]
                if len(halves) == 2:
                    for t in range(NT // 2):
                        d = yield
                        q = [ld16(d, pltpu.bitcast(halves[k][e * NT // 2 + t], BF)) for k in range(2) for e in range(2)]
                        dst = starts[n - ahead] - HM - RS
                        for p, v in enumerate(_lhs7(*q)):
                            oc[p, rows2(base + dst if masked else dst), t * LANES:(t + 1) * LANES] = _pack(v)
                    halves = []

        def out_proj(i, slot):
            for c0 in range(0, HD, TN):
                cs = _strassen1(lambda n: _mm(oc[n], wo[n, :, c0:c0 + TN]), lambda r: None)
                for a in range(2):
                    for b in range(2):
                        cols = pl.ds(b * HD + c0, TN)
                        h_s[pl.ds(mo(slot * TM + a * HM, HM), HM), cols] = (
                            x_s[pl.ds(mo(i * TM + a * HM, HM), HM), cols].astype(F32) + cs[a][b])

        def ln_work(slot, rs, mark=None):
            v = None
            for r in rs:
                tile = yield from ln_stats(h_s, [slot * TM + k * QM + r for k in range(4)])
                if mark is not None and v is not None:
                    mark(v)
                for c in range(QD // LANES):
                    def put(p, v):
                        hc[p, rows2(r), c * LANES:(c + 1) * LANES] = _pack(v)
                    v = yield from two_level(_lhs7, lambda k, n, d: tile(k, n * QD // LANES + c, d), put)

        for t in range(NT, 3 * NT):
            qkv_s[t, 0:HALO, :] = jnp.broadcast_to(qkv_s[t, HALO:HALO + 1, :], (HALO, LANES))
        EU = cfg["EU"]

        lax.fori_loop(0, HM // (RA * EU), lambda r, _: _run(attn_work(mo(r * RA * EU, RA), range(0, RA * EU, RA), True)), None)
        out_proj(0, 0)
        lax.fori_loop(0, QM // RA, lambda r, _: _run(ln_work(0, [mo(r * RA, RA)])), None, unroll=2)

        def out_cp(i, slot):
            return pltpu.make_async_copy(o_s.at[slot], o_h.at[pl.ds(mo(i * TM, TM), TM)], osem.at[slot])

        def step(i, _):
            slot = i % 2
            zero[0] = jnp.minimum(i, 0)

            @pl.when(i >= 2)
            def _():
                out_cp(i - 2, slot).wait()
            nxt = jnp.minimum(i + 1, NB - 1)
            fa = _paced(attn_work(nxt * TM, range(0, HM, RA), False, lambda v: pin(hc, (49,), v) if cfg["PA"] else None),
                        (4 * (NT + W) + NT // 2) * HM // RA, cfg["A0"], cfg["A1"])
            for j in range(NJ):
                c = _strassen2(lambda n: _mm(hc[n], sgu[j, n]), fa)
                act = [[_gelu(v[:, :LANES]) * v[:, LANES:] for v in row] for row in c]
                for p, v in enumerate(_two_level(_lhs7, act)):
                    ac[p, :, j * LANES:(j + 1) * LANES] = _pack(v)
            WP, LL = cfg["WP"], cfg["LL"]
            calls = [0]

            def fo(r):
                calls[0] += 1
                if calls[0] == WP:
                    out_proj(nxt, 1 - slot)
            fl = _paced(ln_work(1 - slot, range(0, QM, RA), (lambda v: pin(sd, (0,), v)) if cfg["PL"] else None),
                        (13 + N2 * QD // LANES) * QM // RA, WP + 1, 49 * QD // TD - LL)
            for c0 in range(0, QD, TD):
                cs = _strassen2(lambda n: _mm(ac[n], sd[n, :QF // 2, c0:c0 + TD]),
                                lambda r: (fa(r), fo(r), fl(r)))
                for a in range(4):
                    for b in range(4):
                        cols = pl.ds(b * QD + c0, TD)
                        o_s[slot, a * QM:(a + 1) * QM, cols] = (
                            h_s[pl.ds(mo(slot * TM + a * QM, QM), QM), cols] + cs[a][b]).astype(o_s.dtype)
            out_cp(i, slot).start()
        lax.fori_loop(0, NB, step, None)
        out_cp(NB - 2, 0).wait()
        out_cp(NB - 1, 1).wait()

    V, DMA = pltpu.VMEM, pltpu.SemaphoreType.DMA
    pl.run_scoped(phase_a, V((NB + 1, 8, HM // 2, HD), U32), V((3, 7, HD // 2, HD), U32), V((2, HD, D), BF),
                  V((2, HD // 8, D), U32), V((NS, 4, QD // NB, 4 * QF), BF), V((NS, 4, QD // NB, 4 * QF), BF),
                  V((NS, 4, QF // NB, D), BF), DMA((NB,)), DMA((4,)), DMA((NS,)))
    pl.run_scoped(phase_b, V((2 * TM, D), F32), V((50, QM // 2, QD), U32), V((49, QM // 2, QF), U32),
                  V((7, HM // 2, HD), U32), V((2, TM, D), o_h.dtype), DMA((2,)))


def make(**kw):
    cfg = dict(TM=256, TN=512, TD=256, G=4, NS=2, LQ=1, EU=2, A0=1, A1=343, WP=4, LL=8, KE=1, FINE=1, PQ=1, PA=0, PL=0, AH=1)
    cfg.update(kw)

    @jax.jit
    def fn(A_x, A_wqkv, A_wo, B_x, B_w_gate, B_w_up, B_w_down):
        del B_x
        B, S, D = A_x.shape
        F = B_w_gate.shape[1]
        anyspec = pl.BlockSpec(memory_space=pl.ANY)
        V = pltpu.VMEM
        out = pl.pallas_call(
            functools.partial(_kernel, **cfg),
            in_specs=[anyspec] * 6,
            out_specs=anyspec,
            out_shape=jax.ShapeDtypeStruct((S, D), A_x.dtype),
            scratch_shapes=[
                V((S, D), BF), V((7, D // 4, D // 2), U32), V((F // 4 // LANES, 49, D // 8, 2 * LANES), U32),
                V((49, F // 8 + RS, D // 4), U32), V((3 * D // LANES, S + HALO, LANES), F32),
            ],
            compiler_params=pltpu.CompilerParams(vmem_limit_bytes=126 * 1024 * 1024),
        )(A_x.reshape(S, D), A_wqkv.reshape(2, D // 2, 3 * D), A_wo.reshape(2, D // 2, D),
          B_w_gate.reshape(4, D // 4, F), B_w_up.reshape(4, D // 4, F), B_w_down.reshape(4, F // 4, D))
        return out.reshape(B, S, D)
    return fn


pallas_sequential_preLN__sliding_local_dilated__glu_gated_geglu__prompt_kernel = make()
```

```python
import functools
import math
import jax
import jax.numpy as jnp
from jax import lax
import jax.experimental.pallas as pl
import jax.experimental.pallas.tpu as pltpu

H = 32
W = 8
DIL = 2
HALO = 16
EPS = 1e-5
LANES = 128
RA = 16
RS = 8
BF = jnp.bfloat16
F32 = jnp.float32
U32 = jnp.uint32
SWAPPED = (0, 1, 4)


def _pack(v):
    return pltpu.bitcast(v.astype(BF), U32)


def _mm(a, b):
    return jnp.dot(pltpu.bitcast(a, BF), pltpu.bitcast(b, BF), preferred_element_type=F32)


def _lane_xor(v, b):
    lane = lax.broadcasted_iota(jnp.int32, v.shape, 1)
    return jnp.take_along_axis(v, lane ^ b, axis=1) if b else v


def _skew(tiles):
    return [x if a == 0 else pltpu.roll(x, 4 * a, 1) for a, x in enumerate(tiles)]


def _unskew(t):
    lane = lax.broadcasted_iota(jnp.int32, t[0].shape, 1)
    t = [t[(-c) % 8] for c in range(8)]
    for b in (1, 2, 4):
        m = (lane & (4 * b)) != 0
        t = [jnp.where(m, t[(c - b) % 8], t[c]) for c in range(8)]
    return [x if c == 0 else pltpu.roll(x, LANES - 4 * c, 1) for c, x in enumerate(t)]


def _gelu(x):
    c = math.sqrt(2.0 / math.pi)
    inner = x * (c + (c * 0.044715) * (x * x))
    hx = 0.5 * x
    return hx + hx * jnp.tanh(inner)


def _lhs7(a11, a12, a21, a22):
    return (a11 + a22, a21 + a22, a11, a22, a11 + a12, a21 - a11, a12 - a22)


def _rhs7(b11, b12, b21, b22):
    return (b11 + b22, b11, b12 - b22, b21 - b11, b22, b11 + b12, b21 + b22)


def _two_level(f, blk, swapped=()):
    o = {(r, c): f(blk[r][c], blk[r][2 + c], blk[2 + r][c], blk[2 + r][2 + c]) for r in range(2) for c in range(2)}
    out = []
    for p in range(7):
        s = int(p in swapped)
        out += f(o[0, s][p], o[0, 1 - s][p], o[1, s][p], o[1, 1 - s][p])
    return out


def _combine(m):
    add = lambda a, b: [x + y for x, y in zip(a, b)]
    sub = lambda a, b: [x - y for x, y in zip(a, b)]
    m1 = m(0)
    m4 = m(3)
    c11 = add(m1, m4)
    m2 = m(1)
    c21 = add(m2, m4)
    c22 = sub(m1, m2)
    c11 = add(c11, m(6))
    m5 = m(4)
    c11 = sub(c11, m5)
    m3 = m(2)
    c12 = add(m3, m5)
    c22 = add(c22, m3)
    c22 = add(c22, m(5))
    return c11, c12, c21, c22


def _strassen1(prod, fill):
    def m(p):
        r = prod(p)
        fill(r)
        return [r]
    c = _combine(m)
    return [c[0] + c[1], c[2] + c[3]]


def _strassen2(prod, fill):
    def m(p):
        (a, b), (c, d) = _strassen1(lambda q: prod(7 * p + q), fill)
        return [b, a, d, c] if p in SWAPPED else [a, b, c, d]
    c = _combine(m)
    return [[c[2 * (r // 2) + k // 2][2 * (r % 2) + k % 2] for k in range(4)] for r in range(4)]


def _paced(work, steps, first, last):
    calls = [0]

    def fill(r):
        calls[0] += 1
        if calls[0] == first:
            next(work, None)
        if first <= calls[0] <= last:
            k, n = calls[0] - first, last - first + 1
            rows, tiles = r.shape[0] // RS, r.shape[1] // LANES
            for g in range(-(-k * steps // n), -(-(k + 1) * steps // n)):
                t, a = divmod((g * n - k * steps) * rows * tiles // steps, rows)
                try:
                    work.send(r[a * RS:(a + 1) * RS, t * LANES:(t + 1) * LANES])
                    assert g + 1 < steps
                except StopIteration:
                    assert g + 1 == steps, (g, steps)
    return fill


def _run(work):
    for _ in work:
        pass


def _kernel(x_h, wqkv_h, wo_h, wg_h, wu_h, wd_h, o_h, x_s, wo, sgu, sd, qkv_s, cen, **cfg):
    S, D = x_h.shape
    QF = wd_h.shape[1]
    TM, TN, TD, G, NS = cfg["TM"], cfg["TN"], cfg["TD"], cfg["G"], cfg["NS"]
    NT, NB, NJ = D // LANES, S // TM, QF // LANES
    HM, HD, QM, QD = TM // 2, D // 2, TM // 4, D // 4
    NP = 7 * HD // TN
    mo = pl.multiple_of
    zero = [None]

    def pin(ref, lead, val):
        rows = pl.ds(mo(ref.shape[-2] - RS + zero[0], RS), RS)
        ref[(*lead, rows, slice(0, LANES))] = pltpu.bitcast(val[-RS:, -LANES:], ref.dtype)

    def behind(dep, v):
        lane = lax.broadcasted_iota(jnp.int32, v.shape, 1)
        return jnp.where(lane < zero[0], pltpu.bitcast(dep[-RS:, -LANES:], v.dtype), v)

    def rows2(r, n=RA):
        return pl.ds(r // 2 if isinstance(r, int) else mo(r // 2, RS), n // 2)

    def ld16(dep, v):
        if dep is None:
            return v.astype(F32)
        if v.dtype == BF:
            return pltpu.bitcast(behind(dep, pltpu.bitcast(v, U32)), BF).astype(F32)
        return jnp.concatenate([behind(dep, v[:RS]), behind(dep, v[RS:])], axis=0)

    def ln_stats(src, rows, cen):
        add = lambda a, b: a + b
        at = lambda k, t: (slice(k * RA, (k + 1) * RA), slice(t * LANES, (t + 1) * LANES))
        ld = lambda k, t: src[pl.ds(mo(rows[k], RA), RA), t * LANES:(t + 1) * LANES]
        ms, rs = [], []
        for k in range(len(rows)):
            d = yield
            xs = [ld16(d if src.dtype == BF or t == 0 else None, ld(k, t)) for t in range(NT)]
            if src.dtype == BF:
                for t in range(NT):
                    cen[at(k, t)] = xs[t]
            m = jnp.sum(functools.reduce(add, xs), axis=-1, keepdims=True)
            ms.append(jnp.broadcast_to(m * (1.0 / D), (RA, LANES)))
        for k in range(len(rows)):
            v = []
            for t in range(NT):
                if t % (NT // 2) == 0:
                    m = ld16((yield), ms[k])
                c = (cen[at(k, t)] if src.dtype == BF else ld(k, t)) - m
                cen[at(k, t)] = c
                v.append(c * c)
            v = jnp.sum(functools.reduce(add, v), axis=-1, keepdims=True)
            rs.append(jnp.broadcast_to(lax.rsqrt(v * (1.0 / D) + EPS), (RA, LANES)))
        yield
        ready = functools.reduce(add, rs)

        def tile(k, t, d):
            if d is not None and k == 0 and t == 0:
                d = d + (ready[:RS] + ready[RS:])
            return cen[at(k, t)] * ld16(d, rs[k])
        return tile

    def two_level(f, load, put, swapped=()):
        quad = lambda a, b, d: [load(2 * a + r, 2 * b + c, d) for r in range(2) for c in range(2)]

        def inner(p, q):
            for n, v in enumerate(f(q[1], q[0], q[3], q[2]) if p in swapped else f(*q)):
                put(7 * p + n, v)
            return v

        def later(q):
            if cfg["FINE"]:
                d = yield
                return [ld16(d, v) for v in q]
            return q
        q11 = quad(0, 0, (yield))
        inner(2 if f is _lhs7 else 1, q11)
        q22 = quad(1, 1, (yield))
        inner(3 if f is _lhs7 else 4, q22)
        q22 = yield from later(q22)
        inner(0, [a + b for a, b in zip(q11, q22)])
        q12 = quad(0, 1, (yield))
        inner(4 if f is _lhs7 else 5, [a + b for a, b in zip(q11, q12)])
        q12 = yield from later(q12)
        inner(6 if f is _lhs7 else 2, [a - b for a, b in zip(q12, q22)])
        q21 = quad(1, 0, (yield))
        inner(5 if f is _lhs7 else 3, [a - b for a, b in zip(q21, q11)])
        q21 = yield from later(q21)
        return inner(1 if f is _lhs7 else 6, [a + b for a, b in zip(q21, q22)])
    N2 = 7 if cfg["FINE"] else 4

    def phase_a(xc, wq, wkv, stg, tmp, fg, fu, fd, xsem, wsem, fsem):
        CH = HD // 4
        CU, CD, CO = QD // NB, QF // NB, HD // NB

        def x_cp(i):
            rows = pl.ds(mo(i * TM, TM), TM)
            return pltpu.make_async_copy(x_h.at[rows], x_s.at[rows], xsem.at[i])

        def w_cp(c):
            return pltpu.make_async_copy(wqkv_h.at[:, pl.ds(mo(c % 4 * CH, CH), CH), pl.ds(mo(c // 4 * D, D), D)],
                                         stg.at[:, pl.ds(mo(c % 4 * CH, CH), CH)], wsem.at[c % 4])

        def wo_cp(c):
            rows = pl.ds(mo(c * CH, CH), CH)
            return pltpu.make_async_copy(wo_h.at[:, rows], stg.at[:, rows], wsem.at[c])

        def f_cp(i):
            s = i % NS
            return [pltpu.make_async_copy(src.at[:, pl.ds(mo(i * n, RA), n)], dst.at[s], fsem.at[s])
                    for src, dst, n in ((wg_h, fg, CU), (wu_h, fu, CU), (wd_h, fd, CD))]

        def ln_work(src, dst, rs):
            tile = yield from ln_stats(x_s, [src + (k * HM + r) for r in rs for k in range(2)], cen)
            for g, r in enumerate(rs):
                for t in range(NT // 2):
                    d = yield
                    q = [tile(2 * g + k, n * NT // 2 + t, d) for k in range(2) for n in range(2)]
                    for p, v in enumerate(_lhs7(*q)):
                        xc[p, t, pl.ds(mo(dst(r // 2), RS), RS), :] = _pack(v)

        def att_work(c, wa, p):
            for r in range(0, CH, RA):
                for k in range(2):
                    d = yield
                    ts = [pltpu.bitcast(stg[k, pl.ds(mo(c % 4 * CH + r, RA), RA), t * LANES:(t + 1) * LANES], U32)
                          for t in range(NT)]
                    tmp[k, rows2(r), :] = jnp.concatenate(
                        _skew(ts if d is None else [behind(d, v) for v in ts]), axis=1)
            for r in range(0, CH, RA):
                for k in range(2):
                    d = yield
                    ts = [tmp[k, rows2(r), t * LANES:(t + 1) * LANES] for t in range(NT)]
                    tmp[k, rows2(r), :] = jnp.concatenate(
                        _unskew(ts if d is None else [behind(d, v) for v in ts]), axis=1)
            for r in range(0, CH, RA):
                for t in range(0, HD, LANES):
                    d = yield
                    q = [ld16(d, pltpu.bitcast(tmp[k, rows2(r), pl.ds(n * HD + t, LANES)], BF))
                         for k in range(2) for n in range(2)]
                    for n, v in enumerate(_rhs7(*q)):
                        wa[p, n, pl.ds(mo(c % 4 * (CH // 2) + r // 2, RS), RS), t:t + LANES] = _pack(v)

        def ffn_work(i):
            s = i % NS
            for e, src in enumerate((fg, fu)):
                for r in range(0, CU, RA):
                    for j in range(NJ):
                        def put(n, v):
                            sgu[j, n, rows2(i * CU + r), e * LANES:(e + 1) * LANES] = _pack(v)
                        yield from two_level(
                            _rhs7, lambda k, n, d: ld16(d, src[s, k, r:r + RA, pl.ds(n * QF + j * LANES, LANES)]),
                            put, SWAPPED)
            for r in range(0, CD, RA):
                for c in range(0, QD, LANES):
                    def put(n, v):
                        sd[n, rows2(i * CD + r), c:c + LANES] = _pack(v)
                    yield from two_level(
                        _rhs7, lambda k, n, d: ld16(d, fd[s, k, r:r + RA, pl.ds(n * QD + c, LANES)]), put, SWAPPED)
            for r in range(0, CO, RA):
                for c in range(0, HD, LANES):
                    d = yield
                    q = [ld16(d, stg[k, pl.ds(mo(i * CO + r, RA), RA), pl.ds(n * HD + c, LANES)])
                         for k in range(2) for n in range(2)]
                    for n, v in enumerate(_rhs7(*q)):
                        wo[n, rows2(i * CO + r), c:c + LANES] = _pack(v)
        ffn_steps = N2 * (2 * CU * NJ + CD * QD // LANES) // RA + CO * HD // (RA * LANES)

        def project(p, i, fill):
            for c0 in range(0, HD, TN):
                cs = _strassen1(lambda n: _mm(jnp.concatenate(
                    [xc[n, t, pl.ds(mo(i * QM, QM), QM)] for t in range(NT // 2)], axis=1), (wkv if p else wq)[p // 2, n, :, c0:c0 + TN]), fill)
                for a in range(2):
                    for b in range(2):
                        for t in range(TN // LANES):
                            qkv_s[p * NT + (b * HD + c0) // LANES + t, pl.ds(mo(i * TM + (HALO + a * HM), RS), HM)] = (
                                cs[a][b][:, t * LANES:(t + 1) * LANES])

        x_cp(0).start()
        w_cp(0).start()
        w_cp(1).start()
        x_cp(0).wait()
        w_cp(2).start()
        lax.fori_loop(0, 2, lambda r, _: _run(ln_work(r * QM, lambda e: r * (QM // 2) + e, range(0, QM, RA))), None)

        def first_weights(c, _):
            w_cp(c).wait()

            @pl.when(c < 3)
            def _():
                w_cp(c + 3).start()

            @pl.when(c >= 2)
            def _():
                x_cp(c - 1).start()
            _run(att_work(c, wq, 0))
        lax.fori_loop(0, 4, first_weights, None)

        def q_step(i, _):
            zero[0] = jnp.minimum(i, 0)

            @pl.when(i + 6 < 12)
            def _():
                w_cp(i + 6).start()

            @pl.when(i + 6 >= 12)
            def _():
                wo_cp(i - 6).start()

            @pl.when(i + 3 < NB)
            def _():
                x_cp(i + 3).start()

            @pl.when(i >= NB - NS + 1)
            def _():
                for c in f_cp(i - (NB - NS + 1)):
                    c.start()

            @pl.when(i + 1 < NB)
            def _():
                x_cp(i + 1).wait()
            w_cp(i + 4).wait()
            nxt = jnp.minimum(i + 1, NB - 1)
            fl = _paced(ln_work(nxt * TM, lambda e: i * QM + (QM + e), range(0, HM, RA)), 10 * HM // RA + 1, *cfg["LR"])
            fw = _paced(att_work(i + 4, wkv, i // 4), 8 * CH // RA, *cfg["LQ"])
            project(0, i, lambda r: (fl(r), fw(r)))
        lax.fori_loop(0, NB, q_step, None)

        def kv_step(i, _):
            zero[0] = jnp.minimum(i, 0)

            @pl.when(i + NS - 1 < NB)
            def _():
                for c in f_cp(i + NS - 1):
                    c.start()

            @pl.when(i % 2 == 0)
            def _():
                @pl.when(i < 4)
                def _():
                    wo_cp(i // 2 + 2).start()
                wo_cp(i // 2).wait()
            for c in f_cp(i):
                c.wait()
            fw = _paced(ffn_work(i), ffn_steps, 1, 2 * NP - cfg['KE'])
            project(1, i, fw)
            project(2, i, fw)
        lax.fori_loop(0, NB, kv_step, None)

    def phase_b(h_s, hc, ac, oc, o_s, osem):
        scale = (D // H) ** -0.5

        def attn_work(base, rs, masked):
            lane = lax.broadcasted_iota(jnp.int32, (RS, LANES), 1)

            def ld(r0, t, w):
                return qkv_s[t, pl.ds(base + (HALO + r0 - DIL * w), RS), :]

            def scores(r0, done):
                ls = [None] * W
                for t in range(NT):
                    d = yield
                    if d is not None and done and t >= NT // 2 and cfg["PA"]:
                        d = behind(done.pop(0), d)
                    q = ld(r0, t, 0) if d is None else behind(d, ld(r0, t, 0))
                    for w in range(W):
                        c = q * ld(r0, NT + t, w)
                        ls[w] = c if t == 0 else ls[w] + c
                for b in (1, 2):
                    m = (lane & b) != 0
                    ls = [jnp.where(m, y, x) + _lane_xor(jnp.where(m, x, y), b) for x, y in zip(ls[0::2], ls[1::2])]
                for b in (2, 1):
                    m = (lane & b) != 0
                    ls = [v for a, c in [(a, _lane_xor(a, b)) for a in ls]
                          for v in (jnp.where(m, c, a), jnp.where(m, a, c))]
                if masked and r0 < HALO:
                    pos = base + r0 + lax.broadcasted_iota(jnp.int32, (RS, LANES), 0)
                    ls = [jnp.where(pos >= DIL * w, a, -1e9 / scale) if w else a for w, a in enumerate(ls)]
                m = functools.reduce(jnp.maximum, ls)
                ps = [jnp.exp2((a - m) * (scale * math.log2(math.e))) for a in ls]
                inv = 1.0 / functools.reduce(lambda a, b: a + b, ps)
                return [p * inv for p in ps]

            def values(r0, ps):
                os_ = [None] * NT
                for w, p in enumerate(ps):
                    d = yield
                    p = p if d is None else behind(d, p)
                    for t in range(NT):
                        c = p * ld(r0, 2 * NT + t, w)
                        os_[t] = c if w == 0 else os_[t] + c
                return os_

            starts = [r + k * HM + e for r in rs for k in range(2) for e in range(0, RA, RS)]
            ahead = cfg["AF"] if masked else cfg["AH"]
            ps, outs, halves, done = [], [], [], []
            for n in range(len(starts) + ahead):
                if n < len(starts):
                    ps.append((yield from scores(starts[n], done)))
                if n >= ahead:
                    outs.append((yield from values(starts[n - ahead], ps.pop(0))))
                if len(outs) == 2:
                    halves.append(_unskew(_skew([_pack(jnp.concatenate(o, axis=0)) for o in zip(*outs)])))
                    outs = []
                if len(halves) == 2:
                    for t in range(NT // 2):
                        d = yield
                        q = [ld16(d, pltpu.bitcast(halves[k][e * NT // 2 + t], BF)) for k in range(2) for e in range(2)]
                        dst = starts[n - ahead] - HM - RS
                        for p, v in enumerate(_lhs7(*q)):
                            oc[p, rows2(base + dst if masked else dst), t * LANES:(t + 1) * LANES] = _pack(v)
                        done.append(v)
                    halves = []

        def out_proj(i, slot):
            for c0 in range(0, HD, TN):
                cs = _strassen1(lambda n: _mm(oc[n], wo[n, :, c0:c0 + TN]), lambda r: None)
                for a in range(2):
                    for b in range(2):
                        cols = pl.ds(b * HD + c0, TN)
                        h_s[pl.ds(mo(slot * TM + a * HM, HM), HM), cols] = (
                            x_s[pl.ds(mo(i * TM + a * HM, HM), HM), cols].astype(F32) + cs[a][b])

        def ln_work(slot, rs):
            tile = yield from ln_stats(h_s, [slot * TM + (k * QM + r) for r in rs for k in range(4)], cen)
            for g, r in enumerate(rs):
                for c in range(QD // LANES):
                    def put(p, v):
                        hc[p, rows2(r), c * LANES:(c + 1) * LANES] = _pack(v)
                    yield from two_level(_lhs7, lambda k, n, d: tile(4 * g + k, n * QD // LANES + c, d), put)

        for t in range(NT, 3 * NT):
            qkv_s[t, 0:HALO, :] = jnp.broadcast_to(qkv_s[t, HALO:HALO + 1, :], (HALO, LANES))
        EU = cfg["EU"]

        lax.fori_loop(0, HM // (RA * EU), lambda r, _: _run(attn_work(mo(r * RA * EU, RA), range(0, RA * EU, RA), True)), None)
        out_proj(0, 0)
        lax.fori_loop(0, 2, lambda r, _: _run(ln_work(0, [mo(r * QM // 2 + e, RA) for e in range(0, QM // 2, RA)])), None)

        def out_cp(i, slot):
            return pltpu.make_async_copy(o_s.at[slot], o_h.at[pl.ds(mo(i * TM, TM), TM)], osem.at[slot])

        def step(i, _):
            slot = i % 2
            zero[0] = jnp.minimum(i, 0)

            @pl.when(i >= 2)
            def _():
                out_cp(i - 2, slot).wait()
            nxt = jnp.minimum(i + 1, NB - 1)
            fa = _paced(attn_work(nxt * TM, range(0, HM, RA), False),
                        (4 * (NT + W) + NT // 2) * HM // RA, cfg["A0"], cfg["A1"])
            for j in range(NJ):
                c = _strassen2(lambda n: _mm(hc[n], sgu[j, n]), fa)
                act = [[_gelu(v[:, :LANES]) * v[:, LANES:] for v in row] for row in c]
                for p, v in enumerate(_two_level(_lhs7, act)):
                    ac[p, :, j * LANES:(j + 1) * LANES] = _pack(v)
            WP, LL = cfg["WP"], cfg["LL"]
            calls = [0]

            def fo(r):
                calls[0] += 1
                if calls[0] == WP:
                    out_proj(nxt, 1 - slot)
            fl = _paced(ln_work(1 - slot, range(0, QM, RA)), (12 + N2 * QD // LANES) * QM // RA + 1, WP + 1, 49 * QD // TD - LL)
            for c0 in range(0, QD, TD):
                cs = _strassen2(lambda n: _mm(ac[n], sd[n, :QF // 2, c0:c0 + TD]),
                                lambda r: (fa(r), fo(r), fl(r)))
                for a in range(4):
                    for b in range(4):
                        cols = pl.ds(b * QD + c0, TD)
                        o_s[slot, a * QM:(a + 1) * QM, cols] = (
                            h_s[pl.ds(mo(slot * TM + a * QM, QM), QM), cols] + cs[a][b]).astype(o_s.dtype)
            out_cp(i, slot).start()
        lax.fori_loop(0, NB, step, None)
        out_cp(NB - 2, 0).wait()
        out_cp(NB - 1, 1).wait()

    V, DMA = pltpu.VMEM, pltpu.SemaphoreType.DMA
    pl.run_scoped(phase_a, V((7, NT // 2, (NB + 1) * QM, LANES), U32), V((1, 7, HD // 2, HD), U32), V((2, 7, HD // 2, HD), U32), V((2, HD, D), BF), V((2, HD // 8, D), U32),
                  V((NS, 4, QD // NB, 4 * QF), BF), V((NS, 4, QD // NB, 4 * QF), BF),
                  V((NS, 4, QF // NB, D), BF), DMA((NB,)), DMA((4,)), DMA((NS,)))
    pl.run_scoped(phase_b, V((2 * TM, D), F32), V((49, QM // 2, QD), U32), V((49, QM // 2, QF), U32),
                  V((7, HM // 2, HD), U32), V((2, TM, D), o_h.dtype), DMA((2,)))


def make(**kw):
    cfg = dict(TM=256, TN=256, TD=256, G=4, NS=2, LQ=(9, 13), EU=2, A0=1, A1=343, WP=6, LL=4, KE=1, FINE=1, PQ=1, PA=0, AF=3, PL=0, AH=1, LR=(1, 8))
    cfg.update(kw)

    @jax.jit
    def fn(A_x, A_wqkv, A_wo, B_x, B_w_gate, B_w_up, B_w_down):
        del B_x
        B, S, D = A_x.shape
        F = B_w_gate.shape[1]
        anyspec = pl.BlockSpec(memory_space=pl.ANY)
        V = pltpu.VMEM
        out = pl.pallas_call(
            functools.partial(_kernel, **cfg),
            in_specs=[anyspec] * 6,
            out_specs=anyspec,
            out_shape=jax.ShapeDtypeStruct((S, D), A_x.dtype),
            scratch_shapes=[
                V((S, D), BF), V((7, D // 4, D // 2), U32), V((F // 4 // LANES, 49, D // 8, 2 * LANES), U32),
                V((49, F // 8 + RS, D // 4), U32), V((3 * D // LANES, S + HALO, LANES), F32), V((cfg['TM'], D), F32),
            ],
            compiler_params=pltpu.CompilerParams(vmem_limit_bytes=127 * 1024 * 1024),
        )(A_x.reshape(S, D), A_wqkv.reshape(2, D // 2, 3 * D), A_wo.reshape(2, D // 2, D),
          B_w_gate.reshape(4, D // 4, F), B_w_up.reshape(4, D // 4, F), B_w_down.reshape(4, F // 4, D))
        return out.reshape(B, S, D)
    return fn


pallas_sequential_preLN__sliding_local_dilated__glu_gated_geglu__prompt_kernel = make()
```

```python
import functools
import math
import jax
import jax.numpy as jnp
from jax import lax
import jax.experimental.pallas as pl
import jax.experimental.pallas.tpu as pltpu

H = 32
W = 8
DIL = 2
HALO = 16
EPS = 1e-5
LANES = 128
RA = 16
RS = 8
BF = jnp.bfloat16
F32 = jnp.float32
U32 = jnp.uint32
SWAPPED = (0, 1, 4)


def _pack(v):
    return pltpu.bitcast(v.astype(BF), U32)


def _mm(a, b):
    return jnp.dot(pltpu.bitcast(a, BF), pltpu.bitcast(b, BF), preferred_element_type=F32)


def _lane_xor(v, b):
    lane = lax.broadcasted_iota(jnp.int32, v.shape, 1)
    return jnp.take_along_axis(v, lane ^ b, axis=1) if b else v


def _skew(tiles):
    return [x if a == 0 else pltpu.roll(x, 4 * a, 1) for a, x in enumerate(tiles)]


def _unskew(t):
    lane = lax.broadcasted_iota(jnp.int32, t[0].shape, 1)
    t = [t[(-c) % 8] for c in range(8)]
    for b in (1, 2, 4):
        m = (lane & (4 * b)) != 0
        t = [jnp.where(m, t[(c - b) % 8], t[c]) for c in range(8)]
    return [x if c == 0 else pltpu.roll(x, LANES - 4 * c, 1) for c, x in enumerate(t)]


def _gelu(x):
    c = math.sqrt(2.0 / math.pi)
    inner = x * (c + (c * 0.044715) * (x * x))
    hx = 0.5 * x
    return hx + hx * jnp.tanh(inner)


def _lhs7(a11, a12, a21, a22):
    return (a11 + a22, a21 + a22, a11, a22, a11 + a12, a21 - a11, a12 - a22)


def _rhs7(b11, b12, b21, b22):
    return (b11 + b22, b11, b12 - b22, b21 - b11, b22, b11 + b12, b21 + b22)


def _two_level(f, blk, swapped=()):
    o = {(r, c): f(blk[r][c], blk[r][2 + c], blk[2 + r][c], blk[2 + r][2 + c]) for r in range(2) for c in range(2)}
    out = []
    for p in range(7):
        s = int(p in swapped)
        out += f(o[0, s][p], o[0, 1 - s][p], o[1, s][p], o[1, 1 - s][p])
    return out


_USES = (((0, 1), (3, 1)), ((2, 1), (3, -1)), ((1, 1), (3, 1)), ((0, 1), (2, 1)), ((0, -1), (1, 1)), ((3, 1),), ((0, 1),))


def _accumulate(acc, key, sign, v):
    acc[key] = (v if sign > 0 else -v) if key not in acc else acc[key] + v if sign > 0 else acc[key] - v
    return acc[key]


def _strassen1(prod, fill, emit, order=(6, 3, 1, 5, 0, 4, 2)):
    acc = {}
    last = {c: p for p in order for c, _ in _USES[p]}
    for p in order:
        m = prod(p)
        for c, sign in _USES[p]:
            v = _accumulate(acc, c, sign, m)
            if last[c] == p:
                emit(c // 2, c % 2, v)
        fill(m)


def _combine(m):
    add = lambda a, b: [x + y for x, y in zip(a, b)]
    sub = lambda a, b: [x - y for x, y in zip(a, b)]
    m1 = m(0)
    m4 = m(3)
    c11 = add(m1, m4)
    m2 = m(1)
    c21 = add(m2, m4)
    c22 = sub(m1, m2)
    c11 = add(c11, m(6))
    m5 = m(4)
    c11 = sub(c11, m5)
    m3 = m(2)
    c12 = add(m3, m5)
    c22 = add(c22, m3)
    c22 = add(c22, m(5))
    return c11, c12, c21, c22


def _strassen2(prod, fill):
    def inner(n):
        r = prod(n)
        fill(r)
        return [r]

    def outer(p):
        a, b, c, d = _combine(lambda q: inner(7 * p + q))
        return b + a + d + c if p in SWAPPED else a + b + c + d
    c = _combine(outer)
    return [[c[2 * (r // 2) + k // 2][2 * (r % 2) + k % 2] for k in range(4)] for r in range(4)]


def _paced(work, steps, first, last):
    calls = [0]

    def fill(r):
        calls[0] += 1
        if calls[0] == first:
            next(work, None)
        if first <= calls[0] <= last:
            k, n = calls[0] - first, last - first + 1
            rows, tiles = r.shape[0] // RS, r.shape[1] // LANES
            for g in range(-(-k * steps // n), -(-(k + 1) * steps // n)):
                t, a = divmod((g * n - k * steps) * rows * tiles // steps, rows)
                try:
                    work.send(r[a * RS:(a + 1) * RS, t * LANES:(t + 1) * LANES])
                    assert g + 1 < steps
                except StopIteration:
                    assert g + 1 == steps, (g, steps)
    return fill


def _run(work):
    for _ in work:
        pass


def _kernel(x_h, wqkv_h, wo_h, wg_h, wu_h, wd_h, o_h, x_s, wo, sgu, sd, qkv_s, cen, **cfg):
    S, D = x_h.shape
    QF = wd_h.shape[1]
    TM, TN, TD, NS = cfg["TM"], cfg["TN"], cfg["TD"], cfg["NS"]
    NT, NB, NJ = D // LANES, S // TM, QF // LANES
    HM, HD, QM, QD = TM // 2, D // 2, TM // 4, D // 4
    NP = 7 * HD // TN
    mo = pl.multiple_of
    zero = [None]

    def behind(dep, v):
        lane = lax.broadcasted_iota(jnp.int32, v.shape, 1)
        return jnp.where(lane < zero[0], pltpu.bitcast(dep[-RS:, -LANES:], v.dtype), v)

    def rows2(r, n=RA):
        return pl.ds(r // 2 if isinstance(r, int) else mo(r // 2, RS), n // 2)

    def ld16(dep, v):
        if dep is None:
            return v.astype(F32)
        if v.dtype == BF:
            return pltpu.bitcast(behind(dep, pltpu.bitcast(v, U32)), BF).astype(F32)
        return jnp.concatenate([behind(dep, v[:RS]), behind(dep, v[RS:])], axis=0)

    def ln_stats(src, rows, cen):
        add = lambda a, b: a + b
        at = lambda k, t: (slice(k * RA, (k + 1) * RA), slice(t * LANES, (t + 1) * LANES))
        ld = lambda k, t: src[pl.ds(mo(rows[k], RA), RA), t * LANES:(t + 1) * LANES]
        ms, rs = [], []
        for k in range(len(rows)):
            d = yield
            xs = [ld16(d if src.dtype == BF or t == 0 else None, ld(k, t)) for t in range(NT)]
            if src.dtype == BF:
                for t in range(NT):
                    cen[at(k, t)] = xs[t]
            m = jnp.sum(functools.reduce(add, xs), axis=-1, keepdims=True)
            ms.append(jnp.broadcast_to(m * (1.0 / D), (RA, LANES)))
        for k in range(len(rows)):
            v = []
            for t in range(NT):
                if t % (NT // 2) == 0:
                    m = ld16((yield), ms[k])
                c = (cen[at(k, t)] if src.dtype == BF else ld(k, t)) - m
                cen[at(k, t)] = c
                v.append(c * c)
            v = jnp.sum(functools.reduce(add, v), axis=-1, keepdims=True)
            rs.append(jnp.broadcast_to(lax.rsqrt(v * (1.0 / D) + EPS), (RA, LANES)))
        yield
        ready = functools.reduce(add, rs)

        def tile(k, t, d):
            if d is not None and k == 0 and t == 0:
                d = d + (ready[:RS] + ready[RS:])
            return cen[at(k, t)] * ld16(d, rs[k])
        return tile

    def two_level(f, load, put, swapped=()):
        quad = lambda a, b, d: [load(2 * a + r, 2 * b + c, d) for r in range(2) for c in range(2)]

        def inner(p, q):
            for n, v in enumerate(f(q[1], q[0], q[3], q[2]) if p in swapped else f(*q)):
                put(7 * p + n, v)
            return v

        def later(q):
            if cfg["FINE"]:
                d = yield
                return [ld16(d, v) for v in q]
            return q
        q11 = quad(0, 0, (yield))
        inner(2 if f is _lhs7 else 1, q11)
        q22 = quad(1, 1, (yield))
        inner(3 if f is _lhs7 else 4, q22)
        q22 = yield from later(q22)
        inner(0, [a + b for a, b in zip(q11, q22)])
        q12 = quad(0, 1, (yield))
        inner(4 if f is _lhs7 else 5, [a + b for a, b in zip(q11, q12)])
        q12 = yield from later(q12)
        inner(6 if f is _lhs7 else 2, [a - b for a, b in zip(q12, q22)])
        q21 = quad(1, 0, (yield))
        inner(5 if f is _lhs7 else 3, [a - b for a, b in zip(q21, q11)])
        q21 = yield from later(q21)
        return inner(1 if f is _lhs7 else 6, [a + b for a, b in zip(q21, q22)])
    N2 = 7 if cfg["FINE"] else 4

    def phase_a(xc, wq, wkv, stg, tmp, fg, fu, fd, xsem, wsem, fsem):
        CH = HD // 4
        CU, CD, CO = QD // NB, QF // NB, HD // NB

        def x_cp(i):
            rows = pl.ds(mo(i * TM, TM), TM)
            return pltpu.make_async_copy(x_h.at[rows], x_s.at[rows], xsem.at[i])

        def w_cp(c):
            return pltpu.make_async_copy(wqkv_h.at[:, pl.ds(mo(c % 4 * CH, CH), CH), pl.ds(mo(c // 4 * D, D), D)],
                                         stg.at[:, pl.ds(mo(c % 4 * CH, CH), CH)], wsem.at[c % 4])

        def wo_cp(c):
            rows = pl.ds(mo(c * CH, CH), CH)
            return pltpu.make_async_copy(wo_h.at[:, rows], stg.at[:, rows], wsem.at[c])

        def f_cp(i):
            s = i % NS
            return [pltpu.make_async_copy(src.at[:, pl.ds(mo(i * n, RA), n)], dst.at[s], fsem.at[s])
                    for src, dst, n in ((wg_h, fg, CU), (wu_h, fu, CU), (wd_h, fd, CD))]

        def ln_work(src, dst, rs):
            tile = yield from ln_stats(x_s, [src + (k * HM + r) for r in rs for k in range(2)], cen)
            for g, r in enumerate(rs):
                for t in range(NT // 2):
                    d = yield
                    q = [tile(2 * g + k, n * NT // 2 + t, d) for k in range(2) for n in range(2)]
                    for p, v in enumerate(_lhs7(*q)):
                        xc[p, t, pl.ds(mo(dst(r // 2), RS), RS), :] = _pack(v)

        def att_work(c, wa, p):
            for r in range(0, CH, RA):
                for k in range(2):
                    d = yield
                    ts = [pltpu.bitcast(stg[k, pl.ds(mo(c % 4 * CH + r, RA), RA), t * LANES:(t + 1) * LANES], U32)
                          for t in range(NT)]
                    tmp[k, rows2(r), :] = jnp.concatenate(
                        _skew(ts if d is None else [behind(d, v) for v in ts]), axis=1)
            for r in range(0, CH, RA):
                for k in range(2):
                    d = yield
                    ts = [tmp[k, rows2(r), t * LANES:(t + 1) * LANES] for t in range(NT)]
                    tmp[k, rows2(r), :] = jnp.concatenate(
                        _unskew(ts if d is None else [behind(d, v) for v in ts]), axis=1)
            for r in range(0, CH, RA):
                for t in range(0, HD, LANES):
                    d = yield
                    q = [ld16(d, pltpu.bitcast(tmp[k, rows2(r), pl.ds(n * HD + t, LANES)], BF))
                         for k in range(2) for n in range(2)]
                    for n, v in enumerate(_rhs7(*q)):
                        wa[p, n, pl.ds(mo(c % 4 * (CH // 2) + r // 2, RS), RS), t:t + LANES] = _pack(v)

        def ffn_work(i):
            s = i % NS
            for e, src in enumerate((fg, fu)):
                for r in range(0, CU, RA):
                    for j in range(NJ):
                        def put(n, v):
                            sgu[j, n, rows2(i * CU + r), e * LANES:(e + 1) * LANES] = _pack(v)
                        yield from two_level(
                            _rhs7, lambda k, n, d: ld16(d, src[s, k, r:r + RA, pl.ds(n * QF + j * LANES, LANES)]),
                            put, SWAPPED)
            for r in range(0, CD, RA):
                for c in range(0, QD, LANES):
                    def put(n, v):
                        sd[n, rows2(i * CD + r), c:c + LANES] = _pack(v)
                    yield from two_level(
                        _rhs7, lambda k, n, d: ld16(d, fd[s, k, r:r + RA, pl.ds(n * QD + c, LANES)]), put, SWAPPED)
            for r in range(0, CO, RA):
                for c in range(0, HD, LANES):
                    d = yield
                    q = [ld16(d, stg[k, pl.ds(mo(i * CO + r, RA), RA), pl.ds(n * HD + c, LANES)])
                         for k in range(2) for n in range(2)]
                    for n, v in enumerate(_rhs7(*q)):
                        wo[n, rows2(i * CO + r), c:c + LANES] = _pack(v)
        ffn_steps = N2 * (2 * CU * NJ + CD * QD // LANES) // RA + CO * HD // (RA * LANES)

        def project(p, i, fill):
            for c0 in range(0, HD, TN):
                def emit(a, b, v):
                    for t in range(TN // LANES):
                        qkv_s[p * NT + (b * HD + c0) // LANES + t, pl.ds(mo(i * TM + (HALO + a * HM), RS), HM)] = (
                            v[:, t * LANES:(t + 1) * LANES])
                _strassen1(lambda n: _mm(
                    jnp.concatenate([xc[n, t, pl.ds(mo(i * QM, QM), QM)] for t in range(NT // 2)], axis=1),
                    (wkv if p else wq)[p // 2, n, :, c0:c0 + TN]), fill, emit)

        x_cp(0).start()
        w_cp(0).start()
        w_cp(1).start()
        x_cp(0).wait()
        w_cp(2).start()
        lax.fori_loop(0, 2, lambda r, _: _run(ln_work(r * QM, lambda e: r * (QM // 2) + e, range(0, QM, RA))), None)

        def first_weights(c, _):
            w_cp(c).wait()

            @pl.when(c < 3)
            def _():
                w_cp(c + 3).start()

            @pl.when(c >= 2)
            def _():
                x_cp(c - 1).start()
            _run(att_work(c, wq, 0))
        lax.fori_loop(0, 4, first_weights, None)

        def q_step(i, _):
            zero[0] = jnp.minimum(i, 0)

            @pl.when(i + 6 < 12)
            def _():
                w_cp(i + 6).start()

            @pl.when(i + 6 >= 12)
            def _():
                wo_cp(i - 6).start()

            @pl.when(i + 3 < NB)
            def _():
                x_cp(i + 3).start()

            @pl.when(i >= NB - NS + 1)
            def _():
                for c in f_cp(i - (NB - NS + 1)):
                    c.start()

            @pl.when(i + 1 < NB)
            def _():
                x_cp(i + 1).wait()
            w_cp(i + 4).wait()
            nxt = jnp.minimum(i + 1, NB - 1)
            fl = _paced(ln_work(nxt * TM, lambda e: i * QM + (QM + e), range(0, HM, RA)), 10 * HM // RA + 1, *cfg["LR"])
            fw = _paced(att_work(i + 4, wkv, i // 4), 8 * CH // RA, *cfg["LQ"])
            project(0, i, lambda r: (fl(r), fw(r)))
        lax.fori_loop(0, NB, q_step, None)

        def kv_step(i, _):
            zero[0] = jnp.minimum(i, 0)

            @pl.when(i + NS - 1 < NB)
            def _():
                for c in f_cp(i + NS - 1):
                    c.start()

            @pl.when(i % 2 == 0)
            def _():
                @pl.when(i < 4)
                def _():
                    wo_cp(i // 2 + 2).start()
                wo_cp(i // 2).wait()
            for c in f_cp(i):
                c.wait()
            fw = _paced(ffn_work(i), ffn_steps, 1, 2 * NP - cfg['KE'])
            project(1, i, fw)
            project(2, i, fw)
        lax.fori_loop(0, NB, kv_step, None)

    def phase_b(h_s, hc, ac, oc, o_s, osem):
        scale = (D // H) ** -0.5

        def attn_work(base, rs, first, sq, sv, ahead):
            lane = lax.broadcasted_iota(jnp.int32, (RS, LANES), 1)

            def taps(r0, t, n):
                for back in range(-(n - 1) * RS, DIL * W, DIL):
                    v = qkv_s[t, pl.ds(base + (HALO + r0 - back), RS), :]
                    yield v, [(g, (back + g * RS) // DIL) for g in range(n) if 0 <= back + g * RS < DIL * W]

            def softmax(r0, ls):
                for b in (1, 2):
                    m = (lane & b) != 0
                    ls = [jnp.where(m, y, x) + _lane_xor(jnp.where(m, x, y), b) for x, y in zip(ls[0::2], ls[1::2])]
                for b in (2, 1):
                    m = (lane & b) != 0
                    ls = [v for a, c in [(a, _lane_xor(a, b)) for a in ls]
                          for v in (jnp.where(m, c, a), jnp.where(m, a, c))]
                out = []
                for g in range(len(ls) // W):
                    lg = ls[g * W:(g + 1) * W]
                    if first and r0 + g * RS < HALO:
                        pos = base + (r0 + g * RS) + lax.broadcasted_iota(jnp.int32, (RS, LANES), 0)
                        lg = [jnp.where(pos >= DIL * w, a, -1e9 / scale) if w else a for w, a in enumerate(lg)]
                    m = functools.reduce(jnp.maximum, lg)
                    ps = [jnp.exp2((a - m) * (scale * math.log2(math.e))) for a in lg]
                    inv = 1.0 / functools.reduce(lambda a, b: a + b, ps)
                    out.append([p * inv for p in ps])
                return out

            def scores(r0):
                acc = {}
                for t in range(NT):
                    q = []
                    for g in range(sq):
                        d = yield
                        v = qkv_s[t, pl.ds(base + (HALO + r0 + g * RS), RS), :]
                        q.append(v if d is None else behind(d, v))
                    for v, uses in taps(r0, NT + t, sq):
                        for g, w in uses:
                            _accumulate(acc, (g, w), 1, q[g] * v)
                return softmax(r0, [acc[g, w] for g in range(sq) for w in range(W)])

            def values(r0, ps):
                acc = {}
                for row in zip(*[taps(r0, 2 * NT + t, sv) for t in range(NT)]):
                    for g, w in row[0][1]:
                        d = yield
                        p = ps[g][w] if d is None else behind(d, ps[g][w])
                        for t in range(NT):
                            _accumulate(acc, (g, t), 1, p * row[t][0])
                return [[acc[g, t] for t in range(NT)] for g in range(sv)]

            starts = [r + k * HM + e for r in rs for k in range(2) for e in range(0, RA, RS)]
            ps, outs, halves, nq, nv = [], [], [], 0, 0
            while nv < len(starts):
                if nq < len(starts) and nq < nv + sv + ahead:
                    ps += yield from scores(starts[nq])
                    nq += sq
                    continue
                outs += yield from values(starts[nv], ps[nv:nv + sv])
                nv += sv
                if len(outs) == 2:
                    halves.append(_unskew(_skew([_pack(jnp.concatenate(o, axis=0)) for o in zip(*outs)])))
                    outs = []
                if len(halves) == 2:
                    dst = starts[nv - 4]
                    for t in range(NT // 2):
                        d = yield
                        q = [ld16(d, pltpu.bitcast(halves[k][e * NT // 2 + t], BF)) for k in range(2) for e in range(2)]
                        for p, v in enumerate(_lhs7(*q)):
                            oc[p, rows2(base + dst if first else dst), t * LANES:(t + 1) * LANES] = _pack(v)
                    halves = []

        def out_proj(i, slot):
            for c0 in range(0, HD, TN):
                def emit(a, b, v):
                    cols = pl.ds(b * HD + c0, TN)
                    h_s[pl.ds(mo(slot * TM + a * HM, HM), HM), cols] = (
                        x_s[pl.ds(mo(i * TM + a * HM, HM), HM), cols].astype(F32) + v)
                _strassen1(lambda n: _mm(oc[n], wo[n, :, c0:c0 + TN]), lambda r: None, emit, cfg['WO'])

        def ln_work(slot, rs):
            tile = yield from ln_stats(h_s, [slot * TM + (k * QM + r) for r in rs for k in range(4)], cen)
            for g, r in enumerate(rs):
                for c in range(QD // LANES):
                    def put(p, v):
                        hc[p, rows2(r), c * LANES:(c + 1) * LANES] = _pack(v)
                    yield from two_level(_lhs7, lambda k, n, d: tile(4 * g + k, n * QD // LANES + c, d), put)

        for t in range(NT, 3 * NT):
            qkv_s[t, 0:HALO, :] = jnp.broadcast_to(qkv_s[t, HALO:HALO + 1, :], (HALO, LANES))
        EU = cfg["EU"]

        lax.fori_loop(0, HM // (RA * EU), lambda r, _: _run(attn_work(mo(r * RA * EU, RA), range(0, RA * EU, RA), True, *cfg['AF'])), None)
        out_proj(0, 0)
        lax.fori_loop(0, 2, lambda r, _: _run(ln_work(0, [mo(r * QM // 2 + e, RA) for e in range(0, QM // 2, RA)])), None)

        def out_cp(i, slot):
            return pltpu.make_async_copy(o_s.at[slot], o_h.at[pl.ds(mo(i * TM, TM), TM)], osem.at[slot])

        def step(i, _):
            slot = i % 2
            zero[0] = jnp.minimum(i, 0)

            @pl.when(i >= 2)
            def _():
                out_cp(i - 2, slot).wait()
            nxt = jnp.minimum(i + 1, NB - 1)
            fa = _paced(attn_work(nxt * TM, range(0, HM, RA), False, *cfg['AH']),
                        (4 * (NT + W) + NT // 2) * HM // RA, cfg["A0"], cfg["A1"])
            for j in range(NJ):
                if cfg["CAT"]:
                    c = _strassen2(lambda n: _mm(hc[n], sgu[j, n]), fa)
                    act = [[_gelu(v[:, :LANES]) * v[:, LANES:] for v in row] for row in c]
                else:
                    g = _strassen2(lambda n: _mm(hc[n], sgu[j, n, :, :LANES]), fa)
                    g = [[_gelu(v) for v in row] for row in g]
                    u = _strassen2(lambda n: _mm(hc[n], sgu[j, n, :, LANES:]), fa)
                    act = [[a * b for a, b in zip(*rows)] for rows in zip(g, u)]
                for p, v in enumerate(_two_level(_lhs7, act)):
                    ac[p, :, j * LANES:(j + 1) * LANES] = _pack(v)
            out_proj(nxt, 1 - slot)
            fl = _paced(ln_work(1 - slot, range(0, QM, RA)), (12 + N2 * QD // LANES) * QM // RA + 1,
                        cfg["L0"], 49 * QD // TD - cfg["LL"])
            for c0 in range(0, QD, TD):
                cs = _strassen2(lambda n: _mm(ac[n], sd[n, :, c0:c0 + TD]), fl)
                for a in range(4):
                    for b in range(4):
                        cols = pl.ds(b * QD + c0, TD)
                        o_s[slot, a * QM:(a + 1) * QM, cols] = (
                            h_s[pl.ds(mo(slot * TM + a * QM, QM), QM), cols] + cs[a][b]).astype(o_s.dtype)
            out_cp(i, slot).start()
        lax.fori_loop(0, NB, step, None)
        out_cp(NB - 2, 0).wait()
        out_cp(NB - 1, 1).wait()

    V, DMA = pltpu.VMEM, pltpu.SemaphoreType.DMA
    pl.run_scoped(phase_a, V((7, NT // 2, (NB + 1) * QM, LANES), U32), V((1, 7, HD // 2, HD), U32), V((2, 7, HD // 2, HD), U32), V((2, HD, D), BF), V((2, HD // 8, D), U32),
                  V((NS, 4, QD // NB, 4 * QF), BF), V((NS, 4, QD // NB, 4 * QF), BF),
                  V((NS, 4, QF // NB, D), BF), DMA((NB,)), DMA((4,)), DMA((NS,)))
    pl.run_scoped(phase_b, V((2 * TM, D), F32), V((49, QM // 2, QD), U32), V((49, QM // 2, QF), U32),
                  V((7, HM // 2, HD), U32), V((2, TM, D), o_h.dtype), DMA((2,)))


def make(**kw):
    cfg = dict(TM=256, TN=256, TD=256, NS=2, LQ=(9, 13), LR=(1, 8), EU=2, A0=1, A1=640, L0=1, LL=4, KE=1, FINE=1,
               AF=(2, 2, 2), AH=(2, 2, 2), WO=(0, 3, 1, 6, 4, 2, 5), CAT=0, NB=1)
    cfg.update(kw)

    @jax.jit
    def fn(A_x, A_wqkv, A_wo, B_x, B_w_gate, B_w_up, B_w_down):
        del B_x
        B, S, D = A_x.shape
        F = B_w_gate.shape[1]
        anyspec = pl.BlockSpec(memory_space=pl.ANY)
        V = pltpu.VMEM
        out = pl.pallas_call(
            functools.partial(_kernel, **cfg),
            in_specs=[anyspec] * 6,
            out_specs=anyspec,
            out_shape=jax.ShapeDtypeStruct((S, D), A_x.dtype),
            scratch_shapes=[
                V((S, D), BF), V((7, D // 4, D // 2), U32), V((F // 4 // LANES, 49, D // 8, 2 * LANES), U32),
                V((49, F // 8, D // 4), U32), V((3 * D // LANES, S + HALO, LANES), F32), V((cfg['TM'], D), F32),
            ],
            compiler_params=pltpu.CompilerParams(vmem_limit_bytes=127 * 1024 * 1024, disable_bounds_checks=bool(cfg.get("NB", 0))),
        )(A_x.reshape(S, D), A_wqkv.reshape(2, D // 2, 3 * D), A_wo.reshape(2, D // 2, D),
          B_w_gate.reshape(4, D // 4, F), B_w_up.reshape(4, D // 4, F), B_w_down.reshape(4, F // 4, D))
        return out.reshape(B, S, D)
    return fn


pallas_sequential_preLN__sliding_local_dilated__glu_gated_geglu__prompt_kernel = make()
```

```python
import functools
import math
import jax
import jax.numpy as jnp
from jax import lax
import jax.experimental.pallas as pl
import jax.experimental.pallas.tpu as pltpu

H = 32
W = 8
DIL = 2
HALO = 16
EPS = 1e-5
LANES = 128
RA = 16
RS = 8
BF = jnp.bfloat16
F32 = jnp.float32
U32 = jnp.uint32
SWAPPED = (0, 1, 4)


def _pack(v):
    return pltpu.bitcast(v.astype(BF), U32)


def _mm(a, b):
    return jnp.dot(pltpu.bitcast(a, BF), pltpu.bitcast(b, BF), preferred_element_type=F32)


def _operand(ref, n, tiles, rows=slice(None)):
    return jnp.concatenate([ref[t, rows, n].reshape(-1, LANES) for t in tiles], axis=1)


def _lane_xor(v, b):
    lane = lax.broadcasted_iota(jnp.int32, v.shape, 1)
    return jnp.take_along_axis(v, lane ^ b, axis=1) if b else v


def _skew(tiles):
    return [x if a == 0 else pltpu.roll(x, 4 * a, 1) for a, x in enumerate(tiles)]


def _unskew(t):
    lane = lax.broadcasted_iota(jnp.int32, t[0].shape, 1)
    t = [t[(-c) % 8] for c in range(8)]
    for b in (1, 2, 4):
        m = (lane & (4 * b)) != 0
        t = [jnp.where(m, t[(c - b) % 8], t[c]) for c in range(8)]
    return [x if c == 0 else pltpu.roll(x, LANES - 4 * c, 1) for c, x in enumerate(t)]


def _gelu(x):
    c = math.sqrt(2.0 / math.pi)
    inner = x * (c + (c * 0.044715) * (x * x))
    hx = 0.5 * x
    return hx + hx * jnp.tanh(inner)


def _lhs7(a11, a12, a21, a22):
    return (a11 + a22, a21 + a22, a11, a22, a11 + a12, a21 - a11, a12 - a22)


def _rhs7(b11, b12, b21, b22):
    return (b11 + b22, b11, b12 - b22, b21 - b11, b22, b11 + b12, b21 + b22)


def _two_level(f, blk, swapped=()):
    o = {(r, c): f(blk[r][c], blk[r][2 + c], blk[2 + r][c], blk[2 + r][2 + c]) for r in range(2) for c in range(2)}
    out = []
    for p in range(7):
        s = int(p in swapped)
        out += f(o[0, s][p], o[0, 1 - s][p], o[1, s][p], o[1, 1 - s][p])
    return out


_USES = (((0, 1), (3, 1)), ((2, 1), (3, -1)), ((1, 1), (3, 1)), ((0, 1), (2, 1)), ((0, -1), (1, 1)), ((3, 1),), ((0, 1),))


def _accumulate(acc, key, sign, v):
    acc[key] = (v if sign > 0 else -v) if key not in acc else acc[key] + v if sign > 0 else acc[key] - v
    return acc[key]


def _strassen1(prod, fill, emit, order=(6, 3, 1, 5, 0, 4, 2)):
    acc = {}
    last = {c: p for p in order for c, _ in _USES[p]}
    for p in order:
        m = prod(p)
        for c, sign in _USES[p]:
            v = _accumulate(acc, c, sign, m)
            if last[c] == p:
                emit(c // 2, c % 2, v)
        fill(m)


def _combine(m):
    add = lambda a, b: [x + y for x, y in zip(a, b)]
    sub = lambda a, b: [x - y for x, y in zip(a, b)]
    m1 = m(0)
    m4 = m(3)
    c11 = add(m1, m4)
    m2 = m(1)
    c21 = add(m2, m4)
    c22 = sub(m1, m2)
    c11 = add(c11, m(6))
    m5 = m(4)
    c11 = sub(c11, m5)
    m3 = m(2)
    c12 = add(m3, m5)
    c22 = add(c22, m3)
    c22 = add(c22, m(5))
    return c11, c12, c21, c22


def _strassen2(prod, fill):
    def inner(n):
        r = prod(n)
        fill(r)
        return [r]

    def outer(p):
        a, b, c, d = _combine(lambda q: inner(7 * p + q))
        return b + a + d + c if p in SWAPPED else a + b + c + d
    c = _combine(outer)
    return [[c[2 * (r // 2) + k // 2][2 * (r % 2) + k % 2] for k in range(4)] for r in range(4)]


def _paced(work, steps, first, last):
    calls = [0]

    def fill(r):
        calls[0] += 1
        if calls[0] == first:
            next(work, None)
        if first <= calls[0] <= last:
            k, n = calls[0] - first, last - first + 1
            rows, tiles = r.shape[0] // RS, r.shape[1] // LANES
            for g in range(-(-k * steps // n), -(-(k + 1) * steps // n)):
                t, a = divmod((g * n - k * steps) * rows * tiles // steps, rows)
                try:
                    work.send(r[a * RS:(a + 1) * RS, t * LANES:(t + 1) * LANES])
                    assert g + 1 < steps
                except StopIteration:
                    assert g + 1 == steps, (g, steps)
    return fill


def _run(work):
    for _ in work:
        pass


def _kernel(x_h, wqkv_h, wo_h, wg_h, wu_h, wd_h, o_h, x_s, wo, sgu, sd, qkv_s, cen, **cfg):
    S, D = x_h.shape
    QF = wd_h.shape[1]
    TM, TN, TD, NS = cfg["TM"], cfg["TN"], cfg["TD"], cfg["NS"]
    NT, NB, NJ = D // LANES, S // TM, QF // LANES
    HM, HD, QM, QD = TM // 2, D // 2, TM // 4, D // 4
    NP = 7 * HD // TN
    mo = pl.multiple_of
    zero = [None]

    def behind(dep, v):
        lane = lax.broadcasted_iota(jnp.int32, v.shape, 1)
        return jnp.where(lane < zero[0], pltpu.bitcast(dep[-RS:, -LANES:], v.dtype), v)

    def rows2(r, n=RA):
        return pl.ds(r // 2 if isinstance(r, int) else mo(r // 2, RS), n // 2)

    def ld16(dep, v):
        if dep is None:
            return v.astype(F32)
        if v.dtype == BF:
            return pltpu.bitcast(behind(dep, pltpu.bitcast(v, U32)), BF).astype(F32)
        return jnp.concatenate([behind(dep, v[:RS]), behind(dep, v[RS:])], axis=0)

    def ln_stats(src, rows, cen):
        add = lambda a, b: a + b
        at = lambda k, t: (slice(k * RA, (k + 1) * RA), slice(t * LANES, (t + 1) * LANES))
        ld = lambda k, t: src[pl.ds(mo(rows[k], RA), RA), t * LANES:(t + 1) * LANES]
        ms, rs = [], []
        for k in range(len(rows)):
            d = yield
            xs = [ld16(d if src.dtype == BF or t == 0 else None, ld(k, t)) for t in range(NT)]
            if src.dtype == BF:
                for t in range(NT):
                    cen[at(k, t)] = xs[t]
            m = jnp.sum(functools.reduce(add, xs), axis=-1, keepdims=True)
            ms.append(jnp.broadcast_to(m * (1.0 / D), (RA, LANES)))
        for k in range(len(rows)):
            v = []
            for t in range(NT):
                if t % (NT // 2) == 0:
                    m = ld16((yield), ms[k])
                c = (cen[at(k, t)] if src.dtype == BF else ld(k, t)) - m
                cen[at(k, t)] = c
                v.append(c * c)
            v = jnp.sum(functools.reduce(add, v), axis=-1, keepdims=True)
            rs.append(jnp.broadcast_to(lax.rsqrt(v * (1.0 / D) + EPS), (RA, LANES)))
        yield
        ready = functools.reduce(add, rs)

        def tile(k, t, d):
            if d is not None and k == 0 and t == 0:
                d = d + (ready[:RS] + ready[RS:])
            return cen[at(k, t)] * ld16(d, rs[k])
        return tile

    def two_level(f, load, put, swapped=()):
        quad = lambda a, b, d: [load(2 * a + r, 2 * b + c, d) for r in range(2) for c in range(2)]

        def inner(p, q):
            for n, v in enumerate(f(q[1], q[0], q[3], q[2]) if p in swapped else f(*q)):
                put(7 * p + n, v)
            return v

        def later(q):
            if cfg["FINE"]:
                d = yield
                return [ld16(d, v) for v in q]
            return q
        q11 = quad(0, 0, (yield))
        inner(2 if f is _lhs7 else 1, q11)
        q22 = quad(1, 1, (yield))
        inner(3 if f is _lhs7 else 4, q22)
        q22 = yield from later(q22)
        inner(0, [a + b for a, b in zip(q11, q22)])
        q12 = quad(0, 1, (yield))
        inner(4 if f is _lhs7 else 5, [a + b for a, b in zip(q11, q12)])
        q12 = yield from later(q12)
        inner(6 if f is _lhs7 else 2, [a - b for a, b in zip(q12, q22)])
        q21 = quad(1, 0, (yield))
        inner(5 if f is _lhs7 else 3, [a - b for a, b in zip(q21, q11)])
        q21 = yield from later(q21)
        return inner(1 if f is _lhs7 else 6, [a + b for a, b in zip(q21, q22)])
    N2 = 7 if cfg["FINE"] else 4

    def phase_a(xc, wq, wkv, stg, tmp, fg, fu, fd, xsem, wsem, fsem):
        CH = HD // 4
        CU, CD, CO = QD // NB, QF // NB, HD // NB

        def x_cp(i):
            rows = pl.ds(mo(i * TM, TM), TM)
            return pltpu.make_async_copy(x_h.at[rows], x_s.at[rows], xsem.at[i])

        def w_cp(c):
            return pltpu.make_async_copy(wqkv_h.at[:, pl.ds(mo(c % 4 * CH, CH), CH), pl.ds(mo(c // 4 * D, D), D)],
                                         stg.at[:, pl.ds(mo(c % 4 * CH, CH), CH)], wsem.at[c % 4])

        def wo_cp(c):
            rows = pl.ds(mo(c * CH, CH), CH)
            return pltpu.make_async_copy(wo_h.at[:, rows], stg.at[:, rows], wsem.at[c])

        def f_cp(i):
            s = i % NS
            return [pltpu.make_async_copy(src.at[:, pl.ds(mo(i * n, RA), n)], dst.at[s], fsem.at[s])
                    for src, dst, n in ((wg_h, fg, CU), (wu_h, fu, CU), (wd_h, fd, CD))]

        def ln_work(src, dst, rs):
            tile = yield from ln_stats(x_s, [src + (k * HM + r) for r in rs for k in range(2)], cen)
            for g, r in enumerate(rs):
                for t in range(NT // 2):
                    d = yield
                    q = [tile(2 * g + k, n * NT // 2 + t, d) for k in range(2) for n in range(2)]
                    for p, v in enumerate(_lhs7(*q)):
                        xc[t, dst(r // RA), p] = _pack(v)

        def att_work(c, wa, p, wait=None):
            if wait is not None:
                wait()
            for r in range(0, CH, RA):
                for k in range(2):
                    d = yield
                    ts = [pltpu.bitcast(stg[k, pl.ds(mo(c % 4 * CH + r, RA), RA), t * LANES:(t + 1) * LANES], U32)
                          for t in range(NT)]
                    tmp[k, rows2(r), :] = jnp.concatenate(
                        _skew(ts if d is None else [behind(d, v) for v in ts]), axis=1)
            for r in range(0, CH, RA):
                for k in range(2):
                    d = yield
                    ts = [tmp[k, rows2(r), t * LANES:(t + 1) * LANES] for t in range(NT)]
                    tmp[k, rows2(r), :] = jnp.concatenate(
                        _unskew(ts if d is None else [behind(d, v) for v in ts]), axis=1)
            for r in range(0, CH, RA):
                for t in range(0, HD, LANES):
                    d = yield
                    q = [ld16(d, pltpu.bitcast(tmp[k, rows2(r), pl.ds(n * HD + t, LANES)], BF))
                         for k in range(2) for n in range(2)]
                    for n, v in enumerate(_rhs7(*q)):
                        wa[p * (NT // 2) + t // LANES, c % 4 * (CH // RA) + r // RA, n] = _pack(v)

        def ffn_work(i):
            s = i % NS
            for e, src in enumerate((fg, fu)):
                for r in range(0, CU, RA):
                    for j in range(NJ):
                        def put(n, v):
                            sgu[2 * j + e, i * (CU // RA) + r // RA, n] = _pack(v)
                        yield from two_level(
                            _rhs7, lambda k, n, d: ld16(d, src[s, k, r:r + RA, pl.ds(n * QF + j * LANES, LANES)]),
                            put, SWAPPED)
            for r in range(0, CD, RA):
                for c in range(0, QD, LANES):
                    def put(n, v):
                        sd[c // LANES, i * (CD // RA) + r // RA, n] = _pack(v)
                    yield from two_level(
                        _rhs7, lambda k, n, d: ld16(d, fd[s, k, r:r + RA, pl.ds(n * QD + c, LANES)]), put, SWAPPED)
            for r in range(0, CO, RA):
                for c in range(0, HD, LANES):
                    d = yield
                    q = [ld16(d, stg[k, pl.ds(mo(i * CO + r, RA), RA), pl.ds(n * HD + c, LANES)])
                         for k in range(2) for n in range(2)]
                    for n, v in enumerate(_rhs7(*q)):
                        wo[c // LANES, i * (CO // RA) + r // RA, n] = _pack(v)
        ffn_steps = N2 * (2 * CU * NJ + CD * QD // LANES) // RA + CO * HD // (RA * LANES)

        def project(p, i, fill):
            for c0 in range(0, HD, TN):
                def emit(a, b, v):
                    for t in range(TN // LANES):
                        qkv_s[p * NT + (b * HD + c0) // LANES + t, pl.ds(mo(i * TM + (HALO + a * HM), RS), HM)] = (
                            v[:, t * LANES:(t + 1) * LANES])
                _strassen1(lambda n: _mm(
                    _operand(xc, n, range(NT // 2), pl.ds(i * (HM // RA), HM // RA)),
                    _operand(wkv if p else wq, n, [(p // 2 * HD + c) // LANES for c in range(c0, c0 + TN, LANES)])), fill, emit)

        x_cp(0).start()
        w_cp(0).start()
        w_cp(1).start()
        x_cp(0).wait()
        w_cp(2).start()
        lax.fori_loop(0, 2, lambda r, _: _run(ln_work(r * QM, lambda e: r * (QM // RA) + e, range(0, QM, RA))), None)

        def first_weights(c, _):
            w_cp(c).wait()

            pl.when(c == cfg["D3"])(w_cp(3).start)
            pl.when(c == cfg["DX"])(x_cp(1).start)
            pl.when(c == 3)(w_cp(4).start)
            _run(att_work(c, wq, 0))
        lax.fori_loop(0, 4, first_weights, None)

        def q_step(i, _):
            zero[0] = jnp.minimum(i, 0)

            pl.when(i + 2 < NB)(lambda: x_cp(i + 2).start())
            pl.when(i + 5 < 12)(lambda: w_cp(i + 5).start())
            pl.when(i + 5 >= 12)(wo_cp(0).start)
            for n, c in enumerate(f_cp(0)):
                pl.when(i == NB - 4 + n)(c.start)
            pl.when(i + 1 < NB)(lambda: x_cp(i + 1).wait())
            nxt = jnp.minimum(i + 1, NB - 1)
            fl = _paced(ln_work(nxt * TM, lambda e: i * (HM // RA) + (HM // RA + e), range(0, HM, RA)), 10 * HM // RA + 1, *cfg["LR"])
            fw = _paced(att_work(i + 4, wkv, i // 4, w_cp(i + 4).wait), 8 * CH // RA, *cfg["LQ"])
            project(0, i, lambda r: (fl(r), fw(r)))
        lax.fori_loop(0, NB, q_step, None)

        def kv_step(i, _):
            zero[0] = jnp.minimum(i, 0)

            @pl.when(i + NS - 1 < NB)
            def _():
                for c in f_cp(i + NS - 1):
                    c.start()

            pl.when(i < 3)(lambda: wo_cp(i + 1).start())
            pl.when(i < 4)(lambda: wo_cp(i).wait())
            for c in f_cp(i):
                c.wait()
            fw = _paced(ffn_work(i), ffn_steps, 1, 2 * NP - cfg['KE'])
            project(1, i, fw)
            project(2, i, fw)
        lax.fori_loop(0, NB, kv_step, None)

    def phase_b(h_s, hc, ac, oc, o_s, osem, word):
        scale = (D // H) ** -0.5
        attn_steps = (4 * (NT + W) + NT // 2) * HM // RA
        ln_steps = (12 + N2 * QD // LANES) * QM // RA

        def attn_work(base, rs, first, sq, sv, ahead):
            lane = lax.broadcasted_iota(jnp.int32, (RS, LANES), 1)

            def taps(r0, t, n):
                for back in range(-(n - 1) * RS, DIL * W, DIL):
                    v = qkv_s[t, pl.ds(base + (HALO + r0 - back), RS), :]
                    yield v, [(g, (back + g * RS) // DIL) for g in range(n) if 0 <= back + g * RS < DIL * W]

            def softmax(r0, ls):
                for b in (1, 2):
                    m = (lane & b) != 0
                    ls = [jnp.where(m, y, x) + _lane_xor(jnp.where(m, x, y), b) for x, y in zip(ls[0::2], ls[1::2])]
                for b in (2, 1):
                    m = (lane & b) != 0
                    ls = [v for a, c in [(a, _lane_xor(a, b)) for a in ls]
                          for v in (jnp.where(m, c, a), jnp.where(m, a, c))]
                out = []
                for g in range(len(ls) // W):
                    lg = ls[g * W:(g + 1) * W]
                    if first and r0 + g * RS < HALO:
                        pos = base + (r0 + g * RS) + lax.broadcasted_iota(jnp.int32, (RS, LANES), 0)
                        lg = [jnp.where(pos >= DIL * w, a, -1e9 / scale) if w else a for w, a in enumerate(lg)]
                    m = functools.reduce(jnp.maximum, lg)
                    ps = [jnp.exp2((a - m) * (scale * math.log2(math.e))) for a in lg]
                    inv = 1.0 / functools.reduce(lambda a, b: a + b, ps)
                    out.append([p * inv for p in ps])
                return out

            def scores(r0):
                acc = {}
                for t in range(NT):
                    q = []
                    for g in range(sq):
                        d = yield
                        v = qkv_s[t, pl.ds(base + (HALO + r0 + g * RS), RS), :]
                        q.append(v if d is None else behind(d, v))
                    for v, uses in taps(r0, NT + t, sq):
                        for g, w in uses:
                            _accumulate(acc, (g, w), 1, q[g] * v)
                return softmax(r0, [acc[g, w] for g in range(sq) for w in range(W)])

            def values(r0, ps):
                acc = {}
                for row in zip(*[taps(r0, 2 * NT + t, sv) for t in range(NT)]):
                    for g, w in row[0][1]:
                        d = yield
                        p = ps[g][w] if d is None else behind(d, ps[g][w])
                        for t in range(NT):
                            _accumulate(acc, (g, t), 1, p * row[t][0])
                return [[acc[g, t] for t in range(NT)] for g in range(sv)]

            starts = [r + k * HM + e for r in rs for k in range(2) for e in range(0, RA, RS)]
            ps, outs, halves, nq, nv = [], [], [], 0, 0
            while nv < len(starts):
                if nq < len(starts) and nq < nv + sv + ahead:
                    ps += yield from scores(starts[nq])
                    nq += sq
                    continue
                outs += yield from values(starts[nv], ps[nv:nv + sv])
                nv += sv
                if len(outs) == 2:
                    halves.append(_unskew(_skew([_pack(jnp.concatenate(o, axis=0)) for o in zip(*outs)])))
                    outs = []
                if len(halves) == 2:
                    dst = starts[nv - 4]
                    for t in range(NT // 2):
                        d = yield
                        q = [ld16(d, pltpu.bitcast(halves[k][e * NT // 2 + t], BF)) for k in range(2) for e in range(2)]
                        for p, v in enumerate(_lhs7(*q)):
                            oc[t, (base + dst if first else dst) // RA, p] = _pack(v)
                    halves = []

        def out_proj(i, slot, rs, fill):
            for c0 in range(0, HD, TN):
                def emit(a, b, v):
                    cols = pl.ds(b * HD + c0, TN)
                    for g, r in enumerate(rs):
                        h_s[pl.ds(mo(slot * TM + (a * HM + r), RA), RA), cols] = (
                            x_s[pl.ds(mo(i * TM + (a * HM + r), RA), RA), cols].astype(F32) + v[g * RA:(g + 1) * RA])

                def prod(n):
                    lhs = jnp.concatenate([_operand(oc, n, range(NT // 2), pl.ds(r // RA, 1)) for r in rs], axis=0)
                    return _mm(lhs, _operand(wo, n, range(c0 // LANES, (c0 + TN) // LANES)))
                _strassen1(prod, fill, emit, cfg['WO'])

        def ln_work(slot, rs):
            tile = yield from ln_stats(h_s, [slot * TM + (k * QM + r) for r in rs for k in range(4)], cen)
            for g, r in enumerate(rs):
                for c in range(QD // LANES):
                    def put(p, v):
                        hc[c, r // RA, p] = _pack(v)
                    yield from two_level(_lhs7, lambda k, n, d: tile(4 * g + k, n * QD // LANES + c, d), put)

        for t in range(NT, 3 * NT):
            qkv_s[t, 0:HALO, :] = jnp.broadcast_to(qkv_s[t, HALO:HALO + 1, :], (HALO, LANES))
        word[0] = 0
        part = [[r + k * QM for k in range(2) for r in range(h * QM // 2, (h + 1) * QM // 2, RA)] for h in range(2)]
        lax.fori_loop(0, 2, lambda k, _: _run(attn_work(mo(k * QM, QM), part[0][:len(part[0]) // 2], True,
                                                        *cfg['AF'])), None)
        zero[0] = word[0]
        out_proj(0, 0, part[0], _paced(attn_work(0, part[1], False, *cfg['AG']), attn_steps // 2, 1, NP - cfg["E1"]))
        out_proj(0, 0, part[1], _paced(ln_work(0, range(0, QM // 2, RA)), ln_steps // 2 + 1, 1, NP - cfg["E2"]))
        _run(ln_work(0, range(QM // 2, QM, RA)))

        def out_cp(i, slot):
            return pltpu.make_async_copy(o_s.at[slot], o_h.at[pl.ds(mo(i * TM, TM), TM)], osem.at[slot])

        def step(i, _):
            slot = i % 2
            zero[0] = jnp.minimum(i, 0)

            @pl.when(i >= 2)
            def _():
                out_cp(i - 2, slot).wait()
            nxt = jnp.minimum(i + 1, NB - 1)
            fa = _paced(attn_work(nxt * TM, range(0, HM, RA), False, *cfg['AH']),
                        attn_steps, cfg["A0"], cfg["A1"])
            for j in range(NJ):
                g = _strassen2(lambda n: _mm(_operand(hc, n, range(QD // LANES)), _operand(sgu, n, [2 * j])), fa)
                g = [[_gelu(v) for v in row] for row in g]
                u = _strassen2(lambda n: _mm(_operand(hc, n, range(QD // LANES)), _operand(sgu, n, [2 * j + 1])), fa)
                act = [[a * b for a, b in zip(*rows)] for rows in zip(g, u)]
                for p, v in enumerate(_two_level(_lhs7, act)):
                    ac[j, :, p] = _pack(v).reshape(-1, RS, LANES)
            out_proj(nxt, 1 - slot, range(0, HM, RA), lambda r: None)
            fl = _paced(ln_work(1 - slot, range(0, QM, RA)), ln_steps + 1,
                        cfg["L0"], 49 * QD // TD - cfg["LL"])
            for c0 in range(0, QD, TD):
                cs = _strassen2(lambda n: _mm(_operand(ac, n, range(NJ)), _operand(sd, n, range(c0 // LANES, (c0 + TD) // LANES))), fl)
                for a in range(4):
                    for b in range(4):
                        cols = pl.ds(b * QD + c0, TD)
                        o_s[slot, a * QM:(a + 1) * QM, cols] = (
                            h_s[pl.ds(mo(slot * TM + a * QM, QM), QM), cols] + cs[a][b]).astype(o_s.dtype)
            out_cp(i, slot).start()
        lax.fori_loop(0, NB, step, None)
        out_cp(NB - 2, 0).wait()
        out_cp(NB - 1, 1).wait()

    V, DMA = pltpu.VMEM, pltpu.SemaphoreType.DMA
    pl.run_scoped(phase_a, V((NT // 2, (NB + 1) * HM // RA, 7, RS, LANES), U32), V((NT // 2, HD // RA, 7, RS, LANES), U32), V((NT, HD // RA, 7, RS, LANES), U32), V((2, HD, D), BF), V((2, HD // 8, D), U32),
                  V((NS, 4, QD // NB, 4 * QF), BF), V((NS, 4, QD // NB, 4 * QF), BF),
                  V((NS, 4, QF // NB, D), BF), DMA((NB,)), DMA((4,)), DMA((NS,)))
    pl.run_scoped(phase_b, V((2 * TM, D), F32), V((QD // LANES, QM // RA, 49, RS, LANES), U32), V((NJ + 1, QM // RA, 49, RS, LANES), U32),
                  V((NT // 2, HM // RA, 7, RS, LANES), U32), V((2, TM, D), o_h.dtype), DMA((2,)), pltpu.SMEM((1,), jnp.int32))


def make(**kw):
    cfg = dict(TM=256, TN=256, TD=256, NS=2, LQ=(9, 13), LR=(1, 8), EU=2, A0=1, A1=640, L0=1, LL=4, KE=1, FINE=1,
               AF=(2, 2, 2), AH=(2, 2, 2), WO=(0, 3, 1, 6, 4, 2, 5), CAT=0, NB=1, E1=2, E2=1, AG=(1, 1, 2), D3=0, DX=1)
    cfg.update(kw)

    @jax.jit
    def fn(A_x, A_wqkv, A_wo, B_x, B_w_gate, B_w_up, B_w_down):
        del B_x
        B, S, D = A_x.shape
        F = B_w_gate.shape[1]
        anyspec = pl.BlockSpec(memory_space=pl.ANY)
        V = pltpu.VMEM
        out = pl.pallas_call(
            functools.partial(_kernel, **cfg),
            in_specs=[anyspec] * 6,
            out_specs=anyspec,
            out_shape=jax.ShapeDtypeStruct((S, D), A_x.dtype),
            scratch_shapes=[
                V((S, D), BF), V((D // 2 // LANES, D // 2 // RA, 7, RS, LANES), U32), V((F // 2 // LANES, D // 4 // RA, 49, RS, LANES), U32),
                V((D // 4 // LANES, F // 4 // RA, 49, RS, LANES), U32), V((3 * D // LANES, S + HALO, LANES), F32), V((cfg['TM'], D), F32),
            ],
            compiler_params=pltpu.CompilerParams(vmem_limit_bytes=127 * 1024 * 1024, disable_bounds_checks=bool(cfg.get("NB", 0))),
        )(A_x.reshape(S, D), A_wqkv.reshape(2, D // 2, 3 * D), A_wo.reshape(2, D // 2, D),
          B_w_gate.reshape(4, D // 4, F), B_w_up.reshape(4, D // 4, F), B_w_down.reshape(4, F // 4, D))
        return out.reshape(B, S, D)
    return fn


pallas_sequential_preLN__sliding_local_dilated__glu_gated_geglu__prompt_kernel = make()
```

```python
import functools
import math
import jax
import jax.numpy as jnp
from jax import lax
import jax.experimental.pallas as pl
import jax.experimental.pallas.tpu as pltpu

H = 32
W = 8
DIL = 2
HALO = 16
EPS = 1e-5
LANES = 128
RA = 16
RS = 8
BF = jnp.bfloat16
F32 = jnp.float32
U32 = jnp.uint32
SWAPPED = (0, 1, 4)


def _pack(v):
    return pltpu.bitcast(v.astype(BF), U32)


def _mm(a, b):
    return jnp.dot(pltpu.bitcast(a, BF), pltpu.bitcast(b, BF), preferred_element_type=F32)


def _operand(ref, n, tiles, rows=slice(None)):
    return jnp.concatenate([ref[t, rows, n].reshape(-1, LANES) for t in tiles], axis=1)


def _lane_xor(v, b):
    lane = lax.broadcasted_iota(jnp.int32, v.shape, 1)
    return jnp.take_along_axis(v, lane ^ b, axis=1) if b else v


def _skew(tiles):
    return [x if a == 0 else pltpu.roll(x, 4 * a, 1) for a, x in enumerate(tiles)]


def _unskew(t):
    lane = lax.broadcasted_iota(jnp.int32, t[0].shape, 1)
    t = [t[(-c) % 8] for c in range(8)]
    for b in (1, 2, 4):
        m = (lane & (4 * b)) != 0
        t = [jnp.where(m, t[(c - b) % 8], t[c]) for c in range(8)]
    return [x if c == 0 else pltpu.roll(x, LANES - 4 * c, 1) for c, x in enumerate(t)]


def _gelu(x):
    c = math.sqrt(2.0 / math.pi)
    inner = x * (c + (c * 0.044715) * (x * x))
    hx = 0.5 * x
    return hx + hx * jnp.tanh(inner)


def _lhs7(a11, a12, a21, a22):
    return (a11 + a22, a21 + a22, a11, a22, a11 + a12, a21 - a11, a12 - a22)


def _rhs7(b11, b12, b21, b22):
    return (b11 + b22, b11, b12 - b22, b21 - b11, b22, b11 + b12, b21 + b22)


def _two_level(f, blk, swapped=()):
    o = {(r, c): f(blk[r][c], blk[r][2 + c], blk[2 + r][c], blk[2 + r][2 + c]) for r in range(2) for c in range(2)}
    out = []
    for p in range(7):
        s = int(p in swapped)
        out += f(o[0, s][p], o[0, 1 - s][p], o[1, s][p], o[1, 1 - s][p])
    return out


_USES = (((0, 1), (3, 1)), ((2, 1), (3, -1)), ((1, 1), (3, 1)), ((0, 1), (2, 1)), ((0, -1), (1, 1)), ((3, 1),), ((0, 1),))


def _accumulate(acc, key, sign, v):
    acc[key] = (v if sign > 0 else -v) if key not in acc else acc[key] + v if sign > 0 else acc[key] - v
    return acc[key]


def _strassen1(prod, fill, emit, order=(6, 3, 1, 5, 0, 4, 2)):
    acc = {}
    last = {c: p for p in order for c, _ in _USES[p]}
    for p in order:
        m = prod(p)
        for c, sign in _USES[p]:
            v = _accumulate(acc, c, sign, m)
            if last[c] == p:
                emit(c // 2, c % 2, v)
        fill(m)


def _combine(m):
    add = lambda a, b: [x + y for x, y in zip(a, b)]
    sub = lambda a, b: [x - y for x, y in zip(a, b)]
    m1 = m(0)
    m4 = m(3)
    c11 = add(m1, m4)
    m2 = m(1)
    c21 = add(m2, m4)
    c22 = sub(m1, m2)
    c11 = add(c11, m(6))
    m5 = m(4)
    c11 = sub(c11, m5)
    m3 = m(2)
    c12 = add(m3, m5)
    c22 = add(c22, m3)
    c22 = add(c22, m(5))
    return c11, c12, c21, c22


def _strassen2(prod, fill):
    def inner(n):
        r = prod(n)
        fill(r)
        return [r]

    def outer(p):
        a, b, c, d = _combine(lambda q: inner(7 * p + q))
        return b + a + d + c if p in SWAPPED else a + b + c + d
    c = _combine(outer)
    return [[c[2 * (r // 2) + k // 2][2 * (r % 2) + k % 2] for k in range(4)] for r in range(4)]


def _paced(work, steps, first, last):
    calls = [0]

    def fill(r):
        calls[0] += 1
        if calls[0] == first:
            next(work, None)
        if first <= calls[0] <= last:
            k, n = calls[0] - first, last - first + 1
            rows, tiles = r.shape[0] // RS, r.shape[1] // LANES
            for g in range(-(-k * steps // n), -(-(k + 1) * steps // n)):
                t, a = divmod((g * n - k * steps) * rows * tiles // steps, rows)
                try:
                    work.send(r[a * RS:(a + 1) * RS, t * LANES:(t + 1) * LANES])
                    assert g + 1 < steps
                except StopIteration:
                    assert g + 1 == steps, (g, steps)
    return fill


def _run(work):
    for _ in work:
        pass


def _kernel(x_h, wqkv_h, wo_h, wg_h, wu_h, wd_h, o_h, x_s, wo, sgu, sd, qkv_s, cen, xc, wq, **cfg):
    S, D = x_h.shape
    QF = wd_h.shape[1]
    TM, TN, TD, NS = cfg["TM"], cfg["TN"], cfg["TD"], cfg["NS"]
    NT, NB, NJ = D // LANES, S // TM, QF // LANES
    HM, HD, QM, QD = TM // 2, D // 2, TM // 4, D // 4
    NP = 7 * HD // TN
    CK = -(-HD // (RA * (NB - 1))) * RA
    mo = pl.multiple_of
    zero = [None]

    def behind(dep, v):
        lane = lax.broadcasted_iota(jnp.int32, v.shape, 1)
        return jnp.where(lane < zero[0], pltpu.bitcast(dep[-RS:, -LANES:], v.dtype), v)

    def rows2(r, n=RA):
        return pl.ds(r // 2 if isinstance(r, int) else mo(r // 2, RS), n // 2)

    def ld16(dep, v):
        if dep is None:
            return v.astype(F32)
        if v.dtype == BF:
            return pltpu.bitcast(behind(dep, pltpu.bitcast(v, U32)), BF).astype(F32)
        return jnp.concatenate([behind(dep, v[:RS]), behind(dep, v[RS:])], axis=0)

    def ln_stats(src, rows, cen):
        add = lambda a, b: a + b
        at = lambda k, t: (slice(k * RA, (k + 1) * RA), slice(t * LANES, (t + 1) * LANES))
        ld = lambda k, t: src[pl.ds(mo(rows[k], RA), RA), t * LANES:(t + 1) * LANES]
        ms, rs = [], []
        for k in range(len(rows)):
            d = yield
            xs = [ld16(d if src.dtype == BF or t == 0 else None, ld(k, t)) for t in range(NT)]
            if src.dtype == BF:
                for t in range(NT):
                    cen[at(k, t)] = xs[t]
            m = jnp.sum(functools.reduce(add, xs), axis=-1, keepdims=True)
            ms.append(jnp.broadcast_to(m * (1.0 / D), (RA, LANES)))
        for k in range(len(rows)):
            v = []
            for t in range(NT):
                if t % (NT // 2) == 0:
                    m = ld16((yield), ms[k])
                c = (cen[at(k, t)] if src.dtype == BF else ld(k, t)) - m
                cen[at(k, t)] = c
                v.append(c * c)
            v = jnp.sum(functools.reduce(add, v), axis=-1, keepdims=True)
            rs.append(jnp.broadcast_to(lax.rsqrt(v * (1.0 / D) + EPS), (RA, LANES)))
        yield
        ready = functools.reduce(add, rs)

        def tile(k, t, d):
            if d is not None and k == 0 and t == 0:
                d = d + (ready[:RS] + ready[RS:])
            return cen[at(k, t)] * ld16(d, rs[k])
        return tile

    def two_level(f, load, put, swapped=()):
        quad = lambda a, b, d: [load(2 * a + r, 2 * b + c, d) for r in range(2) for c in range(2)]

        def inner(p, q):
            for n, v in enumerate(f(q[1], q[0], q[3], q[2]) if p in swapped else f(*q)):
                put(7 * p + n, v)
            return v

        def later(q):
            if cfg["FINE"]:
                d = yield
                return [ld16(d, v) for v in q]
            return q
        q11 = quad(0, 0, (yield))
        inner(2 if f is _lhs7 else 1, q11)
        q22 = quad(1, 1, (yield))
        inner(3 if f is _lhs7 else 4, q22)
        q22 = yield from later(q22)
        inner(0, [a + b for a, b in zip(q11, q22)])
        q12 = quad(0, 1, (yield))
        inner(4 if f is _lhs7 else 5, [a + b for a, b in zip(q11, q12)])
        q12 = yield from later(q12)
        inner(6 if f is _lhs7 else 2, [a - b for a, b in zip(q12, q22)])
        q21 = quad(1, 0, (yield))
        inner(5 if f is _lhs7 else 3, [a - b for a, b in zip(q21, q11)])
        q21 = yield from later(q21)
        return inner(1 if f is _lhs7 else 6, [a + b for a, b in zip(q21, q22)])
    N2 = 7 if cfg["FINE"] else 4

    def project(wa, p, i, fill):
        for c0 in range(0, HD, TN):
            def emit(a, b, v):
                for t in range(TN // LANES):
                    qkv_s[p * NT + (b * HD + c0) // LANES + t, pl.ds(mo(i * TM + (HALO + a * HM), RS), HM)] = (
                        v[:, t * LANES:(t + 1) * LANES])
            _strassen1(lambda n: _mm(
                _operand(xc, n, range(NT // 2), pl.ds(i * (HM // RA), HM // RA)),
                _operand(wa, n, [(p // 2 * HD + c) // LANES for c in range(c0, c0 + TN, LANES)])), fill, emit)

    def phase_a(wkv, stg, skv, tmp, fg, fu, fd, xsem, wsem, ksem, fsem):
        CH = HD // 4
        CU, CD, CO = QD // NB, QF // NB, HD // NB

        def x_cp(i):
            rows = pl.ds(mo(i * TM, TM), TM)
            return pltpu.make_async_copy(x_h.at[rows], x_s.at[rows], xsem.at[i])

        def w_cp(src, c):
            rows = pl.ds(mo(c * CH, CH), CH)
            return pltpu.make_async_copy(src.at[:, rows, pl.ds(0, D)], stg.at[:, rows], wsem.at[c])

        def kv_group(i):
            return jnp.minimum(i * (CK // RA), (HD - CK) // RA)

        def kv_cp(i):
            return pltpu.make_async_copy(wqkv_h.at[:, pl.ds(mo(kv_group(i) * RA, RA), CK), pl.ds(D, 2 * D)],
                                         skv.at[i % 2], ksem.at[i % 2])

        def f_cp(i):
            s = i % NS
            return [pltpu.make_async_copy(src.at[:, pl.ds(mo(i * n, RA), n)], dst.at[s], fsem.at[s])
                    for src, dst, n in ((wg_h, fg, CU), (wu_h, fu, CU), (wd_h, fd, CD))]

        def ln_work(src, dst, rs):
            tile = yield from ln_stats(x_s, [src + (k * HM + r) for r in rs for k in range(2)], cen)
            for g, r in enumerate(rs):
                for t in range(NT // 2):
                    d = yield
                    q = [tile(2 * g + k, n * NT // 2 + t, d) for k in range(2) for n in range(2)]
                    for p, v in enumerate(_lhs7(*q)):
                        xc[t, dst(r // RA), p] = _pack(v)

        def att_work(wa, items, wait):
            wait()
            for e, (load, _, _) in enumerate(items):
                for k in range(2):
                    d = yield
                    ts = [pltpu.bitcast(load(k, t), U32) for t in range(NT)]
                    tmp[2 * e + k] = jnp.concatenate(_skew(ts if d is None else [behind(d, v) for v in ts]), axis=1)
            for e in range(2 * len(items)):
                d = yield
                ts = [tmp[e, :, t * LANES:(t + 1) * LANES] for t in range(NT)]
                tmp[e] = jnp.concatenate(_unskew(ts if d is None else [behind(d, v) for v in ts]), axis=1)
            for e, (_, tile, group) in enumerate(items):
                for t in range(NT // 2):
                    d = yield
                    q = [ld16(d, pltpu.bitcast(tmp[2 * e + k, :, pl.ds(n * HD + t * LANES, LANES)], BF))
                         for k in range(2) for n in range(2)]
                    for n, v in enumerate(_rhs7(*q)):
                        wa[tile + t, group, n] = _pack(v)

        def ffn_work(i):
            s = i % NS
            for e, src in enumerate((fg, fu)):
                for r in range(0, CU, RA):
                    for j in range(NJ):
                        def put(n, v):
                            sgu[2 * j + e, i * (CU // RA) + r // RA, n] = _pack(v)
                        yield from two_level(
                            _rhs7, lambda k, n, d: ld16(d, src[s, k, r:r + RA, pl.ds(n * QF + j * LANES, LANES)]),
                            put, SWAPPED)
            for r in range(0, CD, RA):
                for c in range(0, QD, LANES):
                    def put(n, v):
                        sd[c // LANES, i * (CD // RA) + r // RA, n] = _pack(v)
                    yield from two_level(
                        _rhs7, lambda k, n, d: ld16(d, fd[s, k, r:r + RA, pl.ds(n * QD + c, LANES)]), put, SWAPPED)
            for r in range(0, CO, RA):
                for c in range(0, HD, LANES):
                    d = yield
                    q = [ld16(d, stg[k, pl.ds(mo(i * CO + r, RA), RA), pl.ds(n * HD + c, LANES)])
                         for k in range(2) for n in range(2)]
                    for n, v in enumerate(_rhs7(*q)):
                        wo[c // LANES, i * (CO // RA) + r // RA, n] = _pack(v)
        ffn_steps = N2 * (2 * CU * NJ + CD * QD // LANES) // RA + CO * HD // (RA * LANES)

        x_cp(0).start()
        w_cp(wqkv_h, 0).start()
        w_cp(wqkv_h, 1).start()
        x_cp(0).wait()
        w_cp(wqkv_h, 2).start()
        lax.fori_loop(0, 2, lambda r, _: _run(ln_work(r * QM, lambda e: r * (QM // RA) + e, range(0, QM, RA))), None)

        def first_weights(c, _):
            w_cp(wqkv_h, c).wait()
            pl.when(c == 0)(w_cp(wqkv_h, 3).start)
            pl.when(c == 1)(x_cp(1).start)
            pl.when(c == cfg["DK"])(lambda: kv_cp(0).start())
            _run(att_work(wq, [(lambda k, t, r=r: stg[k, pl.ds(mo(c * CH + r, RA), RA), t * LANES:(t + 1) * LANES],
                                0, c * (CH // RA) + r // RA) for r in range(0, CH, RA)], lambda: None))
        lax.fori_loop(0, 4, first_weights, None)

        def q_step(i, _):
            zero[0] = jnp.minimum(i, 0)
            pl.when(i + 2 < NB)(lambda: (x_cp(i + 2).start(), kv_cp(i + 1).start(), None)[-1])
            for n, c in enumerate(f_cp(0) + [w_cp(wo_h, 0)]):
                pl.when(i == NB - 5 + n)(c.start)
            x_cp(i + 1).wait()
            if not cfg["MW"]:
                kv_cp(i).wait()
            fl = _paced(ln_work(i * TM + TM, lambda e: i * (HM // RA) + (HM // RA + e), range(0, HM, RA)),
                        10 * HM // RA + 1, *cfg["LR"])
            items = [(lambda k, t, p=p, r=r: skv[i % 2, k, r:r + RA, pl.ds(p * D + t * LANES, LANES)],
                      p * NT // 2, kv_group(i) + r // RA) for p in range(2) for r in range(0, CK, RA)]
            fw = _paced(att_work(wkv, items, kv_cp(i).wait if cfg["MW"] else lambda: None), 8 * len(items), *cfg["LQ"])
            project(wq, 0, i, lambda r: (fl(r), fw(r)))
        lax.fori_loop(0, NB - 1, q_step, None)

        def kv_step(i, _):
            zero[0] = jnp.minimum(i, 0)

            @pl.when(i + NS - 1 < NB)
            def _():
                for c in f_cp(i + NS - 1):
                    c.start()

            pl.when(i < 3)(lambda: w_cp(wo_h, i + 1).start())
            pl.when(i < 4)(lambda: w_cp(wo_h, i).wait())
            for c in f_cp(i):
                c.wait()
            fw = _paced(ffn_work(i), ffn_steps, 1, 2 * NP - cfg['KE'])
            project(wkv, 1, i, fw)
            project(wkv, 2, i, fw)
        lax.fori_loop(0, NB, kv_step, None)

    def phase_b(h_s, hc, ac, oc, o_s, osem, word):
        scale = (D // H) ** -0.5
        attn_steps = (4 * (NT + W) + NT // 2) * HM // RA
        ln_steps = (12 + N2 * QD // LANES) * QM // RA

        def attn_work(base, rs, first, sq, sv, ahead):
            lane = lax.broadcasted_iota(jnp.int32, (RS, LANES), 1)

            def taps(r0, t, n):
                for back in range(-(n - 1) * RS, DIL * W, DIL):
                    v = qkv_s[t, pl.ds(base + (HALO + r0 - back), RS), :]
                    yield v, [(g, (back + g * RS) // DIL) for g in range(n) if 0 <= back + g * RS < DIL * W]

            def softmax(r0, ls):
                for b in (1, 2):
                    m = (lane & b) != 0
                    ls = [jnp.where(m, y, x) + _lane_xor(jnp.where(m, x, y), b) for x, y in zip(ls[0::2], ls[1::2])]
                for b in (2, 1):
                    m = (lane & b) != 0
                    ls = [v for a, c in [(a, _lane_xor(a, b)) for a in ls]
                          for v in (jnp.where(m, c, a), jnp.where(m, a, c))]
                out = []
                for g in range(len(ls) // W):
                    lg = ls[g * W:(g + 1) * W]
                    if first and r0 + g * RS < HALO:
                        pos = base + (r0 + g * RS) + lax.broadcasted_iota(jnp.int32, (RS, LANES), 0)
                        lg = [jnp.where(pos >= DIL * w, a, -1e9 / scale) if w else a for w, a in enumerate(lg)]
                    m = functools.reduce(jnp.maximum, lg)
                    ps = [jnp.exp2((a - m) * (scale * math.log2(math.e))) for a in lg]
                    inv = 1.0 / functools.reduce(lambda a, b: a + b, ps)
                    out.append([p * inv for p in ps])
                return out

            def scores(r0):
                acc = {}
                for t in range(NT):
                    q = []
                    for g in range(sq):
                        d = yield
                        v = qkv_s[t, pl.ds(base + (HALO + r0 + g * RS), RS), :]
                        q.append(v if d is None else behind(d, v))
                    for v, uses in taps(r0, NT + t, sq):
                        for g, w in uses:
                            _accumulate(acc, (g, w), 1, q[g] * v)
                return softmax(r0, [acc[g, w] for g in range(sq) for w in range(W)])

            def values(r0, ps):
                acc = {}
                for row in zip(*[taps(r0, 2 * NT + t, sv) for t in range(NT)]):
                    for g, w in row[0][1]:
                        d = yield
                        p = ps[g][w] if d is None else behind(d, ps[g][w])
                        for t in range(NT):
                            _accumulate(acc, (g, t), 1, p * row[t][0])
                return [[acc[g, t] for t in range(NT)] for g in range(sv)]

            starts = [r + k * HM + e for r in rs for k in range(2) for e in range(0, RA, RS)]
            ps, outs, halves, nq, nv = [], [], [], 0, 0
            while nv < len(starts):
                if nq < len(starts) and nq < nv + sv + ahead:
                    ps += yield from scores(starts[nq])
                    nq += sq
                    continue
                outs += yield from values(starts[nv], ps[nv:nv + sv])
                nv += sv
                if len(outs) == 2:
                    halves.append(_unskew(_skew([_pack(jnp.concatenate(o, axis=0)) for o in zip(*outs)])))
                    outs = []
                if len(halves) == 2:
                    dst = starts[nv - 4]
                    for t in range(NT // 2):
                        d = yield
                        q = [ld16(d, pltpu.bitcast(halves[k][e * NT // 2 + t], BF)) for k in range(2) for e in range(2)]
                        for p, v in enumerate(_lhs7(*q)):
                            oc[t, dst // RA, p] = _pack(v)
                    halves = []

        def out_proj(i, slot, rs, fill):
            for c0 in range(0, HD, TN):
                def emit(a, b, v):
                    cols = pl.ds(b * HD + c0, TN)
                    for g, r in enumerate(rs):
                        h_s[pl.ds(mo(slot * TM + (a * HM + r), RA), RA), cols] = (
                            x_s[pl.ds(mo(i * TM + (a * HM + r), RA), RA), cols].astype(F32) + v[g * RA:(g + 1) * RA])

                def prod(n):
                    lhs = jnp.concatenate([_operand(oc, n, range(NT // 2), pl.ds(r // RA, 1)) for r in rs], axis=0)
                    return _mm(lhs, _operand(wo, n, range(c0 // LANES, (c0 + TN) // LANES)))
                _strassen1(prod, fill, emit, cfg['WO'])

        def ln_work(slot, rs):
            tile = yield from ln_stats(h_s, [slot * TM + (k * QM + r) for r in rs for k in range(4)], cen)
            for g, r in enumerate(rs):
                for c in range(QD // LANES):
                    def put(p, v):
                        hc[c, r // RA, p] = _pack(v)
                    yield from two_level(_lhs7, lambda k, n, d: tile(4 * g + k, n * QD // LANES + c, d), put)

        word[0] = 0

        def halo(t, _):
            qkv_s[t, 0:HALO, :] = jnp.broadcast_to(qkv_s[t, HALO:HALO + 1, :], (HALO, LANES))
        lax.fori_loop(NT, 3 * NT, halo, None, unroll=8)
        zero[0] = word[0]
        part = [[r + k * QM for k in range(2) for r in range(h * QM // 2, (h + 1) * QM // 2, RA)] for h in range(2)]
        rs, n = part[0] + part[1], cfg["NA"]
        project(wq, 0, NB - 1, _paced(attn_work(0, rs[:n], True, *cfg['AF']), attn_steps // len(rs) * n,
                                      1, NP - cfg["E0"]))
        out_proj(0, 0, part[0], _paced(attn_work(0, rs[n:], True, *cfg['AG']),
                                       attn_steps // len(rs) * (len(rs) - n), 1, NP - cfg["E1"]))
        out_proj(0, 0, part[1], _paced(ln_work(0, range(0, QM // 2, RA)), ln_steps // 2 + 1, 1, NP - cfg["E2"]))
        _run(ln_work(0, range(QM // 2, QM, RA)))

        def out_cp(i, slot):
            return pltpu.make_async_copy(o_s.at[slot], o_h.at[pl.ds(mo(i * TM, TM), TM)], osem.at[slot])

        def step(i, _):
            slot = i % 2
            zero[0] = jnp.minimum(i, 0)

            @pl.when(i >= 2)
            def _():
                out_cp(i - 2, slot).wait()
            nxt = jnp.minimum(i + 1, NB - 1)
            fa = _paced(attn_work(nxt * TM, range(0, HM, RA), False, *cfg['AH']),
                        attn_steps, cfg["A0"], cfg["A1"])
            for j in range(NJ):
                g = _strassen2(lambda n: _mm(_operand(hc, n, range(QD // LANES)), _operand(sgu, n, [2 * j])), fa)
                g = [[_gelu(v) for v in row] for row in g]
                u = _strassen2(lambda n: _mm(_operand(hc, n, range(QD // LANES)), _operand(sgu, n, [2 * j + 1])), fa)
                act = [[a * b for a, b in zip(*rows)] for rows in zip(g, u)]
                for p, v in enumerate(_two_level(_lhs7, act)):
                    ac[j, :, p] = _pack(v).reshape(-1, RS, LANES)
            out_proj(nxt, 1 - slot, range(0, HM, RA), lambda r: None)
            fl = _paced(ln_work(1 - slot, range(0, QM, RA)), ln_steps + 1,
                        cfg["L0"], 49 * QD // TD - cfg["LL"])
            for c0 in range(0, QD, TD):
                cs = _strassen2(lambda n: _mm(_operand(ac, n, range(NJ)), _operand(sd, n, range(c0 // LANES, (c0 + TD) // LANES))), fl)
                for a in range(4):
                    for b in range(4):
                        cols = pl.ds(b * QD + c0, TD)
                        o_s[slot, a * QM:(a + 1) * QM, cols] = (
                            h_s[pl.ds(mo(slot * TM + a * QM, QM), QM), cols] + cs[a][b]).astype(o_s.dtype)
            out_cp(i, slot).start()
        lax.fori_loop(0, NB, step, None)
        out_cp(NB - 2, 0).wait()
        out_cp(NB - 1, 1).wait()

    V, DMA = pltpu.VMEM, pltpu.SemaphoreType.DMA
    pl.run_scoped(phase_a, V((NT, HD // RA, 7, RS, LANES), U32), V((2, HD, D), BF), V((2, 2, CK, 2 * D), BF), V((4 * CK // RA, RS, D), U32),
                  V((NS, 4, QD // NB, 4 * QF), BF), V((NS, 4, QD // NB, 4 * QF), BF),
                  V((NS, 4, QF // NB, D), BF), DMA((NB,)), DMA((4,)), DMA((2,)), DMA((NS,)))
    pl.run_scoped(phase_b, V((2 * TM, D), F32), V((QD // LANES, QM // RA, 49, RS, LANES), U32), V((NJ + 1, QM // RA, 49, RS, LANES), U32),
                  V((NT // 2, HM // RA, 7, RS, LANES), U32), V((2, TM, D), o_h.dtype), DMA((2,)), pltpu.SMEM((1,), jnp.int32))


def make(**kw):
    cfg = dict(TM=256, TN=256, TD=256, NS=2, LQ=(9, 13), LR=(1, 8), EU=2, A0=1, A1=640, L0=1, LL=4, KE=2, FINE=1,
               AF=(2, 2, 2), AH=(2, 2, 2), WO=(0, 3, 1, 6, 4, 2, 5), CAT=0, NB=1, E0=0, E1=4, E2=2, NA=6, AG=(2, 2, 2), DK=3, MW=1, D3=0, DX=1)
    cfg.update(kw)

    @jax.jit
    def fn(A_x, A_wqkv, A_wo, B_x, B_w_gate, B_w_up, B_w_down):
        del B_x
        B, S, D = A_x.shape
        F = B_w_gate.shape[1]
        anyspec = pl.BlockSpec(memory_space=pl.ANY)
        V = pltpu.VMEM
        out = pl.pallas_call(
            functools.partial(_kernel, **cfg),
            in_specs=[anyspec] * 6,
            out_specs=anyspec,
            out_shape=jax.ShapeDtypeStruct((S, D), A_x.dtype),
            scratch_shapes=[
                V((S, D), BF), V((D // 2 // LANES, D // 2 // RA, 7, RS, LANES), U32), V((F // 2 // LANES, D // 4 // RA, 49, RS, LANES), U32),
                V((D // 4 // LANES, F // 4 // RA, 49, RS, LANES), U32), V((3 * D // LANES, S + HALO, LANES), F32), V((cfg['TM'], D), F32),
                V((D // 2 // LANES, S // 2 // RA, 7, RS, LANES), U32), V((D // 2 // LANES, D // 2 // RA, 7, RS, LANES), U32),
            ],
            compiler_params=pltpu.CompilerParams(vmem_limit_bytes=127 * 1024 * 1024, disable_bounds_checks=bool(cfg.get("NB", 0))),
        )(A_x.reshape(S, D), A_wqkv.reshape(2, D // 2, 3 * D), A_wo.reshape(2, D // 2, D),
          B_w_gate.reshape(4, D // 4, F), B_w_up.reshape(4, D // 4, F), B_w_down.reshape(4, F // 4, D))
        return out.reshape(B, S, D)
    return fn


pallas_sequential_preLN__sliding_local_dilated__glu_gated_geglu__prompt_kernel = make()
```

```python
import functools
import math
import jax
import jax.numpy as jnp
from jax import lax
import jax.experimental.pallas as pl
import jax.experimental.pallas.tpu as pltpu

H = 32
W = 8
DIL = 2
EPS = 1e-5
HALO = 16
TM = 256
LANES = 128
RA = 16
RS = 8
BF = jnp.bfloat16
F32 = jnp.float32
U32 = jnp.uint32

USES = (((0, 1), (3, 1)), ((2, 1), (3, -1)), ((1, 1), (3, 1)), ((0, 1), (2, 1)), ((0, -1), (1, 1)),
        ((3, 1),), ((0, 1),))
SWAPPED = (0, 1, 4)


def _lhs7(a11, a12, a21, a22):
    return (a11 + a22, a21 + a22, a11, a22, a11 + a12, a21 - a11, a12 - a22)


def _rhs7(b11, b12, b21, b22):
    return (b11 + b22, b11, b12 - b22, b21 - b11, b22, b11 + b12, b21 + b22)


def _lhs49(blk):
    o = [_lhs7(blk[r][c], blk[r][2 + c], blk[2 + r][c], blk[2 + r][2 + c]) for r in range(2) for c in range(2)]
    return [v for p in range(7) for v in _lhs7(*[e[p] for e in o])]


def _accumulate(acc, key, sign, v):
    if key in acc:
        acc[key] = acc[key] + v if sign > 0 else acc[key] - v
    else:
        acc[key] = v if sign > 0 else -v
    return acc[key]


def _strassen1(prod, fill, emit, order):
    acc = {}
    last = {c: p for p in order for c, _ in USES[p]}
    for p in order:
        m = prod(p)
        for c, sign in USES[p]:
            v = _accumulate(acc, c, sign, m)
            if last[c] == p:
                emit(c // 2, c % 2, v)
        fill(m)


def _combine(m):
    add = lambda a, b: [x + y for x, y in zip(a, b)]
    sub = lambda a, b: [x - y for x, y in zip(a, b)]
    m1 = m(0)
    m4 = m(3)
    c11 = add(m1, m4)
    m2 = m(1)
    c21 = add(m2, m4)
    c22 = sub(m1, m2)
    c11 = add(c11, m(6))
    m5 = m(4)
    c11 = sub(c11, m5)
    m3 = m(2)
    c12 = add(m3, m5)
    c22 = add(c22, m3)
    c22 = add(c22, m(5))
    return c11, c12, c21, c22


def _strassen2(prod, fill):
    def inner(n):
        r = prod(n)
        fill(r)
        return [r]

    def outer(p):
        a, b, c, d = _combine(lambda q: inner(7 * p + q))
        return b + a + d + c if p in SWAPPED else a + b + c + d
    c = _combine(outer)
    return [[c[2 * (r // 2) + k // 2][2 * (r % 2) + k % 2] for k in range(4)] for r in range(4)]


def _pack(v):
    return pltpu.bitcast(v.astype(BF), U32)


def _operand(ref, n, tiles, groups=slice(None)):
    v = jnp.concatenate([ref[t, groups, n].reshape(-1, LANES) for t in tiles], axis=1)
    return pltpu.bitcast(v, BF)


def _mm(a, b):
    return jnp.dot(a, b, preferred_element_type=F32)


def _skew(tiles):
    return [x if a == 0 else pltpu.roll(x, 4 * a, 1) for a, x in enumerate(tiles)]


def _unskew(t):
    lane = lax.broadcasted_iota(jnp.int32, t[0].shape, 1)
    t = [t[(-c) % 8] for c in range(8)]
    for b in (1, 2, 4):
        m = (lane & (4 * b)) != 0
        t = [jnp.where(m, t[(c - b) % 8], t[c]) for c in range(8)]
    return [x if c == 0 else pltpu.roll(x, LANES - 4 * c, 1) for c, x in enumerate(t)]


def _gelu(x):
    c = math.sqrt(2.0 / math.pi)
    inner = x * (c + (c * 0.044715) * (x * x))
    hx = 0.5 * x
    return hx + hx * jnp.tanh(inner)


def _paced(work, steps, first, last):
    calls = [0]

    def fill(r):
        calls[0] += 1
        if calls[0] == first:
            next(work)
        if first <= calls[0] <= last:
            k, n = calls[0] - first, last - first + 1
            rows, tiles = r.shape[0] // RS, r.shape[1] // LANES
            for g in range(-(-k * steps // n), -(-(k + 1) * steps // n)):
                t, a = divmod((g * n - k * steps) * rows * tiles // steps, rows)
                try:
                    work.send(r[a * RS:(a + 1) * RS, t * LANES:(t + 1) * LANES])
                    assert g + 1 < steps
                except StopIteration:
                    assert g + 1 == steps
    return fill


def _run(work):
    for _ in work:
        pass


def _kernel(x_h, wqkv_h, wo_h, wg_h, wu_h, wd_h, o_h, x_s, wq, wo, wgu, wd, xc, qkv, cen, **cfg):
    S, D = x_h.shape
    QF = wd_h.shape[1]
    NT, NB, NJ = D // LANES, S // TM, QF // LANES
    HM, HD, QM, QD = TM // 2, D // 2, TM // 4, D // 4
    TN = 2 * LANES
    NP = 7 * HD // TN
    CH = HD // 4
    CK = -(-HD // (RA * (NB - 2))) * RA
    mo = pl.multiple_of
    lanes = lambda t: slice(t * LANES, (t + 1) * LANES)
    add = lambda a, b: a + b
    zero = [None]

    def behind(dep, v):
        if dep is None:
            return v
        lane = lax.broadcasted_iota(jnp.int32, v.shape, 1)
        return jnp.where(lane < zero[0], pltpu.bitcast(dep, v.dtype), v)

    def f32_behind(dep, v):
        if v.dtype == BF:
            return pltpu.bitcast(behind(dep, pltpu.bitcast(v, U32)), BF).astype(F32)
        return jnp.concatenate([behind(dep, v[:RS]), behind(dep, v[RS:])], axis=0)

    def layer_norm(src, rows):
        at = lambda k, t: (slice(k * RA, (k + 1) * RA), lanes(t))
        ld = lambda k, t: src[pl.ds(mo(rows[k], RA), RA), lanes(t)]
        ms, rs = [], []
        for k in range(len(rows)):
            d = yield
            xs = [f32_behind(d if src.dtype == BF or t == 0 else None, ld(k, t)) for t in range(NT)]
            if src.dtype == BF:
                for t in range(NT):
                    cen[at(k, t)] = xs[t]
            m = jnp.sum(functools.reduce(add, xs), axis=-1, keepdims=True)
            ms.append(jnp.broadcast_to(m * (1.0 / D), (RA, LANES)))
        for k in range(len(rows)):
            sq = []
            for t in range(NT):
                if t % (NT // 2) == 0:
                    m = f32_behind((yield), ms[k])
                c = (cen[at(k, t)] if src.dtype == BF else ld(k, t)) - m
                cen[at(k, t)] = c
                sq.append(c * c)
            v = jnp.sum(functools.reduce(add, sq), axis=-1, keepdims=True)
            rs.append(jnp.broadcast_to(lax.rsqrt(v * (1.0 / D) + EPS), (RA, LANES)))
        yield
        return lambda k, t, d: cen[at(k, t)] * f32_behind(d, rs[k])

    def operands49(f, load, put, swapped=()):
        quad = lambda a, b, d: [load(2 * a + r, 2 * b + c, d) for r in range(2) for c in range(2)]
        later = lambda q, d: [f32_behind(d, v) for v in q]
        index = (2, 3, 0, 4, 6, 5, 1) if f is _lhs7 else (1, 4, 0, 5, 2, 3, 6)

        def inner(e, q):
            for n, v in enumerate(f(q[1], q[0], q[3], q[2]) if index[e] in swapped else f(*q)):
                put(7 * index[e] + n, _pack(v))
        q11 = quad(0, 0, (yield))
        inner(0, q11)
        q22 = quad(1, 1, (yield))
        inner(1, q22)
        q22 = later(q22, (yield))
        inner(2, [a + b for a, b in zip(q11, q22)])
        q12 = quad(0, 1, (yield))
        inner(3, [a + b for a, b in zip(q11, q12)])
        inner(4, [a - b for a, b in zip(later(q12, (yield)), q22)])
        q21 = quad(1, 0, (yield))
        inner(5, [a - b for a, b in zip(q21, q11)])
        inner(6, [a + b for a, b in zip(later(q21, (yield)), q22)])

    def project(w_ref, p, i, fill):
        for c0 in range(0, HD, TN):
            def emit(a, b, v):
                for t in range(TN // LANES):
                    qkv[p * NT + (b * HD + c0) // LANES + t, pl.ds(mo(i * TM + (HALO + a * HM), RS), HM)] = (
                        v[:, lanes(t)])
            tiles = [(p // 2 * HD + c) // LANES for c in range(c0, c0 + TN, LANES)]
            _strassen1(lambda n: _mm(_operand(xc, n, range(NT // 2), pl.ds(i * (HM // RA), HM // RA)),
                                     _operand(w_ref, n, tiles)), fill, emit, (6, 3, 1, 5, 0, 4, 2))

    def projections(wkv, stage, stage_kv, tmp, stage_g, stage_u, stage_d, xsem, wsem, ksem, fsem):
        CU, CD, CO = QD // NB, QF // NB, HD // NB

        def x_cp(i):
            rows = pl.ds(mo(i * TM, TM), TM)
            return pltpu.make_async_copy(x_h.at[rows], x_s.at[rows], xsem.at[i])

        def w_cp(src, c):
            rows = pl.ds(mo(c * CH, CH), CH)
            return pltpu.make_async_copy(src.at[:, rows, pl.ds(0, D)], stage.at[:, rows], wsem.at[c])

        def kv_group(i):
            return jnp.minimum(i * (CK // RA), (HD - CK) // RA)

        def kv_cp(i):
            return pltpu.make_async_copy(wqkv_h.at[:, pl.ds(mo(kv_group(i) * RA, RA), CK), pl.ds(D, 2 * D)],
                                         stage_kv.at[i % 2], ksem.at[i % 2])

        def ffn_cp(i):
            return [pltpu.make_async_copy(src.at[:, pl.ds(mo(i * n, RA), n)], dst.at[i % 2], fsem.at[i % 2])
                    for src, dst, n in ((wg_h, stage_g, CU), (wu_h, stage_u, CU), (wd_h, stage_d, CD))]

        def norm_work(row, group, rs):
            tile = yield from layer_norm(x_s, [row + (k * HM + r) for r in rs for k in range(2)])
            for g, r in enumerate(rs):
                for t in range(NT // 2):
                    d = yield
                    q = [tile(2 * g + k, n * NT // 2 + t, d) for k in range(2) for n in range(2)]
                    for p, v in enumerate(_lhs7(*q)):
                        xc[t, group(r // RA), p] = _pack(v)

        def qkv_weight_work(w_ref, items):
            for e, (load, _, _) in enumerate(items):
                for k in range(2):
                    d = yield
                    ts = [behind(d, pltpu.bitcast(load(k, t), U32)) for t in range(NT)]
                    tmp[2 * e + k] = jnp.concatenate(_skew(ts), axis=1)
            for e in range(2 * len(items)):
                d = yield
                tmp[e] = jnp.concatenate(_unskew([behind(d, tmp[e, :, lanes(t)]) for t in range(NT)]), axis=1)
            for e, (_, tile, group) in enumerate(items):
                for t in range(NT // 2):
                    d = yield
                    q = [f32_behind(d, pltpu.bitcast(tmp[2 * e + k, :, lanes(n * NT // 2 + t)], BF))
                         for k in range(2) for n in range(2)]
                    for n, v in enumerate(_rhs7(*q)):
                        w_ref[tile + t, group, n] = _pack(v)

        def other_weight_work(i):
            s = i % 2
            for e, src in enumerate((stage_g, stage_u)):
                for r in range(0, CU, RA):
                    for j in range(NJ):
                        def put(n, v):
                            wgu[2 * j + e, i * (CU // RA) + r // RA, n] = v
                        yield from operands49(
                            _rhs7, lambda k, n, d: f32_behind(d, src[s, k, r:r + RA, lanes(n * NJ + j)]), put, SWAPPED)
            for r in range(0, CD, RA):
                for t in range(NT // 4):
                    def put(n, v):
                        wd[t, i * (CD // RA) + r // RA, n] = v
                    yield from operands49(
                        _rhs7, lambda k, n, d: f32_behind(d, stage_d[s, k, r:r + RA, lanes(n * NT // 4 + t)]),
                        put, SWAPPED)
            for r in range(0, CO, RA):
                for t in range(NT // 2):
                    d = yield
                    q = [f32_behind(d, stage[k, pl.ds(mo(i * CO + r, RA), RA), lanes(n * NT // 2 + t)])
                         for k in range(2) for n in range(2)]
                    for n, v in enumerate(_rhs7(*q)):
                        wo[t, i * (CO // RA) + r // RA, n] = _pack(v)
        other_steps = (7 * (2 * CU * NJ + CD * NT // 4) + CO * NT // 2) // RA

        x_cp(0).start()
        w_cp(wqkv_h, 0).start()
        w_cp(wqkv_h, 1).start()
        stage_kv[1] = jnp.zeros(stage_kv.shape[1:], BF)
        x_cp(0).wait()
        w_cp(wqkv_h, 2).start()
        lax.fori_loop(0, 2, lambda r, _: _run(norm_work(r * QM, lambda e: r * (QM // RA) + e, range(0, QM, RA))), None)

        def first_weights(c, _):
            w_cp(wqkv_h, c).wait()
            pl.when(c == 0)(w_cp(wqkv_h, 3).start)
            pl.when(c == 1)(x_cp(1).start)
            _run(qkv_weight_work(wq, [(lambda k, t, r=r: stage[k, pl.ds(mo(c * CH + r, RA), RA), lanes(t)],
                                       0, c * (CH // RA) + r // RA) for r in range(0, CH, RA)]))
        lax.fori_loop(0, 4, first_weights, None)

        def q_step(i, _):
            zero[0] = jnp.minimum(i, 0)

            @pl.when(i + 2 < NB)
            def _():
                x_cp(i + 2).start()
                kv_cp(i).start()
            for n, c in enumerate(ffn_cp(0) + [w_cp(wo_h, 0)]):
                pl.when(i == NB - 5 + n)(c.start)
            x_cp(i + 1).wait()
            pl.when(i > 0)(lambda: kv_cp(i - 1).wait())
            fn = _paced(norm_work(i * TM + TM, lambda e: i * (HM // RA) + (HM // RA + e), range(0, HM, RA)),
                        10 * HM // RA + 1, 1, NP // 2)
            items = [(lambda k, t, p=p, r=r: stage_kv[1 - i % 2, k, r:r + RA, lanes(p * NT + t)],
                      p * NT // 2, kv_group(jnp.maximum(i - 1, 0)) + r // RA)
                     for p in range(2) for r in range(0, CK, RA)]
            fw = _paced(qkv_weight_work(wkv, items), 8 * len(items), NP // 2 + 1, NP - 1)
            project(wq, 0, i, lambda r: (fn(r), fw(r)))
        lax.fori_loop(0, NB - 1, q_step, None)

        def kv_step(i, _):
            zero[0] = jnp.minimum(i, 0)

            @pl.when(i + 1 < NB)
            def _():
                for c in ffn_cp(i + 1):
                    c.start()
            pl.when(i < 3)(lambda: w_cp(wo_h, i + 1).start())
            pl.when(i < 4)(lambda: w_cp(wo_h, i).wait())
            for c in ffn_cp(i):
                c.wait()
            fw = _paced(other_weight_work(i), other_steps, 1, 2 * NP - cfg["KE"])
            project(wkv, 1, i, fw)
            project(wkv, 2, i, fw)
        lax.fori_loop(0, NB, kv_step, None)

    def blocks(h_s, hc, ac, oc, o_s, osem, word):
        scale = (D // H) ** -0.5
        attn_steps = (4 * (NT + W) + NT // 2) * HM // RA
        norm_steps = (12 + 7 * NT // 4) * QM // RA

        def attn_work(base, rs, first, ahead):
            lane = lax.broadcasted_iota(jnp.int32, (RS, LANES), 1)

            def taps(r0, t):
                for back in range(-RS, DIL * W, DIL):
                    v = qkv[t, pl.ds(base + (HALO + r0 - back), RS), :]
                    yield v, [(g, (back + g * RS) // DIL) for g in range(2) if 0 <= back + g * RS < DIL * W]

            def weights(r0):
                acc = {}
                for t in range(NT):
                    q = []
                    for g in range(2):
                        q.append(behind((yield), qkv[t, pl.ds(base + (HALO + r0 + g * RS), RS), :]))
                    for v, uses in taps(r0, NT + t):
                        for g, w in uses:
                            _accumulate(acc, (g, w), 1, q[g] * v)
                ls = [acc[g, w] for g in range(2) for w in range(W)]
                for b in (1, 2):
                    ls = [a + jnp.take_along_axis(a, lane ^ b, axis=1) for a in ls]
                out = []
                for g in range(2):
                    lg = ls[g * W:(g + 1) * W]
                    if first and r0 < HALO:
                        pos = r0 + g * RS + lax.broadcasted_iota(jnp.int32, (RS, LANES), 0)
                        lg = [jnp.where(pos >= DIL * w, a, -1e9 / scale) for w, a in enumerate(lg)]
                    m = functools.reduce(jnp.maximum, lg)
                    ps = [jnp.exp2((a - m) * (scale * math.log2(math.e))) for a in lg]
                    inv = 1.0 / functools.reduce(add, ps)
                    out.append([p * inv for p in ps])
                return out

            def values(r0, ps):
                acc = {}
                for row in zip(*[taps(r0, 2 * NT + t) for t in range(NT)]):
                    for g, w in row[0][1]:
                        p = behind((yield), ps[g][w])
                        for t in range(NT):
                            _accumulate(acc, (g, t), 1, p * row[t][0])
                return _unskew(_skew([_pack(jnp.concatenate([acc[0, t], acc[1, t]], axis=0)) for t in range(NT)]))

            starts = [r + k * HM for r in rs for k in range(2)]
            ps, outs = [], []
            for n, r0 in enumerate(starts):
                while len(ps) < min(len(starts), n + 1 + ahead):
                    ps.append((yield from weights(starts[len(ps)])))
                outs.append((yield from values(r0, ps[n])))
                if n % 2:
                    for t in range(NT // 2):
                        d = yield
                        q = [f32_behind(d, pltpu.bitcast(o[e * NT // 2 + t], BF)) for o in outs[-2:] for e in range(2)]
                        for p, v in enumerate(_lhs7(*q)):
                            oc[t, starts[n - 1] // RA, p] = _pack(v)

        def out_proj(i, slot, rs, fill):
            for c0 in range(0, HD, TN):
                def emit(a, b, v):
                    cols = pl.ds(b * HD + c0, TN)
                    for g, r in enumerate(rs):
                        h_s[pl.ds(mo(slot * TM + (a * HM + r), RA), RA), cols] = (
                            x_s[pl.ds(mo(i * TM + (a * HM + r), RA), RA), cols].astype(F32) + v[g * RA:(g + 1) * RA])

                def prod(n):
                    lhs = jnp.concatenate([_operand(oc, n, range(NT // 2), pl.ds(r // RA, 1)) for r in rs], axis=0)
                    return _mm(lhs, _operand(wo, n, range(c0 // LANES, (c0 + TN) // LANES)))
                _strassen1(prod, fill, emit, (0, 3, 1, 6, 4, 2, 5))

        def norm_work(slot, rs):
            tile = yield from layer_norm(h_s, [slot * TM + (k * QM + r) for r in rs for k in range(4)])
            for g, r in enumerate(rs):
                for t in range(NT // 4):
                    def put(p, v):
                        hc[t, r // RA, p] = v
                    yield from operands49(_lhs7, lambda k, n, d: tile(4 * g + k, n * NT // 4 + t, d), put)

        def halo(t, _):
            qkv[t, 0:HALO, :] = jnp.broadcast_to(qkv[t, HALO:HALO + 1, :], (HALO, LANES))
        word[0] = 0
        lax.fori_loop(NT, 3 * NT, halo, None, unroll=8)

        zero[0] = word[0]
        half = [range(h * QM // 2, (h + 1) * QM // 2, RA) for h in range(2)]
        rows = [[r + k * QM for k in range(2) for r in rs] for rs in half]
        split, calls = cfg["NA"], [0]
        fa = _paced(attn_work(0, rows[0] + rows[1], True, cfg["AF"]), attn_steps, 1, 2 * split + NP - cfg["E1"])
        fn = [_paced(norm_work(0, half[0]), norm_steps // 2 + 1, 1, NP - 2),
              _paced(norm_work(0, half[1]), norm_steps // 2 + 1, split + 1, NP)]

        def fill(r):
            calls[0] += 1
            if calls[0] <= split:
                fa(r[:, :LANES])
                fa(r[:, LANES:])
            fn[1](r)
            if calls[0] == split:
                out_proj(0, 0, rows[0], fa)
                out_proj(0, 0, rows[1], fn[0])
        project(wq, 0, NB - 1, fill)

        def out_cp(i, slot, k):
            return pltpu.make_async_copy(o_s.at[slot, pl.ds(k * HM, HM)],
                                         o_h.at[pl.ds(mo(i * TM + k * HM, HM), HM)], osem.at[2 * slot + k])

        def step(i, _):
            slot = i % 2
            zero[0] = jnp.minimum(i, 0)

            @pl.when(i >= 2)
            def _():
                out_cp(i - 2, slot, 0).wait()
                out_cp(i - 2, slot, 1).wait()
            nxt = jnp.minimum(i + 1, NB - 1)
            fa = _paced(attn_work(nxt * TM, range(0, HM, RA), False, cfg["AH"]), attn_steps, 1, 98 * NJ - cfg["A1"])
            for j in range(NJ):
                g = _strassen2(lambda n: _mm(_operand(hc, n, range(NT // 4)), _operand(wgu, n, [2 * j])), fa)
                g = [[_gelu(v) for v in row] for row in g]
                u = _strassen2(lambda n: _mm(_operand(hc, n, range(NT // 4)), _operand(wgu, n, [2 * j + 1])), fa)
                for p, v in enumerate(_lhs49([[a * b for a, b in zip(*gu)] for gu in zip(g, u)])):
                    ac[j, :, p] = _pack(v).reshape(-1, RS, LANES)
            out_proj(nxt, 1 - slot, range(0, HM, RA), lambda r: None)
            fn = _paced(norm_work(1 - slot, range(0, QM, RA)), norm_steps + 1, 1, 49 - cfg["LL"])
            y = _strassen2(lambda n: _mm(_operand(ac, n, range(NJ)), _operand(wd, n, range(NT // 4))), fn)
            for a in range(4):
                for b in range(4):
                    cols = pl.ds(b * QD, QD)
                    o_s[slot, a * QM:(a + 1) * QM, cols] = (
                        h_s[pl.ds(mo(slot * TM + a * QM, QM), QM), cols] + y[a][b]).astype(o_s.dtype)
                if a % 2:
                    out_cp(i, slot, a // 2).start()
        lax.fori_loop(0, NB, step, None)
        for i in (NB - 2, NB - 1):
            out_cp(i, i % 2, 0).wait()
            out_cp(i, i % 2, 1).wait()

    V, DMA = pltpu.VMEM, pltpu.SemaphoreType.DMA
    pl.run_scoped(projections, V((NT, HD // RA, 7, RS, LANES), U32), V((2, HD, D), BF), V((2, 2, CK, 2 * D), BF),
                  V((4 * CK // RA, RS, D), U32), V((2, 4, QD // NB, 4 * QF), BF), V((2, 4, QD // NB, 4 * QF), BF),
                  V((2, 4, QF // NB, D), BF), DMA((NB,)), DMA((4,)), DMA((2,)), DMA((2,)))
    pl.run_scoped(blocks, V((2 * TM, D), F32), V((NT // 4, QM // RA, 49, RS, LANES), U32),
                  V((NJ + 1, QM // RA, 49, RS, LANES), U32), V((NT // 2, HM // RA, 7, RS, LANES), U32),
                  V((2, TM, D), o_h.dtype), DMA((4,)), pltpu.SMEM((1,), jnp.int32))


def make(**kw):
    cfg = dict(KE=2, NA=9, E1=5, AF=1, AH=1, A1=46, LL=4, NB=True)
    cfg.update(kw)

    @jax.jit
    def fn(A_x, A_wqkv, A_wo, B_x, B_w_gate, B_w_up, B_w_down):
        del B_x
        B, S, D = A_x.shape
        F = B_w_gate.shape[1]
        hbm = pl.BlockSpec(memory_space=pl.ANY)
        operands = lambda cols, rows, n: pltpu.VMEM((cols // LANES, rows // RA, n, RS, LANES), U32)
        out = pl.pallas_call(
            functools.partial(_kernel, **cfg),
            in_specs=[hbm] * 6,
            out_specs=hbm,
            out_shape=jax.ShapeDtypeStruct((S, D), A_x.dtype),
            scratch_shapes=[
                pltpu.VMEM((S, D), BF), operands(D // 2, D // 2, 7), operands(D // 2, D // 2, 7),
                operands(F // 2, D // 4, 49), operands(D // 4, F // 4, 49), operands(D // 2, S // 2, 7),
                pltpu.VMEM((3 * D // LANES, S + HALO, LANES), F32), pltpu.VMEM((TM, D), F32),
            ],
            compiler_params=pltpu.CompilerParams(vmem_limit_bytes=127 * 1024 * 1024, disable_bounds_checks=cfg["NB"]),
        )(A_x.reshape(S, D), A_wqkv.reshape(2, D // 2, 3 * D), A_wo.reshape(2, D // 2, D),
          B_w_gate.reshape(4, D // 4, F), B_w_up.reshape(4, D // 4, F), B_w_down.reshape(4, F // 4, D))
        return out.reshape(B, S, D)
    return fn


pallas_sequential_preLN__sliding_local_dilated__glu_gated_geglu__prompt_kernel = make()
```

```python
import functools
import math
import jax
import jax.numpy as jnp
from jax import lax
import jax.experimental.pallas as pl
import jax.experimental.pallas.tpu as pltpu

H = 32
W = 8
DIL = 2
EPS = 1e-5
HALO = 16
TM = 256
LANES = 128
RA = 16
RS = 8
BF = jnp.bfloat16
F32 = jnp.float32
U32 = jnp.uint32

USES = (((0, 1), (3, 1)), ((2, 1), (3, -1)), ((1, 1), (3, 1)), ((0, 1), (2, 1)), ((0, -1), (1, 1)),
        ((3, 1),), ((0, 1),))
SWAPPED = (0, 1, 4)


def _lhs7(a11, a12, a21, a22):
    return (a11 + a22, a21 + a22, a11, a22, a11 + a12, a21 - a11, a12 - a22)


def _rhs7(b11, b12, b21, b22):
    return (b11 + b22, b11, b12 - b22, b21 - b11, b22, b11 + b12, b21 + b22)


def _lhs49(blk):
    o = [_lhs7(blk[r][c], blk[r][2 + c], blk[2 + r][c], blk[2 + r][2 + c]) for r in range(2) for c in range(2)]
    return [v for p in range(7) for v in _lhs7(*[e[p] for e in o])]


def _accumulate(acc, key, sign, v):
    if key in acc:
        acc[key] = acc[key] + v if sign > 0 else acc[key] - v
    else:
        acc[key] = v if sign > 0 else -v
    return acc[key]


def _strassen1(prod, fill, emit, order=(6, 3, 1, 5, 0, 4, 2)):
    acc = {}
    last = {c: p for p in order for c, _ in USES[p]}
    for p in order:
        m = prod(p)
        for c, sign in USES[p]:
            v = _accumulate(acc, c, sign, m)
            if last[c] == p:
                emit(c // 2, c % 2, v)
        fill(m)


def _combine(m):
    add = lambda a, b: [x + y for x, y in zip(a, b)]
    sub = lambda a, b: [x - y for x, y in zip(a, b)]
    m1 = m(0)
    m4 = m(3)
    c11 = add(m1, m4)
    m2 = m(1)
    c21 = add(m2, m4)
    c22 = sub(m1, m2)
    c11 = add(c11, m(6))
    m5 = m(4)
    c11 = sub(c11, m5)
    m3 = m(2)
    c12 = add(m3, m5)
    c22 = add(c22, m3)
    c22 = add(c22, m(5))
    return c11, c12, c21, c22


def _strassen2(prod, fill):
    def inner(n):
        r = prod(n)
        fill(r)
        return [r]

    def outer(p):
        a, b, c, d = _combine(lambda q: inner(7 * p + q))
        return b + a + d + c if p in SWAPPED else a + b + c + d
    c = _combine(outer)
    return [[c[2 * (r // 2) + k // 2][2 * (r % 2) + k % 2] for k in range(4)] for r in range(4)]


def _pack(v):
    return pltpu.bitcast(v.astype(BF), U32)


def _operand(ref, n, tiles, groups=slice(None)):
    v = jnp.concatenate([ref[t, groups, n].reshape(-1, LANES) for t in tiles], axis=1)
    return pltpu.bitcast(v, BF)


def _mm(a, b):
    return jnp.dot(a, b, preferred_element_type=F32)


def _skew(tiles):
    return [x if a == 0 else pltpu.roll(x, 4 * a, 1) for a, x in enumerate(tiles)]


def _unskew(t):
    lane = lax.broadcasted_iota(jnp.int32, t[0].shape, 1)
    t = [t[(-c) % 8] for c in range(8)]
    for b in (1, 2, 4):
        m = (lane & (4 * b)) != 0
        t = [jnp.where(m, t[(c - b) % 8], t[c]) for c in range(8)]
    return [x if c == 0 else pltpu.roll(x, LANES - 4 * c, 1) for c, x in enumerate(t)]


def _gelu(x):
    c = math.sqrt(2.0 / math.pi)
    inner = x * (c + (c * 0.044715) * (x * x))
    hx = 0.5 * x
    return hx + hx * jnp.tanh(inner)


def _paced(work, steps, first, last):
    calls = [0]

    def fill(r):
        calls[0] += 1
        if calls[0] == first:
            next(work)
        if first <= calls[0] <= last:
            k, n = calls[0] - first, last - first + 1
            rows, tiles = r.shape[0] // RS, r.shape[1] // LANES
            for g in range(-(-k * steps // n), -(-(k + 1) * steps // n)):
                t, a = divmod((g * n - k * steps) * rows * tiles // steps, rows)
                try:
                    work.send(r[a * RS:(a + 1) * RS, t * LANES:(t + 1) * LANES])
                    assert g + 1 < steps
                except StopIteration:
                    assert g + 1 == steps
    return fill


def _run(work):
    for _ in work:
        pass


def _kernel(x_h, wqkv_h, wo_h, wg_h, wu_h, wd_h, o_h, x_s, wq, wo, wgu, wd, xc, qkv, cen):
    S, D = x_h.shape
    QF = wd_h.shape[1]
    NT, NB, NJ = D // LANES, S // TM, QF // LANES
    HM, HD, QM, QD = TM // 2, D // 2, TM // 4, D // 4
    TN = 2 * LANES
    NP = 7 * HD // TN
    CH = HD // 4
    CK = -(-HD // (RA * (NB - 2))) * RA
    mo = pl.multiple_of
    lanes = lambda t: slice(t * LANES, (t + 1) * LANES)
    add = lambda a, b: a + b
    zero = [None]

    def behind(dep, v):
        if dep is None:
            return v
        lane = lax.broadcasted_iota(jnp.int32, v.shape, 1)
        return jnp.where(lane < zero[0], pltpu.bitcast(dep, v.dtype), v)

    def f32_behind(dep, v):
        if v.dtype == BF:
            return pltpu.bitcast(behind(dep, pltpu.bitcast(v, U32)), BF).astype(F32)
        return jnp.concatenate([behind(dep, v[:RS]), behind(dep, v[RS:])], axis=0)

    def layer_norm(src, rows):
        at = lambda k, t: (slice(k * RA, (k + 1) * RA), lanes(t))
        ld = lambda k, t: src[pl.ds(mo(rows[k], RA), RA), lanes(t)]
        ms, rs = [], []
        for k in range(len(rows)):
            d = yield
            xs = [f32_behind(d if src.dtype == BF or t == 0 else None, ld(k, t)) for t in range(NT)]
            if src.dtype == BF:
                for t in range(NT):
                    cen[at(k, t)] = xs[t]
            m = jnp.sum(functools.reduce(add, xs), axis=-1, keepdims=True)
            ms.append(jnp.broadcast_to(m * (1.0 / D), (RA, LANES)))
        for k in range(len(rows)):
            sq = []
            for t in range(NT):
                if t % (NT // 2) == 0:
                    m = f32_behind((yield), ms[k])
                c = (cen[at(k, t)] if src.dtype == BF else ld(k, t)) - m
                cen[at(k, t)] = c
                sq.append(c * c)
            v = jnp.sum(functools.reduce(add, sq), axis=-1, keepdims=True)
            rs.append(jnp.broadcast_to(lax.rsqrt(v * (1.0 / D) + EPS), (RA, LANES)))
        yield
        return lambda k, t, d: cen[at(k, t)] * f32_behind(d, rs[k])

    def operands49(f, load, put, swapped=()):
        quad = lambda a, b, d: [load(2 * a + r, 2 * b + c, d) for r in range(2) for c in range(2)]
        later = lambda q, d: [f32_behind(d, v) for v in q]
        index = (2, 3, 0, 4, 6, 5, 1) if f is _lhs7 else (1, 4, 0, 5, 2, 3, 6)

        def inner(e, q):
            for n, v in enumerate(f(q[1], q[0], q[3], q[2]) if index[e] in swapped else f(*q)):
                put(7 * index[e] + n, _pack(v))
        q11 = quad(0, 0, (yield))
        inner(0, q11)
        q22 = quad(1, 1, (yield))
        inner(1, q22)
        q22 = later(q22, (yield))
        inner(2, [a + b for a, b in zip(q11, q22)])
        q12 = quad(0, 1, (yield))
        inner(3, [a + b for a, b in zip(q11, q12)])
        inner(4, [a - b for a, b in zip(later(q12, (yield)), q22)])
        q21 = quad(1, 0, (yield))
        inner(5, [a - b for a, b in zip(q21, q11)])
        inner(6, [a + b for a, b in zip(later(q21, (yield)), q22)])

    def project(w_ref, p, i, fill):
        for c0 in range(0, HD, TN):
            def emit(a, b, v):
                for t in range(TN // LANES):
                    qkv[p * NT + (b * HD + c0) // LANES + t, pl.ds(mo(i * TM + (HALO + a * HM), RS), HM)] = (
                        v[:, lanes(t)])
            tiles = [(p // 2 * HD + c) // LANES for c in range(c0, c0 + TN, LANES)]
            _strassen1(lambda n: _mm(_operand(xc, n, range(NT // 2), pl.ds(i * (HM // RA), HM // RA)),
                                     _operand(w_ref, n, tiles)), fill, emit)

    def projections(wkv, stage_kv, tmp, stage_g, stage_u, stage_d, stage_o, xsem, wsem, ksem, fsem):
        CU, CD = QD // NB, QF // NB

        def x_cp(i):
            rows = pl.ds(mo(i * TM, TM), TM)
            return pltpu.make_async_copy(x_h.at[rows], x_s.at[rows], xsem.at[i])

        def q_cp(c):
            return [pltpu.make_async_copy(wqkv_h.at[k, pl.ds(mo(c * CH, CH), CH), pl.ds(0, D)],
                                          x_s.at[pl.ds(mo(S - D + k * HD + c * CH, CH), CH)], wsem.at[c])
                    for k in range(2)]

        def start(copies):
            for c in copies:
                c.start()

        def kv_group(i):
            return jnp.minimum(i * (CK // RA), (HD - CK) // RA)

        def kv_cp(i):
            return pltpu.make_async_copy(wqkv_h.at[:, pl.ds(mo(kv_group(i) * RA, RA), CK), pl.ds(D, 2 * D)],
                                         stage_kv.at[i % 2], ksem.at[i % 2])

        def ffn_cp(i):
            return [pltpu.make_async_copy(src.at[:, pl.ds(mo(i * n, RA), n)], dst.at[i % 2], fsem.at[i % 2])
                    for src, dst, n in ((wg_h, stage_g, CU), (wu_h, stage_u, CU), (wd_h, stage_d, CD),
                                        (wo_h, stage_o, CU))]

        def norm_work(row, group, rs):
            tile = yield from layer_norm(x_s, [row + (k * HM + r) for r in rs for k in range(2)])
            for g, r in enumerate(rs):
                for t in range(NT // 2):
                    d = yield
                    q = [tile(2 * g + k, n * NT // 2 + t, d) for k in range(2) for n in range(2)]
                    for p, v in enumerate(_lhs7(*q)):
                        xc[t, group(r // RA), p] = _pack(v)

        def qkv_weight_work(w_ref, items):
            for e, (load, _, _) in enumerate(items):
                for k in range(2):
                    d = yield
                    ts = [behind(d, pltpu.bitcast(load(k, t), U32)) for t in range(NT)]
                    tmp[2 * e + k] = jnp.concatenate(_skew(ts), axis=1)
            for e in range(2 * len(items)):
                d = yield
                tmp[e] = jnp.concatenate(_unskew([behind(d, tmp[e, :, lanes(t)]) for t in range(NT)]), axis=1)
            for e, (_, tile, group) in enumerate(items):
                for t in range(NT // 2):
                    d = yield
                    q = [f32_behind(d, pltpu.bitcast(tmp[2 * e + k, :, lanes(n * NT // 2 + t)], BF))
                         for k in range(2) for n in range(2)]
                    for n, v in enumerate(_rhs7(*q)):
                        w_ref[tile + t, group, n] = _pack(v)

        def other_weight_work(i):
            s = i % 2
            for e, src in enumerate((stage_g, stage_u)):
                for r in range(0, CU, RA):
                    for j in range(NJ):
                        def put(n, v):
                            wgu[2 * j + e, i * (CU // RA) + r // RA, n] = v
                        yield from operands49(
                            _rhs7, lambda k, n, d: f32_behind(d, src[s, k, r:r + RA, lanes(n * NJ + j)]), put, SWAPPED)
            for src, dst, rows in ((stage_d, wd, CD), (stage_o, wo, CU)):
                for r in range(0, rows, RA):
                    for t in range(NT // 4):
                        def put(n, v):
                            dst[t, i * (rows // RA) + r // RA, n] = v
                        yield from operands49(
                            _rhs7, lambda k, n, d: f32_behind(d, src[s, k, r:r + RA, lanes(n * NT // 4 + t)]),
                            put, SWAPPED)
        other_steps = 7 * (2 * CU * NJ + (CD + CU) * NT // 4) // RA

        x_cp(0).start()
        start(q_cp(0))
        start(q_cp(1))
        stage_kv[1] = jnp.zeros(stage_kv.shape[1:], BF)
        x_cp(0).wait()
        start(q_cp(2))
        lax.fori_loop(0, 2, lambda r, _: _run(norm_work(r * QM, lambda e: r * (QM // RA) + e, range(0, QM, RA))), None)

        def first_weights(c, _):
            for cp in q_cp(c):
                cp.wait()
            pl.when(c == 0)(lambda: start(q_cp(3)))
            pl.when(c == 1)(x_cp(1).start)
            _run(qkv_weight_work(wq, [(lambda k, t, r=r: x_s[pl.ds(mo(c * CH + (S - D + k * HD + r), RA), RA), lanes(t)],
                                       0, c * (CH // RA) + r // RA) for r in range(0, CH, RA)]))
        lax.fori_loop(0, 4, first_weights, None)

        def q_step(i, _):
            zero[0] = jnp.minimum(i, 0)

            @pl.when(i + 2 < NB)
            def _():
                x_cp(i + 2).start()
                kv_cp(i).start()
            for n, c in enumerate(ffn_cp(0)):
                pl.when(i == NB - 5 + n)(c.start)
            x_cp(i + 1).wait()
            pl.when(i > 0)(lambda: kv_cp(i - 1).wait())
            fn = _paced(norm_work(i * TM + TM, lambda e: i * (HM // RA) + (HM // RA + e), range(0, HM, RA)),
                        10 * HM // RA + 1, 1, NP // 2)
            items = [(lambda k, t, p=p, r=r: stage_kv[1 - i % 2, k, r:r + RA, lanes(p * NT + t)],
                      p * NT // 2, kv_group(jnp.maximum(i - 1, 0)) + r // RA)
                     for p in range(2) for r in range(0, CK, RA)]
            fw = _paced(qkv_weight_work(wkv, items), 8 * len(items), NP // 2 + 1, NP - 1)
            project(wq, 0, i, lambda r: (fn(r), fw(r)))
        lax.fori_loop(0, NB - 1, q_step, None)

        def kv_step(i, _):
            zero[0] = jnp.minimum(i, 0)

            @pl.when(i + 1 < NB)
            def _():
                for c in ffn_cp(i + 1):
                    c.start()
            for c in ffn_cp(i):
                c.wait()
            fw = _paced(other_weight_work(i), other_steps, 1, 2 * NP - 2)
            project(wkv, 1, i, fw)
            project(wkv, 2, i, fw)
        lax.fori_loop(0, NB, kv_step, None)

    def blocks(h_s, hc, ac, oc, o_s, osem, word):
        scale = (D // H) ** -0.5
        attn_steps = (8 * (NT + W) + 7 * NT // 4) * QM // RA + 2 * W
        norm_steps = (12 + 7 * NT // 4) * QM // RA

        def attn_work(base, rs, first):
            lane = lax.broadcasted_iota(jnp.int32, (RS, LANES), 1)

            done = []

            def taps(r0, t):
                for back in range(-RS, DIL * W, DIL):
                    v = qkv[t, pl.ds(base + (HALO + r0 - back), RS), :]
                    yield v, [(g, (back + g * RS) // DIL) for g in range(2) if 0 <= back + g * RS < DIL * W]

            def weights(r0):
                acc = {}
                for t in range(NT):
                    q = []
                    for g in range(2):
                        q.append(behind((yield), qkv[t, pl.ds(base + (HALO + r0 + g * RS), RS), :]))
                    for v, uses in taps(r0, NT + t):
                        for g, w in uses:
                            _accumulate(acc, (g, w), 1, q[g] * v)
                ls = [acc[g, w] for g in range(2) for w in range(W)]
                for b in (1, 2):
                    ls = [a + jnp.take_along_axis(a, lane ^ b, axis=1) for a in ls]
                out = []
                for g in range(2):
                    lg = ls[g * W:(g + 1) * W]
                    if first and r0 < HALO:
                        pos = r0 + g * RS + lax.broadcasted_iota(jnp.int32, (RS, LANES), 0)
                        lg = [jnp.where(pos >= DIL * w, a, -1e9 / scale) for w, a in enumerate(lg)]
                    m = functools.reduce(jnp.maximum, lg)
                    ps = [jnp.exp2((a - m) * (scale * math.log2(math.e))) for a in lg]
                    inv = 1.0 / functools.reduce(add, ps)
                    out.append([p * inv for p in ps])
                return out

            def values(r0, ps):
                acc = {}
                for row in zip(*[taps(r0, 2 * NT + t) for t in range(NT)]):
                    for g, w in row[0][1]:
                        d = yield
                        if done and w == W - 1:
                            d = pltpu.bitcast(d, U32) | done.pop()
                        p = behind(d, ps[g][w])
                        for t in range(NT):
                            _accumulate(acc, (g, t), 1, p * row[t][0])
                return _unskew(_skew([_pack(jnp.concatenate([acc[0, t], acc[1, t]], axis=0)) for t in range(NT)]))

            starts = [r + k * QM for r in rs for k in range(4)]
            ps, outs = [], []
            for n in range(len(starts) + 1):
                while len(ps) < min(len(starts), n + 2):
                    ps.append((yield from weights(starts[len(ps)])))
                if n == len(starts):
                    for _ in range(2 * W):
                        yield
                if n and n % 4 == 0:
                    for t in range(NT // 4):
                        def put(p, v):
                            oc[t, starts[n - 4] // RA, p] = v
                            done[:] = [v | done[0]] if done else [v]
                        yield from operands49(_lhs7, lambda k, e, d: f32_behind(
                            d, pltpu.bitcast(outs[n - 4 + k][e * NT // 4 + t], BF)), put)
                if n < len(starts):
                    outs.append((yield from values(starts[n], ps[n])))

        def out_proj(i, slot, rs, fill):
            groups = pl.ds(rs[0] // RA, len(rs))
            for t in range(NT // 4):
                y = _strassen2(lambda n: _mm(_operand(oc, n, range(NT // 4), groups), _operand(wo, n, [t])), fill)
                for a in range(4):
                    for b in range(4):
                        cols = lanes(b * NT // 4 + t)
                        h_s[pl.ds(mo(slot * TM + (a * QM + rs[0]), RA), len(rs) * RA), cols] = (
                            x_s[pl.ds(mo(i * TM + (a * QM + rs[0]), RA), len(rs) * RA), cols].astype(F32) + y[a][b])

        def norm_work(slot, rs):
            tile = yield from layer_norm(h_s, [slot * TM + (k * QM + r) for r in rs for k in range(4)])
            for g, r in enumerate(rs):
                for t in range(NT // 4):
                    def put(p, v):
                        hc[t, r // RA, p] = v
                    yield from operands49(_lhs7, lambda k, n, d: tile(4 * g + k, n * NT // 4 + t, d), put)

        def halo(t, _):
            qkv[t, 0:HALO, :] = jnp.broadcast_to(qkv[t, HALO:HALO + 1, :], (HALO, LANES))
        word[0] = 0
        lax.fori_loop(NT, 3 * NT, halo, None, unroll=8)

        zero[0] = word[0]
        half = [range(h * QM // 2, (h + 1) * QM // 2, RA) for h in range(2)]
        split, calls = 10, [0]
        fa = _paced(attn_work(0, range(0, QM, RA), True), attn_steps, 1, 16 * split + 49)
        fn = [_paced(norm_work(0, half[0]), norm_steps // 2 + 1, 1, 84),
              _paced(norm_work(0, half[1]), norm_steps // 2 + 1, split + 1, NP)]

        def fill(r):
            calls[0] += 1
            if calls[0] <= split:
                for t in range(TN // LANES):
                    for a in range(0, HM, RA):
                        fa(r[a:a + RA, lanes(t)])
            fn[1](r)
            if calls[0] == split:
                out_proj(0, 0, half[0], fa)
                out_proj(0, 0, half[1], fn[0])
        project(wq, 0, NB - 1, fill)

        def out_cp(i, slot, k):
            return pltpu.make_async_copy(o_s.at[slot, pl.ds(k * HM, HM)],
                                         o_h.at[pl.ds(mo(i * TM + k * HM, HM), HM)], osem.at[2 * slot + k])

        def step(i, _):
            slot = i % 2
            zero[0] = jnp.minimum(i, 0)

            @pl.when(i >= 2)
            def _():
                out_cp(i - 2, slot, 0).wait()
                out_cp(i - 2, slot, 1).wait()
            nxt = jnp.minimum(i + 1, NB - 1)
            fa = _paced(attn_work(nxt * TM, range(0, QM, RA), False), attn_steps, 1, 98 * NJ - 10)
            for j in range(NJ):
                g = _strassen2(lambda n: _mm(_operand(hc, n, range(NT // 4)), _operand(wgu, n, [2 * j])), fa)
                g = [[_gelu(v) for v in row] for row in g]
                u = _strassen2(lambda n: _mm(_operand(hc, n, range(NT // 4)), _operand(wgu, n, [2 * j + 1])), fa)
                for p, v in enumerate(_lhs49([[a * b for a, b in zip(*gu)] for gu in zip(g, u)])):
                    ac[j, :, p] = _pack(v).reshape(-1, RS, LANES)
            out_proj(nxt, 1 - slot, range(0, QM, RA), lambda r: None)
            fn = _paced(norm_work(1 - slot, range(0, QM, RA)), norm_steps + 1, 1, 49 - 7)
            y = _strassen2(lambda n: _mm(_operand(ac, n, range(NJ)), _operand(wd, n, range(NT // 4))), fn)
            for a in range(4):
                for b in range(4):
                    cols = pl.ds(b * QD, QD)
                    o_s[slot, a * QM:(a + 1) * QM, cols] = (
                        h_s[pl.ds(mo(slot * TM + a * QM, QM), QM), cols] + y[a][b]).astype(o_s.dtype)
                if a % 2:
                    out_cp(i, slot, a // 2).start()
        lax.fori_loop(0, NB, step, None)
        for i in (NB - 2, NB - 1):
            out_cp(i, i % 2, 0).wait()
            out_cp(i, i % 2, 1).wait()

    V, DMA = pltpu.VMEM, pltpu.SemaphoreType.DMA
    pl.run_scoped(projections, V((NT, HD // RA, 7, RS, LANES), U32), V((2, 2, CK, 2 * D), BF),
                  V((4 * CK // RA, RS, D), U32), V((2, 4, QD // NB, 4 * QF), BF), V((2, 4, QD // NB, 4 * QF), BF),
                  V((2, 4, QF // NB, D), BF), V((2, 4, QD // NB, D), BF), DMA((NB,)), DMA((4,)), DMA((2,)), DMA((2,)))
    pl.run_scoped(blocks, V((2 * TM, D), F32), V((NT // 4, QM // RA, 49, RS, LANES), U32),
                  V((NJ + 1, QM // RA, 49, RS, LANES), U32), V((NT // 4, QM // RA, 49, RS, LANES), U32),
                  V((2, TM, D), o_h.dtype), DMA((4,)), pltpu.SMEM((1,), jnp.int32))


@jax.jit
def pallas_sequential_preLN__sliding_local_dilated__glu_gated_geglu__prompt_kernel(
        A_x, A_wqkv, A_wo, B_x, B_w_gate, B_w_up, B_w_down):
    del B_x
    B, S, D = A_x.shape
    F = B_w_gate.shape[1]
    hbm = pl.BlockSpec(memory_space=pl.ANY)
    operands = lambda cols, rows, n: pltpu.VMEM((cols // LANES, rows // RA, n, RS, LANES), U32)
    out = pl.pallas_call(
        _kernel,
        in_specs=[hbm] * 6,
        out_specs=hbm,
        out_shape=jax.ShapeDtypeStruct((S, D), A_x.dtype),
        scratch_shapes=[
            pltpu.VMEM((S, D), BF), operands(D // 2, D // 2, 7), operands(D // 4, D // 4, 49),
            operands(F // 2, D // 4, 49), operands(D // 4, F // 4, 49), operands(D // 2, S // 2, 7),
            pltpu.VMEM((3 * D // LANES, S + HALO, LANES), F32), pltpu.VMEM((TM, D), F32),
        ],
        compiler_params=pltpu.CompilerParams(vmem_limit_bytes=127 * 1024 * 1024, disable_bounds_checks=True),
    )(A_x.reshape(S, D), A_wqkv.reshape(2, D // 2, 3 * D), A_wo.reshape(4, D // 4, D),
      B_w_gate.reshape(4, D // 4, F), B_w_up.reshape(4, D // 4, F), B_w_down.reshape(4, F // 4, D))
    return out.reshape(B, S, D)
```

```python
import functools
import math
import jax
import jax.numpy as jnp
from jax import lax
import jax.experimental.pallas as pl
import jax.experimental.pallas.tpu as pltpu

H = 32
W = 8
DIL = 2
EPS = 1e-5
HALO = 16
TM = 256
LANES = 128
RA = 16
RS = 8
BF = jnp.bfloat16
F32 = jnp.float32
U32 = jnp.uint32

USES = (((0, 1), (3, 1)), ((2, 1), (3, -1)), ((1, 1), (3, 1)), ((0, 1), (2, 1)), ((0, -1), (1, 1)),
        ((3, 1),), ((0, 1),))
SWAPPED = (0, 1, 4)


def _lhs7(a11, a12, a21, a22):
    return (a11 + a22, a21 + a22, a11, a22, a11 + a12, a21 - a11, a12 - a22)


def _rhs7(b11, b12, b21, b22):
    return (b11 + b22, b11, b12 - b22, b21 - b11, b22, b11 + b12, b21 + b22)


def _lhs49(blk):
    o = [_lhs7(blk[r][c], blk[r][2 + c], blk[2 + r][c], blk[2 + r][2 + c]) for r in range(2) for c in range(2)]
    return [v for p in range(7) for v in _lhs7(*[e[p] for e in o])]


def _accumulate(acc, key, sign, v):
    if key in acc:
        acc[key] = acc[key] + v if sign > 0 else acc[key] - v
    else:
        acc[key] = v if sign > 0 else -v
    return acc[key]


def _strassen1(prod, fill, emit, order=(6, 3, 1, 5, 0, 4, 2)):
    acc = {}
    last = {c: p for p in order for c, _ in USES[p]}
    for p in order:
        m = prod(p)
        for c, sign in USES[p]:
            v = _accumulate(acc, c, sign, m)
            if last[c] == p:
                emit(c // 2, c % 2, v)
        fill(m)


def _combine(m):
    add = lambda a, b: [x + y for x, y in zip(a, b)]
    sub = lambda a, b: [x - y for x, y in zip(a, b)]
    m1 = m(0)
    m4 = m(3)
    c11 = add(m1, m4)
    m2 = m(1)
    c21 = add(m2, m4)
    c22 = sub(m1, m2)
    c11 = add(c11, m(6))
    m5 = m(4)
    c11 = sub(c11, m5)
    m3 = m(2)
    c12 = add(m3, m5)
    c22 = add(c22, m3)
    c22 = add(c22, m(5))
    return c11, c12, c21, c22


def _strassen2(prod, fill):
    def inner(n):
        r = prod(n)
        fill(r)
        return [r]

    def outer(p):
        a, b, c, d = _combine(lambda q: inner(7 * p + q))
        return b + a + d + c if p in SWAPPED else a + b + c + d
    c = _combine(outer)
    return [[c[2 * (r // 2) + k // 2][2 * (r % 2) + k % 2] for k in range(4)] for r in range(4)]


def _pack(v):
    return pltpu.bitcast(v.astype(BF), U32)


def _pack_all(tiles):
    return _pack(jnp.concatenate(tiles, axis=0)).reshape(-1, RS, LANES)


def _operand(ref, n, tiles, groups=slice(None)):
    v = jnp.concatenate([ref[t, groups, n].reshape(-1, LANES) for t in tiles], axis=1)
    return pltpu.bitcast(v, BF)


def _mm(a, b):
    return jnp.dot(a, b, preferred_element_type=F32)


def _skew(tiles):
    return [x if a == 0 else pltpu.roll(x, 4 * a, 1) for a, x in enumerate(tiles)]


def _unskew(t):
    lane = lax.broadcasted_iota(jnp.int32, t[0].shape, 1)
    t = [t[(-c) % 8] for c in range(8)]
    for b in (1, 2, 4):
        m = (lane & (4 * b)) != 0
        t = [lax.select(m, t[(c - b) % 8], t[c]) for c in range(8)]
    return [x if c == 0 else pltpu.roll(x, LANES - 4 * c, 1) for c, x in enumerate(t)]


def _gelu(x):
    c = math.sqrt(2.0 / math.pi)
    inner = x * (c + (c * 0.044715) * (x * x))
    hx = 0.5 * x
    return hx + hx * jnp.tanh(inner)


def _paced(work, steps, first, last):
    calls = [0]

    def fill(r):
        calls[0] += 1
        if calls[0] == first:
            next(work)
        if first <= calls[0] <= last:
            k, n = calls[0] - first, last - first + 1
            rows, tiles = r.shape[0] // RS, r.shape[1] // LANES
            for g in range(-(-k * steps // n), -(-(k + 1) * steps // n)):
                t, a = divmod((g * n - k * steps) * rows * tiles // steps, rows)
                try:
                    work.send(r[a * RS:(a + 1) * RS, t * LANES:(t + 1) * LANES])
                    assert g + 1 < steps
                except StopIteration:
                    assert g + 1 == steps
    return fill


def _run(work):
    for _ in work:
        pass


def _kernel(x_h, wqkv_h, wo_h, wg_h, wu_h, wd_h, o_h, x_s, wq, wo, wgu, wd, xc, qkv, cen):
    S, D = x_h.shape
    QF = wd_h.shape[1]
    NT, NB, NJ = D // LANES, S // TM, QF // LANES
    HM, HD, QM, QD = TM // 2, D // 2, TM // 4, D // 4
    TN = 2 * LANES
    NP = 7 * HD // TN
    CH = HD // 4
    CK = -(-HD // (RA * (NB - 2))) * RA
    mo = pl.multiple_of
    lanes = lambda t: slice(t * LANES, (t + 1) * LANES)
    add = lambda a, b: a + b
    never = [None]

    def new_region(zero):
        never[0] = lax.broadcasted_iota(jnp.int32, (RS, LANES), 1) < zero

    def behind(dep, v):
        if dep is None:
            return v
        return lax.select(never[0], dep if dep.dtype == v.dtype else pltpu.bitcast(dep, v.dtype), v)

    def f32_behind(dep, v):
        if v.dtype == F32:
            return v if dep is None else jnp.concatenate([behind(dep, v[:RS]), behind(dep, v[RS:])], axis=0)
        return pltpu.bitcast(behind(dep, v if v.dtype == U32 else pltpu.bitcast(v, U32)), BF).astype(F32)

    def layer_norm(src, rows):
        at = lambda k, t: (slice(k * RA, (k + 1) * RA), lanes(t))
        rows = [pl.ds(mo(r, RA), RA) for r in rows]
        ld = lambda k, t: src[rows[k], lanes(t)]
        ms, rs = [], []
        for k in range(len(rows)):
            d = yield
            xs = [f32_behind(d if src.dtype == BF or t == 0 else None, ld(k, t)) for t in range(NT)]
            if src.dtype == BF:
                for t in range(NT):
                    cen[at(k, t)] = xs[t]
            m = jnp.sum(functools.reduce(add, xs), axis=-1, keepdims=True)
            ms.append(jnp.broadcast_to(m * (1.0 / D), (RA, LANES)))
        for k in range(len(rows)):
            sq = []
            for t in range(NT):
                if t % (NT // 2) == 0:
                    m = f32_behind((yield), ms[k])
                c = (cen[at(k, t)] if src.dtype == BF else ld(k, t)) - m
                cen[at(k, t)] = c
                sq.append(c * c)
            v = jnp.sum(functools.reduce(add, sq), axis=-1, keepdims=True)
            rs.append(jnp.broadcast_to(lax.rsqrt(v * (1.0 / D) + EPS), (RA, LANES)))
        yield
        return lambda k, t, d: cen[at(k, t)] * f32_behind(d, rs[k])

    def operands49(f, load, put, swapped=()):
        quad = lambda a, b, d: [load(2 * a + r, 2 * b + c, d) for r in range(2) for c in range(2)]
        later = lambda q, d: [f32_behind(d, v) for v in q]
        index = (2, 3, 0, 4, 6, 5, 1) if f is _lhs7 else (1, 4, 0, 5, 2, 3, 6)

        def inner(e, q):
            for n, v in enumerate(f(q[1], q[0], q[3], q[2]) if index[e] in swapped else f(*q)):
                put(7 * index[e] + n, _pack(v))
        q11 = quad(0, 0, (yield))
        inner(0, q11)
        q22 = quad(1, 1, (yield))
        inner(1, q22)
        q22 = later(q22, (yield))
        inner(2, [a + b for a, b in zip(q11, q22)])
        q12 = quad(0, 1, (yield))
        inner(3, [a + b for a, b in zip(q11, q12)])
        inner(4, [a - b for a, b in zip(later(q12, (yield)), q22)])
        q21 = quad(1, 0, (yield))
        inner(5, [a - b for a, b in zip(q21, q11)])
        inner(6, [a + b for a, b in zip(later(q21, (yield)), q22)])

    def project(w_ref, p, i, fill):
        for c0 in range(0, HD, TN):
            def emit(a, b, v):
                for t in range(TN // LANES):
                    qkv[p * NT + (b * HD + c0) // LANES + t, pl.ds(mo(i * TM + (HALO + a * HM), RS), HM)] = (
                        v[:, lanes(t)])
            tiles = [(p // 2 * HD + c) // LANES for c in range(c0, c0 + TN, LANES)]
            _strassen1(lambda n: _mm(_operand(xc, n, range(NT // 2), pl.ds(i * (HM // RA), HM // RA)),
                                     _operand(w_ref, n, tiles)), fill, emit)

    def projections(wkv, stage_kv, tmp, stage_g, stage_u, stage_d, stage_o, xsem, wsem, ksem, fsem):
        CU, CD = QD // NB, QF // NB

        def x_cp(i):
            rows = pl.ds(mo(i * TM, TM), TM)
            return pltpu.make_async_copy(x_h.at[rows], x_s.at[rows], xsem.at[i])

        def q_cp(c):
            return [pltpu.make_async_copy(wqkv_h.at[k, pl.ds(mo(c * CH, CH), CH), pl.ds(0, D)],
                                          x_s.at[pl.ds(mo(S - D + k * HD + c * CH, CH), CH)], wsem.at[c])
                    for k in range(2)]

        def start(copies):
            for c in copies:
                c.start()

        def kv_group(i):
            return jnp.minimum(i * (CK // RA), (HD - CK) // RA)

        def kv_cp(i):
            return pltpu.make_async_copy(wqkv_h.at[:, pl.ds(mo(kv_group(i) * RA, RA), CK), pl.ds(D, 2 * D)],
                                         stage_kv.at[i % 2], ksem.at[i % 2])

        def ffn_cp(i):
            return [pltpu.make_async_copy(src.at[:, pl.ds(mo(i * n, RA), n)], dst.at[i % 2], fsem.at[i % 2])
                    for src, dst, n in ((wg_h, stage_g, CU), (wu_h, stage_u, CU), (wd_h, stage_d, CD),
                                        (wo_h, stage_o, CU))]

        def norm_work(row, group, rs):
            tile = yield from layer_norm(x_s, [row + (k * HM + r) for r in rs for k in range(2)])
            for g, r in enumerate(rs):
                for t in range(NT // 2):
                    d = yield
                    q = [tile(2 * g + k, n * NT // 2 + t, d) for k in range(2) for n in range(2)]
                    xc[t, group(r // RA)] = _pack_all(_lhs7(*q))

        def qkv_weight_work(w_ref, items):
            for e, (load, _, _) in enumerate(items):
                for k in range(2):
                    d = yield
                    ts = [behind(d, pltpu.bitcast(load(k, t), U32)) for t in range(NT)]
                    tmp[2 * e + k] = jnp.concatenate(_skew(ts), axis=1)
            for e in range(2 * len(items)):
                d = yield
                tmp[e] = jnp.concatenate(_unskew([behind(d, tmp[e, :, lanes(t)]) for t in range(NT)]), axis=1)
            for e, (_, tile, group) in enumerate(items):
                for t in range(NT // 2):
                    d = yield
                    q = [f32_behind(d, tmp[2 * e + k, :, lanes(n * NT // 2 + t)])
                         for k in range(2) for n in range(2)]
                    w_ref[tile + t, group] = _pack_all(_rhs7(*q))

        def other_weight_work(i):
            s = i % 2
            for e, src in enumerate((stage_g, stage_u)):
                for r in range(0, CU, RA):
                    group = i * (CU // RA) + r // RA
                    for j in range(NJ):
                        def put(n, v):
                            wgu[2 * j + e, group, n] = v
                        yield from operands49(
                            _rhs7, lambda k, n, d: f32_behind(d, src[s, k, r:r + RA, lanes(n * NJ + j)]), put, SWAPPED)
            for src, dst, rows in ((stage_d, wd, CD), (stage_o, wo, CU)):
                for r in range(0, rows, RA):
                    group = i * (rows // RA) + r // RA
                    for t in range(NT // 4):
                        def put(n, v):
                            dst[t, group, n] = v
                        yield from operands49(
                            _rhs7, lambda k, n, d: f32_behind(d, src[s, k, r:r + RA, lanes(n * NT // 4 + t)]),
                            put, SWAPPED)
        other_steps = 7 * (2 * CU * NJ + (CD + CU) * NT // 4) // RA

        x_cp(0).start()
        start(q_cp(0))
        start(q_cp(1))
        stage_kv[1] = jnp.zeros(stage_kv.shape[1:], BF)
        x_cp(0).wait()
        start(q_cp(2))
        lax.fori_loop(0, 2, lambda r, _: _run(norm_work(r * QM, lambda e: r * (QM // RA) + e, range(0, QM, RA))), None)

        def first_weights(c, _):
            for cp in q_cp(c):
                cp.wait()
            pl.when(c == 0)(lambda: start(q_cp(3)))
            pl.when(c == 1)(x_cp(1).start)
            _run(qkv_weight_work(wq, [(lambda k, t, r=r: x_s[pl.ds(mo(c * CH + (S - D + k * HD + r), RA), RA), lanes(t)],
                                       0, c * (CH // RA) + r // RA) for r in range(0, CH, RA)]))
        lax.fori_loop(0, 4, first_weights, None)

        def q_step(i, _):
            new_region(jnp.minimum(i, 0))

            @pl.when(i + 2 < NB)
            def _():
                x_cp(i + 2).start()
                kv_cp(i).start()
            for n, c in enumerate(ffn_cp(0)):
                pl.when(i == NB - 5 + n)(c.start)
            x_cp(i + 1).wait()
            pl.when(i > 0)(lambda: kv_cp(i - 1).wait())
            fn = _paced(norm_work(i * TM + TM, lambda e: i * (HM // RA) + (HM // RA + e), range(0, HM, RA)),
                        10 * HM // RA + 1, 1, NP // 2)
            slot, group = 1 - i % 2, kv_group(jnp.maximum(i - 1, 0))
            items = [(lambda k, t, p=p, r=r: stage_kv[slot, k, r:r + RA, lanes(p * NT + t)],
                      p * NT // 2, group + r // RA)
                     for p in range(2) for r in range(0, CK, RA)]
            fw = _paced(qkv_weight_work(wkv, items), 8 * len(items), NP // 2 + 1, NP - 1)
            project(wq, 0, i, lambda r: (fn(r), fw(r)))
        lax.fori_loop(0, NB - 1, q_step, None)

        def kv_step(i, _):
            new_region(jnp.minimum(i, 0))

            @pl.when(i + 1 < NB)
            def _():
                for c in ffn_cp(i + 1):
                    c.start()
            for c in ffn_cp(i):
                c.wait()
            fw = _paced(other_weight_work(i), other_steps, 1, 2 * NP - 2)
            project(wkv, 1, i, fw)
            project(wkv, 2, i, fw)
        lax.fori_loop(0, NB, kv_step, None)

    def blocks(h_s, hc, ac, oc, o_s, osem, word):
        scale = (D // H) ** -0.5
        attn_steps = (8 * (NT + W) + 7 * NT // 4) * QM // RA + 2 * W
        norm_steps = (12 + 7 * NT // 4) * QM // RA

        ready = set()

        def attn_work(base, rs, first):
            lane = lax.broadcasted_iota(jnp.int32, (RS, LANES), 1)

            rows = functools.cache(lambda r: pl.ds(base + (HALO + r), RS))
            ready.clear()
            done = []

            def taps(r0, t):
                for back in range(-RS, DIL * W, DIL):
                    v = qkv[t, rows(r0 - back), :]
                    yield v, [(g, (back + g * RS) // DIL) for g in range(2) if 0 <= back + g * RS < DIL * W]

            def fold(ls, b):
                other = lane ^ b
                return [a + jnp.take_along_axis(a, other, axis=1, mode="promise_in_bounds") for a in ls]

            def logits(r0):
                acc = {}
                for t in range(NT):
                    q = []
                    for g in range(2):
                        q.append(behind((yield), qkv[t, rows(r0 + g * RS), :]))
                    for v, uses in taps(r0, NT + t):
                        for g, w in uses:
                            _accumulate(acc, (g, w), 1, q[g] * v)
                return fold([acc[g, w] for g in range(2) for w in range(W)], 1)

            def softmax(r0, ls):
                ls = fold(ls, 2)
                out = []
                for g in range(2):
                    lg = ls[g * W:(g + 1) * W]
                    if first and r0 < HALO:
                        pos = r0 + g * RS + lax.broadcasted_iota(jnp.int32, (RS, LANES), 0)
                        lg = [jnp.where(pos >= DIL * w, a, -1e9 / scale) for w, a in enumerate(lg)]
                    m = functools.reduce(jnp.maximum, lg)
                    ps = [jnp.exp2((a - m) * (scale * math.log2(math.e))) for a in lg]
                    inv = 1.0 / functools.reduce(add, ps)
                    out.append([p * inv for p in ps])
                return out

            def values(r0, ps):
                acc = {}
                for v, uses in taps(r0, pl.ds(2 * NT, NT)):
                    for g, w in uses:
                        d = yield
                        if done and w == W - 1:
                            d = pltpu.bitcast(d, U32) | done.pop()
                        _accumulate(acc, g, 1, behind(d, ps[g][w])[None] * v)
                return _skew([_pack(jnp.concatenate([acc[0][t], acc[1][t]], axis=0)) for t in range(NT)])

            starts = [r + k * QM for r in rs for k in range(4)]
            ls, ps, outs = {}, {}, {}
            for n in range(-1, len(starts) + 1):
                if n + 1 < len(starts):
                    ls[n + 1] = yield from logits(starts[n + 1])
                if n > 0:
                    outs[n - 1] = _unskew(outs[n - 1])
                if 0 <= n < len(starts):
                    outs[n] = yield from values(starts[n], ps[n])
                else:
                    for _ in range(W):
                        yield
                if n + 1 < len(starts):
                    ps[n + 1] = softmax(starts[n + 1], ls[n + 1])
                if n > 0 and n % 4 == 0:
                    for t in range(NT // 4):
                        def put(p, v):
                            oc[t, starts[n - 4] // RA, p] = v
                            ready.add((t, starts[n - 4], p))
                            done[:] = [v | done[0]] if done else [v]
                        yield from operands49(_lhs7, lambda k, e, d: f32_behind(d, outs[n - 4 + k][e * NT // 4 + t]), put)

        def out_proj(i, slot, rs, fill):
            assert all((t, r, p) in ready for t in range(NT // 4) for r in rs for p in range(49))
            groups = pl.ds(rs[0] // RA, len(rs))
            for t in range(NT // 4):
                y = _strassen2(lambda n: _mm(_operand(oc, n, range(NT // 4), groups), _operand(wo, n, [t])), fill)
                for a in range(4):
                    for b in range(4):
                        cols = lanes(b * NT // 4 + t)
                        h_s[pl.ds(mo(slot * TM + (a * QM + rs[0]), RA), len(rs) * RA), cols] = (
                            x_s[pl.ds(mo(i * TM + (a * QM + rs[0]), RA), len(rs) * RA), cols].astype(F32) + y[a][b])

        def norm_work(slot, rs):
            tile = yield from layer_norm(h_s, [slot * TM + (k * QM + r) for r in rs for k in range(4)])
            for g, r in enumerate(rs):
                for t in range(NT // 4):
                    def put(p, v):
                        hc[t, r // RA, p] = v
                    yield from operands49(_lhs7, lambda k, n, d: tile(4 * g + k, n * NT // 4 + t, d), put)

        def halo(t, _):
            qkv[t, 0:HALO, :] = jnp.broadcast_to(qkv[t, HALO:HALO + 1, :], (HALO, LANES))
        word[0] = 0
        lax.fori_loop(NT, 3 * NT, halo, None, unroll=8)

        new_region(word[0])
        half = [range(h * QM // 2, (h + 1) * QM // 2, RA) for h in range(2)]
        split, calls = 11, [0]
        fa = _paced(attn_work(0, range(0, QM, RA), True), attn_steps, 1, 16 * split + 65)
        fn = [_paced(norm_work(0, half[0]), norm_steps // 2 + 1, 1, 84),
              _paced(norm_work(0, half[1]), norm_steps // 2 + 1, min(split + 1, NP), NP)]

        def fill(r):
            calls[0] += 1
            if calls[0] <= split:
                for t in range(TN // LANES):
                    for a in range(0, HM, RA):
                        fa(r[a:a + RA, lanes(t)])
            fn[1](r)
            if calls[0] == split:
                out_proj(0, 0, half[0], fa)
                out_proj(0, 0, half[1], fn[0])
        project(wq, 0, NB - 1, fill)

        def out_cp(i, slot, k):
            return pltpu.make_async_copy(o_s.at[slot, pl.ds(k * HM, HM)],
                                         o_h.at[pl.ds(mo(i * TM + k * HM, HM), HM)], osem.at[2 * slot + k])

        def step(i, _):
            slot = i % 2
            new_region(jnp.minimum(i, 0))

            @pl.when(i >= 2)
            def _():
                out_cp(i - 2, slot, 0).wait()
                out_cp(i - 2, slot, 1).wait()
            nxt = jnp.minimum(i + 1, NB - 1)
            fa = _paced(attn_work(nxt * TM, range(0, QM, RA), False), attn_steps, 1, 98 * NJ - 40)
            for j in range(NJ):
                g = _strassen2(lambda n: _mm(_operand(hc, n, range(NT // 4)), _operand(wgu, n, [2 * j])), fa)
                g = [[_gelu(v) for v in row] for row in g]
                u = _strassen2(lambda n: _mm(_operand(hc, n, range(NT // 4)), _operand(wgu, n, [2 * j + 1])), fa)
                for p, v in enumerate(_lhs49([[a * b for a, b in zip(*gu)] for gu in zip(g, u)])):
                    ac[j, :, p] = _pack(v).reshape(-1, RS, LANES)
            out_proj(nxt, 1 - slot, range(0, QM, RA), lambda r: None)
            fn = _paced(norm_work(1 - slot, range(0, QM, RA)), norm_steps + 1, 1, 49 - 7)
            y = _strassen2(lambda n: _mm(_operand(ac, n, range(NJ)), _operand(wd, n, range(NT // 4))), fn)
            for a in range(4):
                for b in range(4):
                    cols = pl.ds(b * QD, QD)
                    o_s[slot, a * QM:(a + 1) * QM, cols] = (
                        h_s[pl.ds(mo(slot * TM + a * QM, QM), QM), cols] + y[a][b]).astype(o_s.dtype)
                if a % 2:
                    out_cp(i, slot, a // 2).start()
        lax.fori_loop(0, NB, step, None)
        for i in (NB - 2, NB - 1):
            out_cp(i, i % 2, 0).wait()
            out_cp(i, i % 2, 1).wait()

    V, DMA = pltpu.VMEM, pltpu.SemaphoreType.DMA
    pl.run_scoped(projections, V((NT, HD // RA, 7, RS, LANES), U32), V((2, 2, CK, 2 * D), BF),
                  V((4 * CK // RA, RS, D), U32), V((2, 4, QD // NB, 4 * QF), BF), V((2, 4, QD // NB, 4 * QF), BF),
                  V((2, 4, QF // NB, D), BF), V((2, 4, QD // NB, D), BF), DMA((NB,)), DMA((4,)), DMA((2,)), DMA((2,)))
    pl.run_scoped(blocks, V((2 * TM, D), F32), V((NT // 4, QM // RA, 49, RS, LANES), U32),
                  V((NJ + 1, QM // RA, 49, RS, LANES), U32), V((NT // 4, QM // RA, 49, RS, LANES), U32),
                  V((2, TM, D), o_h.dtype), DMA((4,)), pltpu.SMEM((1,), jnp.int32))


@jax.jit
def pallas_sequential_preLN__sliding_local_dilated__glu_gated_geglu__prompt_kernel(
        A_x, A_wqkv, A_wo, B_x, B_w_gate, B_w_up, B_w_down):
    del B_x
    B, S, D = A_x.shape
    F = B_w_gate.shape[1]
    hbm = pl.BlockSpec(memory_space=pl.ANY)
    operands = lambda cols, rows, n: pltpu.VMEM((cols // LANES, rows // RA, n, RS, LANES), U32)
    out = pl.pallas_call(
        _kernel,
        in_specs=[hbm] * 6,
        out_specs=hbm,
        out_shape=jax.ShapeDtypeStruct((S, D), A_x.dtype),
        scratch_shapes=[
            pltpu.VMEM((S, D), BF), operands(D // 2, D // 2, 7), operands(D // 4, D // 4, 49),
            operands(F // 2, D // 4, 49), operands(D // 4, F // 4, 49), operands(D // 2, S // 2, 7),
            pltpu.VMEM((3 * D // LANES, S + HALO, LANES), F32), pltpu.VMEM((TM, D), F32),
        ],
        compiler_params=pltpu.CompilerParams(vmem_limit_bytes=127 * 1024 * 1024),
    )(A_x.reshape(S, D), A_wqkv.reshape(2, D // 2, 3 * D), A_wo.reshape(4, D // 4, D),
      B_w_gate.reshape(4, D // 4, F), B_w_up.reshape(4, D // 4, F), B_w_down.reshape(4, F // 4, D))
    return out.reshape(B, S, D)
```
